```python
import jax
import jax.numpy as jnp

def _softmax(x, axis=-1):
    return jax.nn.softmax(x, axis=axis)

def _gelu(x):
    return jax.nn.gelu(x, approximate=True)

def _silu(x):
    return jax.nn.silu(x)

def _sigmoid(x):
    return jax.nn.sigmoid(x)

def _layernorm(x, axis=-1, eps=1e-05):
    m = jnp.mean(x, axis=axis, keepdims=True)
    v = jnp.var(x, axis=axis, keepdims=True)
    return (x - m) / jnp.sqrt(v + eps)

def _scatter_add(tgt, idx, src, axis=0):
    return tgt.at[idx].add(src)

def _segment_sum(src, seg, n):
    return jax.ops.segment_sum(src, seg, n)

class _Rng:

    def __init__(self, key):
        self._k = key

    def _next(self):
        self._k, sub = jax.random.split(self._k)
        return sub

    def normal(self, shape):
        return jax.random.normal(self._next(), shape, dtype=jnp.bfloat16)

    def randint(self, lo, hi, shape):
        return jax.random.randint(self._next(), shape, lo, hi, dtype=jnp.int32)

    def uniform(self, shape, lo=0.0, hi=1.0):
        return jax.random.uniform(self._next(), shape, jnp.bfloat16, lo, hi)

    def permutation(self, n):
        return jax.random.permutation(self._next(), n)
kernel_name = 'interleave_layers__sliding_local_dilated__memory_aug_infini_attn__prompt'

def setup_inputs():
    _rng = _Rng(jax.random.key(int.from_bytes(__import__("os").urandom(4), "little")))
    _w = lambda a: (lambda t: t.astype(jnp.bfloat16) if jnp.issubdtype(t.dtype, jnp.floating) else t)(jnp.asarray(a))

    def _A_setup():
        B, S, D = (1, 2048, 1024)
        return {'x': _w((lambda *s: _rng.normal(s) * 0.05)(B, S, D)), 'wqkv': _w((lambda *s: _rng.normal(s) * 0.05)(D, 3 * D)), 'wo': _w((lambda *s: _rng.normal(s) * 0.05)(D, D))}
    _A_in = _A_setup()

    def _B_setup():
        B, S, D, H = (1, 2048, 1024, 32)
        N = 4
        L = max(1, S // N)
        sc = D ** (-0.5)
        return {'x': _w((lambda *s: _rng.normal(s) * 0.05)(B, N * L, D)), 'wq': _w((lambda *s: _rng.normal(s) * 0.05)(D, D) * sc), 'wk': _w((lambda *s: _rng.normal(s) * 0.05)(D, D) * sc), 'wv': _w((lambda *s: _rng.normal(s) * 0.05)(D, D) * sc), 'wo': _w((lambda *s: _rng.normal(s) * 0.05)(D, D) * sc), 'beta': _w((lambda *s: _rng.normal(s) * 0.05)(H))}
    _B_in = _B_setup()
    return {'A_x': _A_in['x'], 'A_wqkv': _A_in['wqkv'], 'A_wo': _A_in['wo'], 'B_x': _B_in['x'], 'B_wq': _B_in['wq'], 'B_wk': _B_in['wk'], 'B_wv': _B_in['wv'], 'B_wo': _B_in['wo'], 'B_beta': _B_in['beta']}

def reference(A_x, A_wqkv, A_wo, B_x, B_wq, B_wk, B_wv, B_wo, B_beta):

    def _A_ref(x, wqkv, wo):
        B, S, D = x.shape
        H = 32
        Dh = D // H
        W, dil = (8, 2)
        qkv = (lambda x, *d: x.transpose(*d))((x @ wqkv).reshape(B, S, 3, H, Dh), 2, 0, 3, 1, 4)
        q, k, v = (qkv[0], qkv[1], qkv[2])
        scale = Dh ** (-0.5)
        pos = jnp.arange(S)
        off = jnp.arange(W) * dil
        idx = pos[:, None] - off[None, :]
        mask = idx >= 0
        idx_c = jnp.where(mask, idx, 0).reshape(-1)
        kg = k[:, :, idx_c, :].reshape(B, H, S, W, Dh)
        vg = v[:, :, idx_c, :].reshape(B, H, S, W, Dh)
        logits = jnp.einsum('bhsd,bhswd->bhsw', q, kg) * scale
        logits = jnp.where(mask[None, None, :, :], logits, -1000000000.0)
        attn = _softmax(logits, axis=-1)
        o = jnp.einsum('bhsw,bhswd->bhsd', attn, vg)
        return (lambda x, *d: x.transpose(*d))(o, 0, 2, 1, 3).reshape(B, S, D) @ wo

    def _B_ref(x, wq, wk, wv, wo, beta):
        B, S, D = x.shape
        H = 32
        Dh = D // H
        N = 4
        L = S // N
        q = (lambda x, *d: x.transpose(*d))((x @ wq).reshape(B, S, H, Dh), 0, 2, 1, 3).reshape(B, H, N, L, Dh)
        k = (lambda x, *d: x.transpose(*d))((x @ wk).reshape(B, S, H, Dh), 0, 2, 1, 3).reshape(B, H, N, L, Dh)
        v = (lambda x, *d: x.transpose(*d))((x @ wv).reshape(B, S, H, Dh), 0, 2, 1, 3).reshape(B, H, N, L, Dh)
        phi = lambda t: jnp.where(t > 0, t + 1.0, jnp.exp(t))
        scale = Dh ** (-0.5)
        ar = jnp.arange(L)
        mask = (lambda x, dt: x.astype(dt))(ar[:, None] < ar[None, :], x.dtype) * -1000000000.0
        g = _sigmoid(beta).reshape(1, H, 1, 1)
        M = jnp.einsum('bhd,bhe->bhde', q[:, :, 0, 0, :] * 0.0, q[:, :, 0, 0, :] * 0.0)
        z = q[:, :, 0, 0, :] * 0.0
        outs = []
        for s in range(N):
            qs, ks, vs = (q[:, :, s].copy(), k[:, :, s].copy(), v[:, :, s].copy())
            logits = jnp.einsum('bhqd,bhkd->bhqk', qs, ks) * scale + mask
            p = _softmax(logits, axis=-1)
            a_dot = jnp.einsum('bhqk,bhkd->bhqd', p, vs)
            pq = phi(qs)
            num = jnp.einsum('bhld,bhde->bhle', pq, M)
            den = jnp.einsum('bhld,bhd->bhl', pq, z)[..., None] + 1e-06
            a_mem = num / den
            o = g * a_mem + (1.0 - g) * a_dot
            outs.append(o)
            pk = phi(ks)
            M = M + jnp.einsum('bhld,bhle->bhde', pk, vs)
            z = z + jnp.einsum('bhld->bhd', pk)
        o = (lambda x, *d: x.transpose(*d))(jnp.stack(outs, 2).reshape(B, H, S, Dh), 0, 2, 1, 3).reshape(B, S, D)
        return o @ wo
    x = A_x
    x = x + _A_ref(_layernorm(x, axis=-1), A_wqkv, A_wo)
    x = x + _B_ref(_layernorm(x, axis=-1), B_wq, B_wk, B_wv, B_wo, B_beta)
    x = x + _A_ref(_layernorm(x, axis=-1), A_wqkv, A_wo)
    x = x + _B_ref(_layernorm(x, axis=-1), B_wq, B_wk, B_wv, B_wo, B_beta)
    return x
```

```python
import functools
import math

import jax
import jax.numpy as jnp
import numpy as np
from jax import lax
from jax.experimental import pallas as pl
from jax.experimental.pallas import tpu as pltpu

S, D, H, DH = 2048, 1024, 32, 32
NSEG = 4
L = S // NSEG
W, DIL = 8, 2
HALO = 16
NT = D // 128
LOG2E = math.log2(math.e)
QSCALE = DH ** -0.5 * LOG2E
NEG = -1e9 * LOG2E
F32, BF16 = jnp.float32, jnp.bfloat16

RC = 128
RA = 16


def _dot(a, b):
    return jnp.dot(a, b, preferred_element_type=F32)


def _dot_nt(a, b):
    return lax.dot_general(a, b, (((1,), (1,)), ((), ())), preferred_element_type=F32)


def _layernorm(x):
    m = jnp.mean(x, axis=-1, keepdims=True)
    xc = x - m
    v = jnp.mean(xc * xc, axis=-1, keepdims=True)
    return xc * lax.rsqrt(v + 1e-5)


def _phi(t):
    return jnp.where(t > 0, t + 1.0, jnp.exp(t))


def _kernel(x_ref, beta_ref, wqkv_hbm, woa_hbm, wq_hbm, wk_hbm, wv_hbm, wob_hbm, out_ref,
            raw_qkv, raw_woa, raw_wv, wa_t, woa, wqk, wv_t, wob, tbuf,
            xs, xn, qb, kb, vb, kc, vc, ob, mt, zs, gate, cmask, sems):
    seg = pl.program_id(0)
    rep = pl.program_id(1)

    @pl.when((seg == 0) & (rep == 0))
    def _prologue():
        cps = []
        for m in range(3):
            cps.append(pltpu.make_async_copy(wqkv_hbm.at[:, pl.ds(m * D, D)], raw_qkv.at[m], sems.at[m]))
        cps.append(pltpu.make_async_copy(woa_hbm, raw_woa, sems.at[3]))
        cps.append(pltpu.make_async_copy(wv_hbm, raw_wv, sems.at[4]))
        cps.append(pltpu.make_async_copy(wob_hbm, wob, sems.at[5]))
        for g in range(NT):
            cps.append(pltpu.make_async_copy(wq_hbm.at[:, pl.ds(g * 128, 128)],
                                             wqk.at[g, :, pl.ds(0, 128)], sems.at[6 + g]))
            cps.append(pltpu.make_async_copy(wk_hbm.at[:, pl.ds(g * 128, 128)],
                                             wqk.at[g, :, pl.ds(128, 128)], sems.at[14 + g]))
        for c in cps:
            c.start()
        kc[...] = jnp.zeros(kc.shape, F32)
        vc[...] = jnp.zeros(vc.shape, F32)
        mt[...] = jnp.zeros(mt.shape, F32)
        zs[...] = jnp.zeros(zs.shape, F32)
        g_all = jax.nn.sigmoid(beta_ref[...].astype(F32))
        lane = lax.broadcasted_iota(jnp.int32, (1, H), 1)
        for h in range(H):
            gh = jnp.sum(jnp.where(lane == h, g_all, 0.0), axis=1, keepdims=True)
            gate[h] = jnp.broadcast_to(gh, (8, 128))
        kk = lax.broadcasted_iota(jnp.int32, (128, 128), 0)
        qq = lax.broadcasted_iota(jnp.int32, (128, 128), 1)
        cmask[...] = jnp.where(qq < kk, NEG, 0.0).astype(F32)

        for m in range(3):
            cps[m].wait()

            def perm(j, carry, m=m):
                r0 = pl.multiple_of(j * 128, 128)
                tbuf[...] = raw_qkv[m, pl.ds(r0, 128), :].astype(F32).T
                for d in range(DH):
                    wa_t[j, pl.ds(m * D + d * H, H), :] = tbuf[pl.ds(d, H, stride=DH), :].astype(BF16)
                return carry
            lax.fori_loop(0, NT, perm, 0)
        cps[3].wait()
        for j in range(NT):
            tbuf[...] = raw_woa[:, j * 128:(j + 1) * 128].astype(F32)
            for d in range(DH):
                woa[d * H:(d + 1) * H, j * 128:(j + 1) * 128] = tbuf[pl.ds(d, H, stride=DH), :].astype(BF16)
        cps[4].wait()
        for g in range(NT):
            wv_t[g] = raw_wv[:, g * 128:(g + 1) * 128].astype(F32).T.astype(BF16)
        for c in cps[5:]:
            c.wait()

    @pl.when(rep == 0)
    def _load_x():
        xs[...] = x_ref[...].astype(F32)

    for c in range(NT):
        kb[c, 0:HALO, :] = kc[rep, c]
        vb[c, 0:HALO, :] = vc[rep, c]

    def a_proj(i):
        r0 = i * RC
        xb = _layernorm(xs[r0:r0 + RC, :]).astype(BF16)
        for m, dst in ((1, kb), (0, qb), (2, vb)):
            wt = jnp.concatenate([wa_t[j, m * D:(m + 1) * D, :] for j in range(NT)], axis=1)
            y = _dot_nt(xb, wt)
            for c in range(NT):
                yc = y[:, c * 128:(c + 1) * 128]
                if m == 0:
                    dst[c, r0:r0 + RC, :] = yc * QSCALE
                else:
                    dst[c, HALO + r0:HALO + r0 + RC, :] = yc

    def a_attn(r0):
        qs = [qb[c, r0:r0 + RA, :] for c in range(NT)]
        ls = []
        for w in range(W):
            o0 = HALO + r0 - DIL * w
            acc = qs[0] * kb[0, o0:o0 + RA, :]
            for c in range(1, NT):
                acc = acc + qs[c] * kb[c, o0:o0 + RA, :]
            acc = acc + pltpu.roll(acc, 64, 1)
            acc = acc + pltpu.roll(acc, 32, 1)
            if r0 < DIL * w:
                pos = seg * L + r0 + lax.broadcasted_iota(jnp.int32, (RA, 128), 0)
                acc = jnp.where(pos >= DIL * w, acc, NEG)
            ls.append(acc)
        mx = functools.reduce(jnp.maximum, ls)
        es = [jnp.exp2(l - mx) for l in ls]
        inv = 1.0 / functools.reduce(jnp.add, es)
        ps = [e * inv for e in es]
        for c in range(NT):
            acc = None
            for w in range(W):
                o0 = HALO + r0 - DIL * w
                t = ps[w] * vb[c, o0:o0 + RA, :]
                acc = t if acc is None else acc + t
            ob[c, r0:r0 + RA, :] = acc.astype(BF16)

    def out_proj(i, w_ref):
        r0 = i * RC
        o = jnp.concatenate([ob[c, r0:r0 + RC, :] for c in range(NT)], axis=1)
        xnew = xs[r0:r0 + RC, :] + _dot(o, w_ref[...])
        xs[r0:r0 + RC, :] = xnew
        return xnew

    nch = L // RC
    a_proj(0)
    for i in range(nch):
        if i + 1 < nch:
            a_proj(i + 1)
        for r0 in range(i * RC, (i + 1) * RC, RA):
            a_attn(r0)
        if i >= 1:
            xn[(i - 1) * RC:i * RC, :] = _layernorm(out_proj(i - 1, woa)).astype(BF16)
    xn[(nch - 1) * RC:nch * RC, :] = _layernorm(out_proj(nch - 1, woa)).astype(BF16)
    for c in range(NT):
        kc[rep, c] = kb[c, L:L + HALO, :]
        vc[rep, c] = vb[c, L:L + HALO, :]

    def b_group(g, carry):
        lane = lax.broadcasted_iota(jnp.int32, (1, 128), 1) // DH
        qk = _dot(xn[...], wqk[g])
        q, k = qk[:, :128], qk[:, 128:]
        vt = _dot_nt(wv_t[g], xn[...]).astype(BF16)
        kb16 = k.astype(BF16)
        qs = q * QSCALE
        pq = _phi(q).astype(BF16)
        pk = _phi(k)
        zrow = lax.broadcasted_iota(jnp.int32, (16, 128), 0)
        zl = jnp.where(zrow == lane, jnp.broadcast_to(zs[rep, g, 0:1, :], (16, 128)), 0.0)
        lhs = jnp.concatenate([mt[rep, g], zl], axis=0).astype(BF16)
        nd = _dot_nt(lhs, pq)
        outs = []
        for h in range(4):
            gh = gate[g * 4 + h][0:1, :]
            row = []
            for j in range(L // 128):
                nk = 128 * (j + 1)
                qm = jnp.where(lane == h, qs[j * 128:(j + 1) * 128, :], 0.0).astype(BF16)
                st = _dot_nt(kb16[:nk], qm)
                diag = st[nk - 128:] + cmask[...]
                st = diag if j == 0 else jnp.concatenate([st[:nk - 128], diag], axis=0)
                mx = jnp.max(st, axis=0, keepdims=True)
                p = jnp.exp2(st - mx)
                l = jnp.sum(p, axis=0, keepdims=True)
                pv = _dot(vt[h * DH:(h + 1) * DH, :nk], p.astype(BF16))
                num = nd[h * DH:(h + 1) * DH, j * 128:(j + 1) * 128]
                den = nd[128 + h:129 + h, j * 128:(j + 1) * 128] + 1e-6
                row.append(num * (gh / den) + pv * ((1.0 - gh) / l))
            outs.append(jnp.concatenate(row, axis=1))
        ot = jnp.concatenate(outs, axis=0)
        ob[g] = ot.T.astype(BF16)
        upd = _dot(vt, pk.astype(BF16))
        rr = lax.broadcasted_iota(jnp.int32, (128, 128), 0) // DH
        mt[rep, g] = mt[rep, g] + jnp.where(rr == lane, upd, 0.0)
        zs[rep, g] = zs[rep, g] + jnp.sum(pk, axis=0, keepdims=True)
        return carry

    lax.fori_loop(0, NT, b_group, 0)
    for i in range(nch):
        out_ref[i * RC:(i + 1) * RC, :] = out_proj(i, wob).astype(BF16)


@jax.jit
def pallas_interleave_layers__sliding_local_dilated__memory_aug_infini_attn__prompt_kernel(
        A_x, A_wqkv, A_wo, B_x, B_wq, B_wk, B_wv, B_wo, B_beta):
    del B_x
    hbm = pl.BlockSpec(memory_space=pl.ANY)
    out = pl.pallas_call(
        _kernel,
        grid=(NSEG, 2),
        in_specs=[pl.BlockSpec((L, D), lambda s, r: (s, 0)),
                  pl.BlockSpec((1, H), lambda s, r: (0, 0)),
                  hbm, hbm, hbm, hbm, hbm, hbm],
        out_specs=pl.BlockSpec((L, D), lambda s, r: (s, 0)),
        out_shape=jax.ShapeDtypeStruct((S, D), BF16),
        scratch_shapes=[
            pltpu.VMEM((3, D, D), BF16),
            pltpu.VMEM((D, D), BF16),
            pltpu.VMEM((D, D), BF16),
            pltpu.VMEM((NT, 3 * D, 128), BF16),
            pltpu.VMEM((D, D), BF16),
            pltpu.VMEM((NT, D, 256), BF16),
            pltpu.VMEM((NT, 128, D), BF16),
            pltpu.VMEM((D, D), BF16),
            pltpu.VMEM((D, 128), F32),
            pltpu.VMEM((L, D), F32),
            pltpu.VMEM((L, D), BF16),
            pltpu.VMEM((NT, L, 128), F32),
            pltpu.VMEM((NT, HALO + L, 128), F32),
            pltpu.VMEM((NT, HALO + L, 128), F32),
            pltpu.VMEM((2, NT, HALO, 128), F32),
            pltpu.VMEM((2, NT, HALO, 128), F32),
            pltpu.VMEM((NT, L, 128), BF16),
            pltpu.VMEM((2, NT, 128, 128), F32),
            pltpu.VMEM((2, NT, 8, 128), F32),
            pltpu.VMEM((H, 8, 128), F32),
            pltpu.VMEM((128, 128), F32),
            pltpu.SemaphoreType.DMA((22,)),
        ],
        compiler_params=pltpu.CompilerParams(
            dimension_semantics=("arbitrary", "arbitrary"),
            vmem_limit_bytes=100 * 2**20),
        name="interleave",
    )(A_x.reshape(S, D), B_beta.reshape(1, H), A_wqkv, A_wo, B_wq, B_wk, B_wv, B_wo)
    return out.reshape(1, S, D)
```

```python
import functools
import math

import jax
import jax.numpy as jnp
import numpy as np
from jax import lax
from jax.experimental import pallas as pl
from jax.experimental.pallas import tpu as pltpu

S, D, H, DH = 2048, 1024, 32, 32
NSEG = 4
L = S // NSEG
W, DIL = 8, 2
HALO = 16
NT = D // 128
LOG2E = math.log2(math.e)
QSCALE = DH ** -0.5 * LOG2E
NEG = -1e9 * LOG2E
F32, BF16, U32 = jnp.float32, jnp.bfloat16, jnp.uint32

RC = 128
RA = 16


def _dot(a, b):
    return jnp.dot(a, b, preferred_element_type=F32)


def _dot_nt(a, b):
    return lax.dot_general(a, b, (((1,), (1,)), ((), ())), preferred_element_type=F32)


def _pack(x):
    return pltpu.bitcast(x.astype(BF16), U32)


def _unpack(x):
    return pltpu.bitcast(x, BF16)


def _layernorm(x):
    m = jnp.mean(x, axis=-1, keepdims=True)
    xc = x - m
    v = jnp.mean(xc * xc, axis=-1, keepdims=True)
    return xc * lax.rsqrt(v + 1e-5)


def _phi(t):
    return jnp.where(t > 0, t + 1.0, jnp.exp(t))


def _kernel(x_ref, beta_ref, wqkv_hbm, woa_hbm, wq_hbm, wk_hbm, wv_hbm, wob_hbm, out_ref,
            raw_qkv, raw_woa, raw_wv, raw_b, wa_t, woa, wqk, wv_t, wob, tbuf,
            xs, xn, qb, kb, vb, kc, vc, ob, mt, zs, gate, cmask, sems):
    seg = pl.program_id(0)
    rep = pl.program_id(1)

    @pl.when((seg == 0) & (rep == 0))
    def _prologue():
        cps = []
        for m in range(3):
            cps.append(pltpu.make_async_copy(wqkv_hbm.at[:, pl.ds(m * D, D)], raw_qkv.at[m], sems.at[m]))
        cps.append(pltpu.make_async_copy(woa_hbm, raw_woa, sems.at[3]))
        cps.append(pltpu.make_async_copy(wv_hbm, raw_wv, sems.at[4]))
        for i, w in enumerate((wq_hbm, wk_hbm, wob_hbm)):
            cps.append(pltpu.make_async_copy(w, raw_b.at[i], sems.at[5 + i]))
        for c in cps:
            c.start()
        kc[...] = jnp.zeros(kc.shape, F32)
        vc[...] = jnp.zeros(vc.shape, F32)
        mt[...] = jnp.zeros(mt.shape, F32)
        zs[...] = jnp.zeros(zs.shape, F32)
        g_all = jax.nn.sigmoid(beta_ref[...].astype(F32))
        lane = lax.broadcasted_iota(jnp.int32, (1, H), 1)
        for h in range(H):
            gh = jnp.sum(jnp.where(lane == h, g_all, 0.0), axis=1, keepdims=True)
            gate[h] = jnp.broadcast_to(gh, (8, 128))
        kk = lax.broadcasted_iota(jnp.int32, (128, 128), 0)
        qq = lax.broadcasted_iota(jnp.int32, (128, 128), 1)
        cmask[...] = jnp.where(qq < kk, NEG, 0.0).astype(F32)

        for m in range(3):
            cps[m].wait()

            def perm(j, carry, m=m):
                r0 = pl.multiple_of(j * 128, 128)
                tbuf[...] = raw_qkv[m, pl.ds(r0, 128), :].astype(F32).T
                for d in range(DH):
                    wa_t[j, pl.ds((m * D + d * H) // 2, H // 2), :] = _pack(tbuf[pl.ds(d, H, stride=DH), :])
                return carry
            lax.fori_loop(0, NT, perm, 0)
        cps[3].wait()
        for j in range(NT):
            tbuf[...] = raw_woa[:, j * 128:(j + 1) * 128].astype(F32)
            for d in range(DH):
                woa[d * H // 2:(d + 1) * H // 2, j * 128:(j + 1) * 128] = _pack(tbuf[pl.ds(d, H, stride=DH), :])
        cps[4].wait()
        for g in range(NT):
            wv_t[g] = _pack(raw_wv[:, g * 128:(g + 1) * 128].astype(F32).T)
        for c in cps[5:]:
            c.wait()
        for g in range(NT):
            wqk[g, :, 0:128] = pltpu.bitcast(raw_b[0, :, g * 128:(g + 1) * 128], U32)
            wqk[g, :, 128:256] = pltpu.bitcast(raw_b[1, :, g * 128:(g + 1) * 128], U32)
        wob[...] = pltpu.bitcast(raw_b[2], U32)

    @pl.when(rep == 0)
    def _load_x():
        xs[...] = x_ref[...].astype(F32)

    for c in range(NT):
        kb[c, 0:HALO, :] = kc[rep, c]
        vb[c, 0:HALO, :] = vc[rep, c]

    def a_proj(i):
        r0 = i * RC
        xb = _layernorm(xs[r0:r0 + RC, :]).astype(BF16)
        for m, dst in ((1, kb), (0, qb), (2, vb)):
            wt = jnp.concatenate([_unpack(wa_t[j, m * D // 2:(m + 1) * D // 2, :]) for j in range(NT)], axis=1)
            y = _dot_nt(xb, wt)
            for c in range(NT):
                yc = y[:, c * 128:(c + 1) * 128]
                if m == 0:
                    dst[c, r0:r0 + RC, :] = yc * QSCALE
                else:
                    dst[c, HALO + r0:HALO + r0 + RC, :] = yc

    def a_attn(r0):
        qs = [qb[c, r0:r0 + RA, :] for c in range(NT)]
        ls = []
        for w in range(W):
            o0 = HALO + r0 - DIL * w
            acc = qs[0] * kb[0, o0:o0 + RA, :]
            for c in range(1, NT):
                acc = acc + qs[c] * kb[c, o0:o0 + RA, :]
            acc = acc + pltpu.roll(acc, 64, 1)
            acc = acc + pltpu.roll(acc, 32, 1)
            if r0 < DIL * w:
                pos = seg * L + r0 + lax.broadcasted_iota(jnp.int32, (RA, 128), 0)
                acc = jnp.where(pos >= DIL * w, acc, NEG)
            ls.append(acc)
        mx = functools.reduce(jnp.maximum, ls)
        es = [jnp.exp2(l - mx) for l in ls]
        inv = 1.0 / functools.reduce(jnp.add, es)
        ps = [e * inv for e in es]
        for c in range(NT):
            acc = None
            for w in range(W):
                o0 = HALO + r0 - DIL * w
                t = ps[w] * vb[c, o0:o0 + RA, :]
                acc = t if acc is None else acc + t
            ob[c, r0 // 2:(r0 + RA) // 2, :] = _pack(acc)

    def out_proj(i, w_ref):
        r0 = i * RC
        o = jnp.concatenate([_unpack(ob[c, r0 // 2:(r0 + RC) // 2, :]) for c in range(NT)], axis=1)
        xnew = xs[r0:r0 + RC, :] + _dot(o, _unpack(w_ref[...]))
        xs[r0:r0 + RC, :] = xnew
        return xnew

    nch = L // RC
    sc = jax.named_scope("sc_A"); sc.__enter__()
    a_proj(0)
    for i in range(nch):
        if i + 1 < nch:
            a_proj(i + 1)
        for r0 in range(i * RC, (i + 1) * RC, RA):
            a_attn(r0)
        if i >= 1:
            xn[(i - 1) * RC // 2:i * RC // 2, :] = _pack(_layernorm(out_proj(i - 1, woa)))
    xn[(nch - 1) * RC // 2:nch * RC // 2, :] = _pack(_layernorm(out_proj(nch - 1, woa)))
    for c in range(NT):
        kc[rep, c] = kb[c, L:L + HALO, :]
        vc[rep, c] = vb[c, L:L + HALO, :]

    def b_group(g, carry):
        lane = lax.broadcasted_iota(jnp.int32, (1, 128), 1) // DH
        qk = _dot(_unpack(xn[...]), _unpack(wqk[g]))
        q, k = qk[:, :128], qk[:, 128:]
        vt = _dot_nt(_unpack(wv_t[g]), _unpack(xn[...])).astype(BF16)
        kb16 = k.astype(BF16)
        qs = q * QSCALE
        nq = L // 128

        def scores(j):
            nk = 128 * (j + 1)
            qj = qs[j * 128:(j + 1) * 128, :]
            qm = jnp.concatenate([jnp.where(lane == h, qj, 0.0).astype(BF16) for h in range(4)], axis=0)
            st = _dot_nt(kb16[:nk], qm)
            cm = cmask[...]
            diag = st[nk - 128:] + jnp.concatenate([cm] * 4, axis=1)
            return diag if j == 0 else jnp.concatenate([st[:nk - 128], diag], axis=0)

        def attend(j, st):
            nk = 128 * (j + 1)
            mx = jnp.max(st, axis=0, keepdims=True)
            p = jnp.exp2(st - mx)
            l = jnp.sum(p, axis=0, keepdims=True)
            p = p.astype(BF16)
            pv = [_dot(vt[h * DH:(h + 1) * DH, :nk], p[:, h * 128:(h + 1) * 128]) for h in range(4)]
            return pv, l

        def memory():
            pq = _phi(q).astype(BF16)
            zrow = lax.broadcasted_iota(jnp.int32, (16, 128), 0)
            zl = jnp.where(zrow == lane, jnp.broadcast_to(zs[rep, g, 0:1, :], (16, 128)), 0.0)
            lhs = jnp.concatenate([mt[rep, g], zl], axis=0).astype(BF16)
            return _dot_nt(lhs, pq)

        def update():
            pk = _phi(k)
            pkb = pk.astype(BF16)
            upd = functools.reduce(jnp.add, [
                _dot(vt[:, i * 128:(i + 1) * 128], pkb[i * 128:(i + 1) * 128]) for i in range(nq)])
            rr = lax.broadcasted_iota(jnp.int32, (128, 128), 0) // DH
            mt[rep, g] = mt[rep, g] + jnp.where(rr == lane, upd, 0.0)
            zs[rep, g] = zs[rep, g] + jnp.sum(pk, axis=0, keepdims=True)

        def finish(j, res, nd):
            pv, l = res
            rows = []
            for h in range(4):
                gh = gate[g * 4 + h][0:1, :]
                num = nd[h * DH:(h + 1) * DH, j * 128:(j + 1) * 128]
                den = nd[128 + h:129 + h, j * 128:(j + 1) * 128] + 1e-6
                rows.append(num * (gh / den) + pv[h] * ((1.0 - gh) / l[:, h * 128:(h + 1) * 128]))
            ob[g, j * 64:(j + 1) * 64, :] = _pack(jnp.concatenate(rows, axis=0).T)

        s3 = scores(3)
        s2 = scores(2)
        nd = memory()
        finish(3, attend(3, s3), nd)
        s1 = scores(1)
        finish(2, attend(2, s2), nd)
        s0 = scores(0)
        finish(1, attend(1, s1), nd)
        update()
        finish(0, attend(0, s0), nd)
        return carry

    sc.__exit__(None, None, None)
    with jax.named_scope("sc_Bloop"):
        lax.fori_loop(0, NT, b_group, 0)
    with jax.named_scope("sc_Bout"):
        for i in range(nch):
            out_ref[i * RC:(i + 1) * RC, :] = out_proj(i, wob).astype(BF16)


@jax.jit
def pallas_interleave_layers__sliding_local_dilated__memory_aug_infini_attn__prompt_kernel(
        A_x, A_wqkv, A_wo, B_x, B_wq, B_wk, B_wv, B_wo, B_beta):
    del B_x
    hbm = pl.BlockSpec(memory_space=pl.ANY)
    out = pl.pallas_call(
        _kernel,
        grid=(NSEG, 2),
        in_specs=[pl.BlockSpec((L, D), lambda s, r: (s, 0)),
                  pl.BlockSpec((1, H), lambda s, r: (0, 0)),
                  hbm, hbm, hbm, hbm, hbm, hbm],
        out_specs=pl.BlockSpec((L, D), lambda s, r: (s, 0)),
        out_shape=jax.ShapeDtypeStruct((S, D), BF16),
        scratch_shapes=[
            pltpu.VMEM((3, D, D), BF16),
            pltpu.VMEM((D, D), BF16),
            pltpu.VMEM((D, D), BF16),
            pltpu.VMEM((3, D, D), BF16),
            pltpu.VMEM((NT, 3 * D // 2, 128), U32),
            pltpu.VMEM((D // 2, D), U32),
            pltpu.VMEM((NT, D // 2, 256), U32),
            pltpu.VMEM((NT, 64, D), U32),
            pltpu.VMEM((D // 2, D), U32),
            pltpu.VMEM((D, 128), F32),
            pltpu.VMEM((L, D), F32),
            pltpu.VMEM((L // 2, D), U32),
            pltpu.VMEM((NT, L, 128), F32),
            pltpu.VMEM((NT, HALO + L, 128), F32),
            pltpu.VMEM((NT, HALO + L, 128), F32),
            pltpu.VMEM((2, NT, HALO, 128), F32),
            pltpu.VMEM((2, NT, HALO, 128), F32),
            pltpu.VMEM((NT, L // 2, 128), U32),
            pltpu.VMEM((2, NT, 128, 128), F32),
            pltpu.VMEM((2, NT, 8, 128), F32),
            pltpu.VMEM((H, 8, 128), F32),
            pltpu.VMEM((128, 128), F32),
            pltpu.SemaphoreType.DMA((8,)),
        ],
        compiler_params=pltpu.CompilerParams(
            dimension_semantics=("arbitrary", "arbitrary"),
            vmem_limit_bytes=100 * 2**20),
        name="interleave",
    )(A_x.reshape(S, D), B_beta.reshape(1, H), A_wqkv, A_wo, B_wq, B_wk, B_wv, B_wo)
    return out.reshape(1, S, D)
```

```python
import functools
import math
import os

import jax
import jax.numpy as jnp
import numpy as np
from jax import lax
from jax.experimental import pallas as pl
from jax.experimental.pallas import tpu as pltpu

S, D, H, DH = 2048, 1024, 32, 32
NSEG = 4
L = S // NSEG
W, DIL = 8, 2
HALO = 16
NT = D // 128
HD = D // 2
PITCH = int(os.environ.get('PITCH', 33))
RC = 256
NCH = L // RC
LOG2E = math.log2(math.e)
QSCALE = DH ** -0.5 * LOG2E
NEG = -1e9 * LOG2E
F32, BF16, U32 = jnp.float32, jnp.bfloat16, jnp.uint32
STRASSEN = int(os.environ.get("STR", 1))
NP = 7 if STRASSEN else 4


def _dot(a, b):
    return jnp.dot(a, b, preferred_element_type=F32)


def _dot_nt(a, b):
    return lax.dot_general(a, b, (((1,), (1,)), ((), ())), preferred_element_type=F32)


def _pack(x):
    return pltpu.bitcast(x.astype(BF16), U32)


def _unpack(x):
    return pltpu.bitcast(x, BF16)


def _lhs_blocks(a11, a12, a21, a22):
    if STRASSEN:
        return [a11 + a22, a21 + a22, a11, a22, a11 + a12, a21 - a11, a12 - a22]
    return [a11, a12, a21, a22]


def _rhs_blocks(b11, b12, b21, b22):
    if STRASSEN:
        return [b11 + b22, b11, b12 - b22, b21 - b11, b22, b11 + b12, b21 + b22]
    return [b11, b12, b21, b22]


def _block_matmul(prod, done):
    if STRASSEN:
        p3 = prod(2, 2); yield
        p5 = prod(4, 4); yield
        done(0, 1, p3 + p5)
        p2 = prod(1, 1); yield
        p4 = prod(3, 3); yield
        done(1, 0, p2 + p4)
        u, v = p4 - p5, p3 - p2
        p1 = prod(0, 0); yield
        u, v = u + p1, v + p1
        p7 = prod(6, 6); yield
        done(0, 0, u + p7)
        p6 = prod(5, 5)
        done(1, 1, v + p6); yield
    else:
        for i in range(2):
            for j in range(2):
                t = prod(2 * i, j); yield
                done(i, j, t + prod(2 * i + 1, 2 + j)); yield


def _run(gen, n=None):
    k = 0
    while n is None or k < n:
        if next(gen, "end") == "end":
            break
        k += 1


def _chain(*gens):
    for g in gens:
        yield from g


def _layernorm(x):
    m = jnp.mean(x, axis=-1, keepdims=True)
    xc = x - m
    v = jnp.mean(xc * xc, axis=-1, keepdims=True)
    return xc * lax.rsqrt(v + 1e-5)


def _phi(t):
    return jnp.where(t > 0, t + 1.0, jnp.exp(t))


def _kernel(x_ref, beta_ref, wqkv_hbm, woa_hbm, wq_hbm, wk_hbm, wv_hbm, wob_hbm, out_ref,
            raw, wa, woa, wqk, wvt, wob, tbuf,
            xs, xa, xb, qb, kb, vb, kc, vc, of, oc, bq, bk, bv, mt, zs, gate, cmask, sems):
    seg = pl.program_id(0)
    rep = pl.program_id(1)

    def row_blocks(xn):
        return _lhs_blocks(xn[:128, :HD], xn[:128, HD:], xn[128:, :HD], xn[128:, HD:])

    def norm_blocks(ch):
        blocks = row_blocks(_layernorm(xs[ch * RC:(ch + 1) * RC, :]))
        for i, b in enumerate(blocks):
            xb[i, ch * 64:(ch + 1) * 64, :] = _pack(b)

    first_step = (seg == 0) & (rep == 0)
    c1 = 256
    srcs = [wqkv_hbm.at[:, pl.ds(D, D)], wqkv_hbm.at[:, pl.ds(0, D)], wqkv_hbm.at[:, pl.ds(2 * D, D)], woa_hbm]
    cps = [pltpu.make_async_copy(s, raw.at[i], sems.at[i]) for i, s in enumerate(srcs)]
    for i, s in enumerate((wq_hbm, wk_hbm, wv_hbm)):
        cps.append(pltpu.make_async_copy(s.at[:, pl.ds(0, c1)], raw.at[4 + i, :, pl.ds(0, c1)], sems.at[4 + i]))
    for i, s in enumerate((wq_hbm, wk_hbm, wv_hbm)):
        cps.append(pltpu.make_async_copy(s.at[:, pl.ds(c1, D - c1)], raw.at[4 + i, :, pl.ds(c1, D - c1)],
                                         sems.at[7 + i]))
    cps.append(pltpu.make_async_copy(wob_hbm, raw.at[7], sems.at[10]))

    def packed_blocks(b11, b12, b21, b22):
        quad = (b11, b12, b21, b22)
        vals = [_unpack(b).astype(F32) for b in quad]
        out = []
        for blk in _rhs_blocks(*vals):
            same = [i for i, v in enumerate(vals) if v is blk]
            out.append(quad[same[0]] if same else _pack(blk))
        return out

    def raw_u32(m, rows, cols):
        return pltpu.bitcast(raw[m, rows, cols], U32)

    def comb_qk(t, carry):
        p, j = t // 4, t % 4
        r0 = pl.multiple_of(j * 128, 128)
        c0 = pl.multiple_of(p * 256, 256)
        for m in range(2):
            top = raw_u32(4 + m, pl.ds(r0, 128), pl.ds(c0, 256))
            bot = raw_u32(4 + m, pl.ds(HD + r0, 128), pl.ds(c0, 256))
            for i, v in enumerate(packed_blocks(top[:, :128], top[:, 128:], bot[:, :128], bot[:, 128:])):
                wqk[p, i, pl.ds(pl.multiple_of(j * 64, 64), 64), m * 128:(m + 1) * 128] = v
        top = raw[6, pl.ds(r0, 128), pl.ds(c0, 256)].astype(F32).T
        bot = raw[6, pl.ds(HD + r0, 128), pl.ds(c0, 256)].astype(F32).T
        for i, v in enumerate(_rhs_blocks(top[:128], top[128:], bot[:128], bot[128:])):
            wvt[p, i, :, pl.ds(r0, 128)] = _pack(v)
        return carry

    @pl.when(first_step)
    def _prologue():
        cps[0].start()
        cps[1].start()
        kc[...] = jnp.zeros(kc.shape, F32)
        vc[...] = jnp.zeros(vc.shape, F32)
        mt[...] = jnp.zeros(mt.shape, F32)
        zs[...] = jnp.zeros(zs.shape, F32)
        g_all = jax.nn.sigmoid(beta_ref[...].astype(F32))
        lane_h = lax.broadcasted_iota(jnp.int32, (1, H), 1)
        for h in range(H):
            gh = jnp.sum(jnp.where(lane_h == h, g_all, 0.0), axis=1, keepdims=True)
            gate[h] = jnp.broadcast_to(gh, (8, 128))
        kk = lax.broadcasted_iota(jnp.int32, (128, 128), 0)
        qq = lax.broadcasted_iota(jnp.int32, (128, 128), 1)
        cmask[...] = jnp.where(qq < kk, NEG, 0.0).astype(F32)

        def load_x(j, carry):
            r0 = pl.multiple_of(j * 64, 64)
            xs[pl.ds(r0, 64), :] = x_ref[pl.ds(r0, 64), :].astype(F32)
            return carry
        lax.fori_loop(0, L // 64, load_x, 0)

        def norm_x(j, carry):
            r0 = pl.multiple_of(j * 64, 64)
            xa[pl.ds(r0, 64), :] = _layernorm(xs[pl.ds(r0, 64), :])
            return carry
        lax.fori_loop(0, RC // 64, norm_x, 0)

        def perm_cols(t, carry):
            m, j = t // 2, t % 2
            for i in range(3):
                @pl.when(t == 2 * i)
                def _():
                    cps[i].wait()
                    if i < 2:
                        cps[i + 2].start()
                    else:
                        for c in cps[4:7]:
                            c.start()
            halves = []
            for half in range(2):
                tt = raw_u32(m, pl.ds(pl.multiple_of(half * HD + j * 256, 256), 256), slice(None)).T
                for h in range(H):
                    tbuf[half, h * PITCH:h * PITCH + DH, :] = tt[h * DH:(h + 1) * DH]
                halves.append([jnp.concatenate(
                    [tbuf[half, pl.ds(4 * c + r, H, stride=PITCH), :] for r in range(4)], axis=0).T
                    for c in range(NT)])
            r0 = pl.multiple_of(j * 128, 128)
            for c in range(NT // 2):
                quad = (halves[0][c], halves[0][NT // 2 + c], halves[1][c], halves[1][NT // 2 + c])
                for i, v in enumerate(packed_blocks(*quad)):
                    wa[m, i, pl.ds(r0, 128), c * 128:(c + 1) * 128] = v
            return carry
        lax.fori_loop(0, 6, perm_cols, 0)

        cps[3].wait()
        for c in cps[7:]:
            c.start()

        def perm_rows(j, carry):
            c0 = pl.multiple_of(j * 128, 128)
            cols = []
            for half in range(2):
                w = pltpu.bitcast(raw[3, :, pl.ds(half * HD + c0, 128)].astype(F32), U32)
                for h in range(H):
                    tbuf[half, h * PITCH:h * PITCH + DH, :] = w[h * DH:(h + 1) * DH]
                cols.append(pltpu.bitcast(jnp.concatenate(
                    [tbuf[half, pl.ds(d, H, stride=PITCH), :] for d in range(DH)], axis=0), F32))
            for i, v in enumerate(_rhs_blocks(cols[0][:HD], cols[1][:HD], cols[0][HD:], cols[1][HD:])):
                woa[i, :, pl.ds(c0, 128)] = _pack(v)
            return carry
        lax.fori_loop(0, NT // 2, perm_rows, 0)
        for c in cps[4:7]:
            c.wait()
        lax.fori_loop(0, 4, comb_qk, 0)

    def _late_weights():
        for c in cps[7:]:
            c.wait()
        lax.fori_loop(4, 16, comb_qk, 0)

        def comb_ob(t, carry):
            p, j = t // 2, t % 2
            r0 = pl.multiple_of(p * 256 + j * 64, 64)
            top = raw_u32(7, pl.ds(r0, 64), slice(None))
            bot = raw_u32(7, pl.ds(r0 + 128, 64), slice(None))
            for i, v in enumerate(packed_blocks(top[:, :HD], top[:, HD:], bot[:, :HD], bot[:, HD:])):
                wob[i, pl.ds(pl.multiple_of(t * 32, 32), 32), :] = v
            return carry
        lax.fori_loop(0, 8, comb_ob, 0)

    for c in range(NT):
        kb[c, 0:HALO, :] = kc[rep, c]
        vb[c, 0:HALO, :] = vc[rep, c]
    a_in = [row_blocks(xa[...])] + [row_blocks(_layernorm(xs[ch * RC:(ch + 1) * RC, :])) for ch in range(1, NCH)]

    def a_proj(ch, m):
        dst, off = ((kb, HALO), (qb, 0), (vb, HALO))[m]

        def done(i, j, y):
            r0 = off + ch * RC + i * 128
            if m == 1:
                y = y * QSCALE
            for c in range(NT // 2):
                dst[j * NT // 2 + c, r0:r0 + 128, :] = y[:, c * 128:(c + 1) * 128]
        return _block_matmul(
            lambda a, b: _dot(a_in[ch][a].astype(BF16), _unpack(wa[m, b])), done)

    def a_attn(r0, n):
        accs = [None] * W
        for c in range(NT):
            qc = qb[c, r0:r0 + n, :]
            for w in range(W):
                o0 = HALO + r0 - DIL * w
                t = qc * kb[c, o0:o0 + n, :]
                accs[w] = t if c == 0 else accs[w] + t
        ls = []
        for w in range(W):
            acc = accs[w]
            acc = acc + pltpu.roll(acc, 64, 1)
            acc = acc + pltpu.roll(acc, 32, 1)
            if r0 < DIL * w:
                pos = seg * L + r0 + lax.broadcasted_iota(jnp.int32, (n, 128), 0)
                acc = jnp.where(pos >= DIL * w, acc, NEG)
            ls.append(acc)
        mx = functools.reduce(jnp.maximum, ls)
        es = [jnp.exp2(l - mx) for l in ls]
        inv = 1.0 / functools.reduce(jnp.add, es)
        ps = [e * inv for e in es]
        outs = []
        for c in range(NT):
            acc = None
            for w in range(W):
                o0 = HALO + r0 - DIL * w
                t = ps[w] * vb[c, o0:o0 + n, :]
                acc = t if acc is None else acc + t
            outs.append(acc)
        return outs

    def a_attn_chunk(ch):
        n = 16
        rows = [jnp.concatenate(a_attn(ch * RC + r, n), axis=1) for r in range(0, RC, n)]
        blocks = row_blocks(jnp.concatenate(rows, axis=0))
        return lambda a: blocks[a].astype(BF16)

    def out_proj(ch, lhs, w_ref, k0, k1):
        def done(i, j, y):
            r0 = ch * RC + i * 128
            xs[r0:r0 + 128, j * HD:(j + 1) * HD] += y
        return _block_matmul(
            lambda a, b: _dot(
                lhs(a),
                _unpack(w_ref[b, k0 // 2:k1 // 2, :])),
            done)

    def b_proj_qk(p, ch):
        def done(i, j, y):
            r0 = ch * RC + i * 128
            bq[j, r0:r0 + 128, :] = y[:, :128]
            bk[j, r0:r0 + 128, :] = y[:, 128:]
        return _block_matmul(
            lambda a, b: _dot(_unpack(xb[a, ch * 64:(ch + 1) * 64, :]), _unpack(wqk[p, b])), done)

    def b_proj_v(p):
        def done(i, j, y):
            for ch in range(NCH):
                c0 = ch * RC + i * 128
                bv[j, :, c0:c0 + 128] = _pack(y[:, ch * 128:(ch + 1) * 128])
        return _block_matmul(lambda a, b: _dot_nt(_unpack(wvt[p, b]), _unpack(xb[a])), done)

    lane = lax.broadcasted_iota(jnp.int32, (1, 128), 1) // DH

    def scores(q, k, j):
        nk = 128 * (j + 1)
        qj = q[j * 128:(j + 1) * 128, :]
        qm = jnp.concatenate([qj * jnp.where(lane == h, QSCALE, 0.0) for h in range(4)], axis=0)
        st = _dot_nt(k[0:nk].astype(BF16), qm.astype(BF16))
        diag = st[nk - 128:] + jnp.concatenate([cmask[...]] * 4, axis=1)
        return diag if j == 0 else jnp.concatenate([st[:nk - 128], diag], axis=0)

    def memory(g, q):
        pq = _phi(q).astype(BF16)
        zrow = lax.broadcasted_iota(jnp.int32, (16, 128), 0)
        zl = jnp.where(zrow == lane, jnp.broadcast_to(zs[rep * NT + g, 0:1, :], (16, 128)), 0.0)
        lhs = jnp.concatenate([mt[rep * NT + g], zl], axis=0).astype(BF16)
        return _dot_nt(lhs, pq)

    def update(g, k, vt):
        pk = _phi(k)
        upd = functools.reduce(jnp.add, [
            _dot(_unpack(vt[:, i * 128:(i + 1) * 128]), pk[i * 128:(i + 1) * 128].astype(BF16)) for i in range(L // 128)])
        rr = lax.broadcasted_iota(jnp.int32, (128, 128), 0) // DH
        mt[rep * NT + g] += jnp.where(rr == lane, upd, 0.0)
        zs[rep * NT + g] += jnp.sum(pk, axis=0, keepdims=True)

    def attend(g, e, j, st, nd, vt):
        nk = 128 * (j + 1)
        mx = jnp.max(st, axis=0, keepdims=True)
        p = jnp.exp2(st - mx)
        l = jnp.sum(p, axis=0, keepdims=True)
        rows = []
        for h in range(4):
            pv = _dot(_unpack(vt[h * 16:(h + 1) * 16, 0:nk]), p[:, h * 128:(h + 1) * 128].astype(BF16))
            gh = gate[g * 4 + h][0:1, :]
            num = nd[h * DH:(h + 1) * DH, j * 128:(j + 1) * 128]
            den = nd[128 + h:129 + h, j * 128:(j + 1) * 128] + 1e-6
            rows.append(num * (gh / den) + pv * ((1.0 - gh) / l[:, h * 128:(h + 1) * 128]))
        of[e, j * 128:(j + 1) * 128, :] = jnp.concatenate(rows, axis=0).T

    def b_out_blocks(p, ch):
        r0 = ch * RC
        blocks = _lhs_blocks(of[0, r0:r0 + 128, :], of[1, r0:r0 + 128, :],
                             of[0, r0 + 128:r0 + 256, :], of[1, r0 + 128:r0 + 256, :])
        for i, b in enumerate(blocks):
            oc[p, i, ch * 64:(ch + 1) * 64, :] = _pack(b)

    def finish_rows(ch):
        xnew = xs[ch * RC:(ch + 1) * RC, :]
        out_ref[ch * RC:(ch + 1) * RC, :] = xnew.astype(BF16)
        nxt = jnp.where(rep == 0, xnew, x_ref[ch * RC:(ch + 1) * RC, :].astype(F32))
        xs[ch * RC:(ch + 1) * RC, :] = nxt
        return nxt

    with jax.named_scope("sc_A"):
        a_out = []
        for ch in range(NCH):
            for m in range(3):
                _run(a_proj(ch, m))
            a_out.append(a_attn_chunk(ch))
        _run(out_proj(0, a_out[0], woa, 0, HD))
        norm_blocks(0)
        first = b_proj_qk(0, 0)
        _run(first, 4)
        _run(out_proj(1, a_out[1], woa, 0, HD))
        norm_blocks(1)
        _run(first)
        _run(b_proj_qk(0, 1))
        _run(b_proj_v(0))

        for c in range(NT):
            kc[rep, c] = kb[c, L:L + HALO, :]
            vc[rep, c] = vb[c, L:L + HALO, :]

    npair = NT // 2
    kf = (npair - 1) * 128

    def b_out(ch, k0, k1):
        def lhs(a):
            return _unpack(jnp.concatenate(
                [oc[c, a, ch * 64:(ch + 1) * 64, :] for c in range(k0 // 128, k1 // 128)], axis=1))
        return out_proj(ch, lhs, wob, k0, k1)

    def b_pair(p, last):
        qs = [bq[e] for e in range(2)]
        ks = [bk[e] for e in range(2)]
        vts = [bv[e] for e in range(2)]
        if last:
            fill = _chain(b_out(0, 0, kf), b_out(1, 0, kf))
        else:
            fill = _chain(b_proj_qk(p + 1, 0), b_proj_qk(p + 1, 1), b_proj_v(p + 1))
        pat = (1, 1, 1, 1, 1, 1, 1, 0) if last else (1, 1, 2, 1, 2, 1, 1, 1)
        for e in range(2):
            g = 2 * p + e
            q, k, vt = qs[e], ks[e], vts[e]
            order = (0, 1, 2, 3) if last else (3, 2, 1, 0)
            _run(fill, pat[0])
            sa = scores(q, k, order[0])
            _run(fill, pat[1])
            sb = scores(q, k, order[1])
            nd = memory(g, q)
            _run(fill, pat[2])
            attend(g, e, order[0], sa, nd, vt)
            _run(fill, pat[3])
            sa = scores(q, k, order[2])
            _run(fill, pat[4])
            attend(g, e, order[1], sb, nd, vt)
            if e:
                b_out_blocks(p, order[0] // 2)
            sb = scores(q, k, order[3])
            _run(fill, pat[5])
            attend(g, e, order[2], sa, nd, vt)
            update(g, k, vt)
            _run(fill, pat[6])
            if last and e:
                _run(fill)
                _run(b_out(0, kf, HD))
                xa[...] = _layernorm(finish_rows(0))
            attend(g, e, order[3], sb, nd, vt)
            if e:
                b_out_blocks(p, order[3] // 2)
            _run(fill, pat[7])
        _run(fill)

    pl.when(first_step)(_late_weights)
    with jax.named_scope("sc_Bloop"):
        lax.fori_loop(0, npair - 1, lambda p, c: (b_pair(p, False), c)[1], 0)
    with jax.named_scope("sc_Blast"):
        b_pair(npair - 1, True)
        _run(b_out(1, kf, HD))
        finish_rows(1)


@jax.jit
def pallas_interleave_layers__sliding_local_dilated__memory_aug_infini_attn__prompt_kernel(
        A_x, A_wqkv, A_wo, B_x, B_wq, B_wk, B_wv, B_wo, B_beta):
    del B_x
    hbm = pl.BlockSpec(memory_space=pl.ANY)
    out = pl.pallas_call(
        _kernel,
        grid=(NSEG, 2),
        in_specs=[pl.BlockSpec((L, D), lambda s, r: (jnp.minimum(s + r, NSEG - 1), 0)),
                  pl.BlockSpec((1, H), lambda s, r: (0, 0)),
                  hbm, hbm, hbm, hbm, hbm, hbm],
        out_specs=pl.BlockSpec((L, D), lambda s, r: (s, 0)),
        out_shape=jax.ShapeDtypeStruct((S, D), BF16),
        scratch_shapes=[
            pltpu.VMEM((8, D, D), BF16),
            pltpu.VMEM((3, NP, HD // 2, HD), U32),
            pltpu.VMEM((NP, HD // 2, HD), U32),
            pltpu.VMEM((NT // 2, NP, HD // 2, 256), U32),
            pltpu.VMEM((NT // 2, NP, 64, HD), U32),
            pltpu.VMEM((NP, HD // 2, HD), U32),
            pltpu.VMEM((2, H * PITCH, 128), U32),
            pltpu.VMEM((L, D), F32),
            pltpu.VMEM((RC, D), F32),
            pltpu.VMEM((NP, L // 4, HD), U32),
            pltpu.VMEM((NT, L, 128), F32),
            pltpu.VMEM((NT, HALO + L, 128), F32),
            pltpu.VMEM((NT, HALO + L, 128), F32),
            pltpu.VMEM((2, NT, HALO, 128), F32),
            pltpu.VMEM((2, NT, HALO, 128), F32),
            pltpu.VMEM((2, L, 128), F32),
            pltpu.VMEM((NT // 2, NP, L // 4, 128), U32),
            pltpu.VMEM((2, L, 128), F32),
            pltpu.VMEM((2, L, 128), F32),
            pltpu.VMEM((2, 64, L), U32),
            pltpu.VMEM((2 * NT, 128, 128), F32),
            pltpu.VMEM((2 * NT, 8, 128), F32),
            pltpu.VMEM((H, 8, 128), F32),
            pltpu.VMEM((128, 128), F32),
            pltpu.SemaphoreType.DMA((11,)),
        ],
        compiler_params=pltpu.CompilerParams(
            dimension_semantics=("arbitrary", "arbitrary"),
            vmem_limit_bytes=110 * 2**20,
            flags={k: True for k in os.environ.get('FL', '').split(',') if k} or None),
        name="interleave",
    )(A_x.reshape(S, D), B_beta.reshape(1, H), A_wqkv, A_wo, B_wq, B_wk, B_wv, B_wo)
    return out.reshape(1, S, D)
```

```python
import functools
import math
import os

import jax
import jax.numpy as jnp
import numpy as np
from jax import lax
from jax.experimental import pallas as pl
from jax.experimental.pallas import tpu as pltpu

S, D, H, DH = 2048, 1024, 32, 32
NSEG = 4
L = S // NSEG
W, DIL = 8, 2
HALO = 16
NT = D // 128
HD = D // 2
SPLIT = int(os.environ.get('SPLIT', 2))
GATE = int(os.environ.get('GATE', 3))
SLACK = int(os.environ.get('SLACK', 4))
FIRST = int(os.environ.get('FIRST', 7))
PITCH = int(os.environ.get('PITCH', 17))
WROWS = 16 * PITCH
RC = 256
NCH = L // RC
LOG2E = math.log2(math.e)
QSCALE = DH ** -0.5 * LOG2E
NEG = -1e9 * LOG2E
F32, BF16, U32 = jnp.float32, jnp.bfloat16, jnp.uint32
STRASSEN = int(os.environ.get("STR", 1))
NP = 7 if STRASSEN else 4


def _dot(a, b):
    return jnp.dot(a, b, preferred_element_type=F32)


def _dot_nt(a, b):
    return lax.dot_general(a, b, (((1,), (1,)), ((), ())), preferred_element_type=F32)


def _pack(x):
    return pltpu.bitcast(x.astype(BF16), U32)


def _unpack(x):
    return pltpu.bitcast(x, BF16)


def _lhs_blocks(a11, a12, a21, a22):
    if STRASSEN:
        return [a11 + a22, a21 + a22, a11, a22, a11 + a12, a21 - a11, a12 - a22]
    return [a11, a12, a21, a22]


def _rhs_blocks(b11, b12, b21, b22):
    if STRASSEN:
        return [b11 + b22, b11, b12 - b22, b21 - b11, b22, b11 + b12, b21 + b22]
    return [b11, b12, b21, b22]


def _whole(fn):
    def prod(a, b):
        y = fn(a, b)
        yield
        return y
    return prod


def _tiled(lhs, rhs, nk, nn, dot, tick):
    def prod(a, b):
        acc = [None] * nn
        cnt = 0
        for n in range(nn):
            for k in range(nk):
                t = dot(lhs(a, k), rhs(b, k, n))
                acc[n] = t if k == 0 else acc[n] + t
                cnt += 1
                if cnt % 4 == 0:
                    tick(t)
                    yield
        return jnp.concatenate(acc, axis=1)
    return prod


def _block_matmul(prod, done):
    if STRASSEN:
        p3 = yield from prod(2, 2)
        p5 = yield from prod(4, 4)
        done(0, 1, p3 + p5)
        p2 = yield from prod(1, 1)
        p4 = yield from prod(3, 3)
        done(1, 0, p2 + p4)
        u, v = p4 - p5, p3 - p2
        p1 = yield from prod(0, 0)
        u, v = u + p1, v + p1
        p7 = yield from prod(6, 6)
        done(0, 0, u + p7)
        p6 = yield from prod(5, 5)
        done(1, 1, v + p6)
    else:
        for i in range(2):
            for j in range(2):
                t = yield from prod(2 * i, j)
                u = yield from prod(2 * i + 1, 2 + j)
                done(i, j, t + u)


def _run(gen, n=None):
    k = 0
    while n is None or k < n:
        if next(gen, "end") == "end":
            break
        k += 1


def _chain(*gens):
    for g in gens:
        yield from g


def _layernorm(x):
    m = jnp.mean(x, axis=-1, keepdims=True)
    xc = x - m
    v = jnp.mean(xc * xc, axis=-1, keepdims=True)
    return xc * lax.rsqrt(v + 1e-5)


def _phi(t):
    return jnp.where(t > 0, t + 1.0, jnp.exp(t))


def _kernel(x_ref, beta_ref, wqkv_hbm, woa_hbm, wq_hbm, wk_hbm, wv_hbm, wob_hbm, out_ref,
            raw, wa, woa, wqk, wvt, wob,
            xs, xa, xb, qb, kb, vb, kc, vc, of, oc, bq, bk, bv, mt, zs, gate, cmask, sems):
    seg = pl.program_id(0)
    rep = pl.program_id(1)

    def row_blocks(xn):
        return _lhs_blocks(xn[:128, :HD], xn[:128, HD:], xn[128:, :HD], xn[128:, HD:])

    def norm_blocks(ch):
        return row_blocks(_layernorm(xs[ch * RC:(ch + 1) * RC, :]))

    first_step = (seg == 0) & (rep == 0)
    c1 = 256

    def early_copy(i):
        m, j = divmod(i, 2)
        if m < 3:
            c0 = (1, 0, 2)[m] * D + j * HD
            return pltpu.make_async_copy(wqkv_hbm.at[:, pl.ds(c0, HD)], raw.at[m, :, pl.ds(j * HD, HD)], sems.at[i])
        return pltpu.make_async_copy(woa_hbm.at[pl.ds(j * HD, HD)], raw.at[3, pl.ds(j * HD, HD)], sems.at[i])

    pair0 = [pltpu.make_async_copy(s.at[:, pl.ds(0, c1)], raw.at[4 + i, :, pl.ds(0, c1)], sems.at[8 + i])
             for i, s in enumerate((wq_hbm, wk_hbm, wv_hbm))]
    late = [pltpu.make_async_copy(s.at[:, pl.ds(c1, D - c1)], raw.at[4 + i, :, pl.ds(c1, D - c1)], sems.at[11 + i])
            for i, s in enumerate((wq_hbm, wk_hbm, wv_hbm))]
    late.append(pltpu.make_async_copy(wob_hbm, raw.at[7], sems.at[14]))

    def selector(head_major):
        row = lax.broadcasted_iota(jnp.int32, (128, 128), 0)
        col = lax.broadcasted_iota(jnp.int32, (128, 128), 1)
        if not head_major:
            row = (((row >> 5) & 1) * 2 + (row & 1)) * DH + (row >> 6) * 16 + ((row >> 1) & 15)
        return jnp.where(row == col, 1.0, 0.0).astype(BF16)

    def packed_blocks(b11, b12, b21, b22):
        quad = (b11, b12, b21, b22)
        vals = [_unpack(b).astype(F32) for b in quad]
        out = []
        for blk in _rhs_blocks(*vals):
            same = [i for i, v in enumerate(vals) if v is blk]
            out.append(quad[same[0]] if same else _pack(blk))
        return out

    def raw_u32(m, rows, cols):
        return pltpu.bitcast(raw[m, rows, cols], U32)

    def prep_pair(t, carry):
        p = t // 2
        c0 = pl.multiple_of(p * 256, 256)
        for jj in range(2):
            j = (t % 2) * 2 + jj
            r0 = pl.multiple_of(j * 128, 128)
            y = _dot_nt(selector(True), jnp.concatenate(
                [raw[6, pl.ds(kh * HD + r0, 128), pl.ds(c0 + e * 128, 128)] for kh in range(2) for e in range(2)],
                axis=0))
            for i, v in enumerate(_rhs_blocks(*[y[:, c:c + 128] for c in range(0, HD, 128)])):
                wvt[p, i, :, pl.ds(r0, 128)] = _pack(v)
            for m in range(2):
                top = raw_u32(4 + m, pl.ds(r0, 128), pl.ds(c0, 256))
                bot = raw_u32(4 + m, pl.ds(HD + r0, 128), pl.ds(c0, 256))
                for i, v in enumerate(packed_blocks(top[:, :128], top[:, 128:], bot[:, :128], bot[:, 128:])):
                    wqk[p, i, pl.ds(pl.multiple_of(j * 64, 64), 64), m * 128:(m + 1) * 128] = v
        return carry

    def arrive(piece, lo, hi):
        for i in range(lo, hi):
            @pl.when(piece == i)
            def _():
                early_copy(i).wait()
                if i == 0:
                    early_copy(2).start()
                if i == 1:
                    for n in range(3, 6):
                        early_copy(n).start()

    def scatter(dst, t, blocks):
        for i, v in enumerate(blocks):
            v = _pack(v)
            for c in range(NT // 2):
                for hp in range(2):
                    dst(i, c)[pl.ds(t * 2 + hp, 16, stride=PITCH), :] = v[hp * 16:(hp + 1) * 16, c * 128:(c + 1) * 128]

    def perm_cols(u, carry):
        m = u // 4
        arrive(jnp.where(u % 2 == 0, u // 2, -1), 0, 6)
        for tt in range(2):
            t = (u % 4) * 2 + tt
            c0 = pl.multiple_of(t * 128, 128)
            top = _dot_nt(selector(False), raw[m, 0:HD, pl.ds(c0, 128)])
            bot = _dot_nt(selector(False), raw[m, HD:D, pl.ds(c0, 128)])
            scatter(lambda i, c: wa.at[m, i, c], t, _rhs_blocks(top[:64], top[64:], bot[:64], bot[64:]))
        return carry
    @pl.when(first_step)
    def _prologue():
        for i in range(2):
            early_copy(i).start()
        kc[...] = jnp.zeros(kc.shape, F32)
        vc[...] = jnp.zeros(vc.shape, F32)
        mt[...] = jnp.zeros(mt.shape, F32)
        zs[...] = jnp.zeros(zs.shape, F32)
        g_all = jax.nn.sigmoid(beta_ref[...].astype(F32))
        lane_h = lax.broadcasted_iota(jnp.int32, (1, H), 1)
        for h in range(H):
            gh = jnp.sum(jnp.where(lane_h == h, g_all, 0.0), axis=1, keepdims=True)
            gate[h] = jnp.broadcast_to(gh, (8, 128))
        kk = lax.broadcasted_iota(jnp.int32, (128, 256), 0)
        qq = lax.broadcasted_iota(jnp.int32, (128, 256), 1)
        qq = jnp.where(qq < 128, qq ^ 64, qq - 128)
        cmask[...] = jnp.where(qq < kk, NEG, 0.0).astype(F32)

        def load_x(j, carry):
            r0 = pl.multiple_of(j * 64, 64)
            xs[pl.ds(r0, 64), :] = x_ref[pl.ds(r0, 64), :].astype(F32)
            return carry
        lax.fori_loop(0, L // 64, load_x, 0)

        def norm_x(j, carry):
            r0 = pl.multiple_of(j * 64, 64)
            xa[pl.ds(r0, 64), :] = _layernorm(xs[pl.ds(r0, 64), :])
            return carry
        lax.fori_loop(0, RC // 64, norm_x, 0)

        lax.fori_loop(0, 4, perm_cols, 0)

    def _mid_weights():
        for c in [early_copy(6), early_copy(7)] + pair0:
            c.start()
        lax.fori_loop(4, 12, perm_cols, 0)

        def perm_rows(u, carry):
            arrive(jnp.where(u % 2 == 0, 6 + u // 2, -1), 6, 8)
            for tt in range(2):
                t = u * 2 + tt
                y = _dot(selector(False), raw[3, pl.ds(pl.multiple_of(t * 128, 128), 128), :])
                scatter(lambda i, c: woa.at[i, c], t, _rhs_blocks(y[:64, :HD], y[:64, HD:], y[64:, :HD], y[64:, HD:]))
            return carry
        lax.fori_loop(0, 4, perm_rows, 0)
        for c in late:
            c.start()
        for c in pair0:
            c.wait()
        lax.fori_loop(0, 2, prep_pair, 0)

    def _late_weights():
        for c in late:
            c.wait()
        lax.fori_loop(2, NT, prep_pair, 0)

        def comb_ob(t, carry):
            p, j = t // 2, t % 2
            r0 = pl.multiple_of(p * 256 + j * 64, 64)
            top = raw_u32(7, pl.ds(r0, 64), slice(None))
            bot = raw_u32(7, pl.ds(r0 + 128, 64), slice(None))
            for i, v in enumerate(packed_blocks(top[:, :HD], top[:, HD:], bot[:, :HD], bot[:, HD:])):
                wob[i, pl.ds(pl.multiple_of(t * 32, 32), 32), :] = v
            return carry
        lax.fori_loop(0, 8, comb_ob, 0)

    for c in range(NT):
        kb[c, 0:HALO, :] = kc[rep, c]
        vb[c, 0:HALO, :] = vc[rep, c]
    xa[RC:L, :] = _layernorm(xs[RC:L, :])
    a_in = [row_blocks(xa[ch * RC:(ch + 1) * RC, :]) for ch in range(NCH)]

    ticks = []

    def tick(y):
        ticks.extend(y[0:8, c:c + 128] for c in range(0, y.shape[1], 128))
        return y

    def after(t, x):
        return x if t < 0 else jnp.where(cmask[0:8, 0:128] > 1.0, ticks[min(t, len(ticks) - 1)], x)

    def before(deps, a):
        if not deps:
            return a
        head = a[0:8, 0:128]
        for d in deps:
            head = jnp.where(cmask[0:8, 0:128] > 1.0, d, head)
        top = jnp.concatenate([head, a[0:8, 128:]], axis=1)
        return jnp.concatenate([top, a[8:]], axis=0)

    def permuted(ref):
        return _unpack(jnp.concatenate([jnp.concatenate(
            [ref[c, d * PITCH:d * PITCH + 16, :] for d in range(16)], axis=0) for c in range(NT // 2)], axis=1))

    def a_proj(ch, m):
        dst, off = ((kb, HALO), (qb, 0), (vb, HALO))[m]

        def done(i, j, y):
            r0 = off + ch * RC + i * 128
            if m == 1:
                y = y * QSCALE
            for c in range(NT // 2):
                dst[j * NT // 2 + c, r0:r0 + 128, :] = y[:, c * 128:(c + 1) * 128]
        return _block_matmul(
            _whole(lambda a, b: tick(_dot_nt(a_in[ch][a].astype(BF16), permuted(wa.at[m, b])))), done)

    def a_probs(r0, t):
        accs = [None] * W
        for c in range(NT):
            qc = after(t, qb[c, r0:r0 + 8, :])
            for w in range(W):
                o0 = HALO + r0 - DIL * w
                u = qc * kb[c, o0:o0 + 8, :]
                accs[w] = u if c == 0 else accs[w] + u
        ls = []
        for w in range(W):
            acc = accs[w]
            acc = acc + pltpu.roll(acc, 64, 1)
            acc = acc + pltpu.roll(acc, 32, 1)
            if r0 < DIL * w:
                pos = seg * L + r0 + lax.broadcasted_iota(jnp.int32, (8, 128), 0)
                acc = jnp.where(pos >= DIL * w, acc, NEG)
            ls.append(acc)
        mx = functools.reduce(jnp.maximum, ls)
        es = [jnp.exp2(l - mx) for l in ls]
        inv = 1.0 / functools.reduce(jnp.add, es)
        return es, inv

    def a_mix(r0, es, inv):
        ps = [e * inv for e in es]
        outs = []
        for c in range(NT):
            acc = None
            for w in range(W):
                o0 = HALO + r0 - DIL * w
                u = ps[w] * vb[c, o0:o0 + 8, :]
                acc = u if acc is None else acc + u
            outs.append(acc)
        return jnp.concatenate(outs, axis=1)

    def a_attn_chunk(ch, t0, dt0, t1, dt1):
        n = RC // 8
        rows = [None] * n
        for i in range(n):
            r = i // 2 + (i % 2) * (n // 2)
            es, inv = a_probs(ch * RC + r * 8, int(t0 + i * dt0))
            rows[r] = a_mix(ch * RC + r * 8, es, after(int(t1 + i * dt1), inv))
        return rows

    def add_rows(ch):
        def done(i, j, y):
            r0 = ch * RC + i * 128
            xs[r0:r0 + 128, j * HD:(j + 1) * HD] += y
        return done

    def a_out(ch, lhs):
        return _block_matmul(_whole(lambda a, b: tick(_dot(lhs(a), permuted(woa.at[b])))), add_rows(ch))

    def tile(i):
        return slice(i * 128, (i + 1) * 128)

    def b_proj_qk(p, ch, lhs=None):
        def done(i, j, y):
            r0 = ch * RC + i * 128
            bq[j, r0:r0 + 128, :] = y[:, :128]
            bk[j, r0:r0 + 128, :] = y[:, 128:]
        if lhs is not None:
            return _block_matmul(_whole(lambda a, b: tick(_dot(lhs[a].astype(BF16), _unpack(wqk[p, b])))), done)
        return _block_matmul(_tiled(
            lambda a, k: _unpack(xb[a, ch * 64:(ch + 1) * 64, tile(k)]),
            lambda b, k, n: _unpack(wqk[p, b, k * 64:(k + 1) * 64, tile(n)]), 4, 2, _dot, tick), done)

    def b_proj_v(p):
        def done(i, j, y):
            for ch in range(NCH):
                c0 = ch * RC + i * 128
                bv[j, :, c0:c0 + 128] = _pack(y[:, tile(ch)])
        return _block_matmul(_tiled(
            lambda a, k: a, lambda b, k, n: (b, k, n), 4, NCH,
            lambda a, t: _dot_nt(_unpack(wvt[p, t[0], :, tile(t[1])]),
                                 _unpack(xb[a, t[2] * 64:(t[2] + 1) * 64, tile(t[1])])), tick), done)

    def finish_rows(ch):
        def done(i, j, y):
            idx = (slice(ch * RC + i * 128, ch * RC + (i + 1) * 128), slice(j * HD, (j + 1) * HD))
            xnew = xs[idx] + y
            out_ref[idx] = xnew.astype(BF16)
            xs[idx] = jnp.where(rep == 0, xnew, x_ref[idx].astype(F32))
        return done

    def b_out(ch, p0, p1):
        def prod(a, b):
            acc = None
            for p in range(p0, p1):
                t = _dot(_unpack(oc[p, a, ch * 64:(ch + 1) * 64, :]), _unpack(wob[b, p * 64:(p + 1) * 64, :]))
                acc = t if acc is None else acc + t
                tick(t[:, 0:128])
                yield
            return acc
        return _block_matmul(prod, finish_rows(ch) if p1 == NT // 2 else add_rows(ch))

    lane = lax.broadcasted_iota(jnp.int32, (1, 128), 1) // DH

    def head_queries(q, j):
        qj = q[tile(j), :]
        qh = [qj * jnp.where(lane == h, QSCALE, 0.0) for h in range(4)]
        return [(t[:64], t[64:]) for t in qh]

    def corner(q, k, j):
        qm = jnp.concatenate([hi for _, hi in head_queries(q, j)], axis=0)
        return _dot_nt(k[j * 128 + 64:(j + 1) * 128].astype(BF16), qm.astype(BF16))

    def scores(q, k, j, cor):
        nk = 128 * j + 64
        qm = jnp.concatenate([part for h, (lo, hi) in enumerate(head_queries(q, j))
                              for part in ((lo, hi) if h % 2 else (hi, lo))], axis=0)
        st = _dot_nt(k[0:nk].astype(BF16), qm.astype(BF16))
        for i in range(j + 1):
            tick(st[i * 128:i * 128 + 8, 0:128])
        diag = jnp.concatenate([st[nk - 64:], jnp.concatenate([cor[:, tile(h // 2)] for h in range(4)], axis=1)],
                               axis=0)
        diag = diag + jnp.concatenate([cmask[...]] * 2, axis=1)
        return diag if j == 0 else jnp.concatenate([st[:nk - 64], diag], axis=0)

    def memory(g, q):
        pq = _phi(q).astype(BF16)
        zrow = lax.broadcasted_iota(jnp.int32, (16, 128), 0)
        zl = jnp.where(zrow == lane, jnp.broadcast_to(zs[rep * NT + g, 0:1, :], (16, 128)), 0.0)
        lhs = jnp.concatenate([mt[rep * NT + g], zl], axis=0).astype(BF16)
        return _dot_nt(lhs, pq)

    def update(g, k, vt):
        pk = _phi(k)
        upd = functools.reduce(jnp.add, [
            _dot(_unpack(vt[:, i * 128:(i + 1) * 128]), pk[i * 128:(i + 1) * 128].astype(BF16)) for i in range(L // 128)])
        rr = lax.broadcasted_iota(jnp.int32, (128, 128), 0) // DH
        mt[rep * NT + g] += jnp.where(rr == lane, upd, 0.0)
        zs[rep * NT + g] += jnp.sum(pk, axis=0, keepdims=True)

    def attend(g, e, j, st, nd, vt):
        mx = jnp.broadcast_to(jnp.max(st, axis=0, keepdims=True), (8, 512))
        pv, l = [None] * 4, None
        for i in range(j + 1):
            mi = jnp.concatenate([after(len(ticks) - GATE, mx[:, tile(h)]) for h in range(4)], axis=1)
            p3 = jnp.exp2(st[tile(i)].reshape(16, 8, 512) - mi)
            p = p3.reshape(128, 512)
            li = jnp.sum(p3, axis=0)
            l = li if i == 0 else l + li
            for h in range(4):
                t = _dot(_unpack(vt[h * 16:(h + 1) * 16, tile(i)]), p[:, tile(h)].astype(BF16))
                pv[h] = t if i == 0 else pv[h] + t
            if i < j:
                yield
        l = jnp.sum(l, axis=0, keepdims=True)
        rows = []
        for h in range(4):
            gh = gate[g * 4 + h][0:1, :]
            num = nd[h * DH:(h + 1) * DH, tile(j)]
            den = nd[128 + h:129 + h, tile(j)] + 1e-6
            loc = pv[h] * ((1.0 - gh) / l[:, tile(h)])
            rows.append(num * (gh / den) + (loc if h % 2 else pltpu.roll(loc, 64, 1)))
        of[e, tile(j), :] = jnp.concatenate(rows, axis=0).T
        yield

    def b_out_blocks(p, ch):
        r0 = ch * RC
        blocks = _lhs_blocks(of[0, r0:r0 + 128, :], of[1, r0:r0 + 128, :],
                             of[0, r0 + 128:r0 + 256, :], of[1, r0 + 128:r0 + 256, :])
        for i, b in enumerate(blocks):
            oc[p, i, ch * 64:(ch + 1) * 64, :] = _pack(b)

    for ch in range(NCH):
        _run(a_proj(ch, 0))
    pl.when(first_step)(_mid_weights)
    del ticks[:]
    a_in = [row_blocks(xa[ch * RC:(ch + 1) * RC, :]) for ch in range(NCH)]
    with jax.named_scope("sc_A"):
        tm = (7 if STRASSEN else 8) * 4
        P = [float(v) for v in os.environ.get("PACE", "1,0.85,2.86,0.75,2,0.85,3.86,0.1").split(",")]
        for ch, m in [divmod(int(c), 3) for c in os.environ.get("ORD", "1425")]:
            _run(a_proj(ch, m))
        o0 = row_blocks(jnp.concatenate(a_attn_chunk(0, P[0] * tm, P[1], P[2] * tm, P[3]), axis=0))
        rows1 = a_attn_chunk(1, P[4] * tm, P[5], P[6] * tm, P[7])
        o1 = row_blocks(jnp.concatenate(rows1, axis=0))
        due = iter([int(v) for v in os.environ.get("DUE", "0,0,3,3,3,3,4").split(",")])
        done_rows = [0]

        def lhs0(a):
            n = next(due)
            deps = [o1[i][r * 8:r * 8 + 8, c:c + 128] for r in range(done_rows[0], done_rows[0] + n)
                    for i in (5, 6) for c in range(0, HD, 128)]
            done_rows[0] += n
            return before(deps, o0[a]).astype(BF16)
        _run(a_out(0, lhs0))
        x0 = norm_blocks(0)
        first = b_proj_qk(0, 0, x0)
        _run(first, FIRST)
        t0 = len(ticks)
        _run(a_out(1, lambda a: o1[a].astype(BF16)))
        _run(first)
        x1 = norm_blocks(1)
        t1 = len(ticks)
        _run(b_proj_qk(0, 1, x1))
        for ch, (blocks, t, dt) in enumerate(((x0, t0, 3), (x1, t1, 1))):
            for i, blk in enumerate(blocks):
                for r in range(0, 128, 32):
                    g = jnp.concatenate([ticks[t + i * dt]] * 4, axis=0)
                    g = jnp.concatenate([g] * 4, axis=1)
                    nv = jnp.concatenate([cmask[0:32, 0:128]] * 4, axis=1) > 1.0
                    xb[i, ch * 64 + r // 2:ch * 64 + r // 2 + 16, :] = _pack(jnp.where(nv, g, blk[r:r + 32]))
        _run(b_proj_v(0))
        for c in range(NT):
            kc[rep, c] = kb[c, L:L + HALO, :]
            vc[rep, c] = vb[c, L:L + HALO, :]

    npair = NT // 2

    def b_pair(p, last):
        del ticks[:]
        qs = [bq[e] for e in range(2)]
        ks = [bk[e] for e in range(2)]
        vts = [bv[e] for e in range(2)]
        if last:
            fill = _chain(b_out(0, 0, p), b_out(1, 0, SPLIT)) if SPLIT else b_out(0, 0, p)
            plan = os.environ.get("PLANL", "f s0 s1 n f p s2 p f p s3 f p f p f p f f p f p f p f p f u f "
                                  "/ s0 s1 n f p f s2 p f p o s3 f p f p f p f x p f x p f x p f x p o f x u f x F X")
            tail = b_out(0, p, p + 1)
        else:
            fill = _chain(b_proj_qk(p + 1, 0), b_proj_qk(p + 1, 1), b_proj_v(p + 1))
            plan = os.environ.get("PLAN", "f f s3 f s2 n f p f p f p f p f f s1 p f p f p f f s0 f p f p f u f p f "
                                  "/ s3 f s2 n f p f p f p f p f f s1 p f p f p o f f s0 f p f p f u f p o F")
        for e, steps in enumerate(plan.split("/")):
            g = 2 * p + e
            q, k, vt = qs[e], ks[e], vts[e]
            todo, cur, nd, seen, cors = [], None, None, [], {}
            for op in steps.split():
                if op == "f":
                    _run(fill, 1)
                elif op == "F":
                    _run(fill)
                elif op == "x":
                    _run(tail, 1)
                elif op == "X":
                    _run(tail)
                    xa[0:RC, :] = _layernorm(xs[0:RC, :])
                elif op[0] == "s":
                    j = int(op[1])
                    if j not in cors:
                        cors.update({i: corner(q, k, i) for i in (j, j ^ 1)})
                    todo.append((j, scores(q, k, j, cors[j])))
                elif op == "n":
                    nd = memory(g, q)
                elif op == "u":
                    update(g, k, vt)
                elif op == "o":
                    if e:
                        b_out_blocks(p, seen[-1] // 2)
                else:
                    if cur is None or next(cur, "end") == "end":
                        j, st = todo.pop(0)
                        seen.append(j)
                        cur = attend(g, e, j, st, nd, vt)
                        next(cur)
            assert not todo and next(cur, "end") == "end"

    pl.when(first_step)(_late_weights)
    with jax.named_scope("sc_Bloop"):
        lax.fori_loop(0, npair - 1, lambda p, c: (b_pair(p, False), c)[1], 0)
    with jax.named_scope("sc_Blast"):
        b_pair(npair - 1, True)
        _run(b_out(1, SPLIT, npair))


@jax.jit
def pallas_interleave_layers__sliding_local_dilated__memory_aug_infini_attn__prompt_kernel(
        A_x, A_wqkv, A_wo, B_x, B_wq, B_wk, B_wv, B_wo, B_beta):
    del B_x
    hbm = pl.BlockSpec(memory_space=pl.ANY)
    out = pl.pallas_call(
        _kernel,
        grid=(NSEG, 2),
        in_specs=[pl.BlockSpec((L, D), lambda s, r: (jnp.minimum(s + r, NSEG - 1), 0)),
                  pl.BlockSpec((1, H), lambda s, r: (0, 0)),
                  hbm, hbm, hbm, hbm, hbm, hbm],
        out_specs=pl.BlockSpec((L, D), lambda s, r: (s, 0)),
        out_shape=jax.ShapeDtypeStruct((S, D), BF16),
        scratch_shapes=[
            pltpu.VMEM((8, D, D), BF16),
            pltpu.VMEM((3, NP, NT // 2, WROWS, 128), U32),
            pltpu.VMEM((NP, NT // 2, WROWS, 128), U32),
            pltpu.VMEM((NT // 2, NP, HD // 2, 256), U32),
            pltpu.VMEM((NT // 2, NP, 64, HD), U32),
            pltpu.VMEM((NP, HD // 2, HD), U32),
            pltpu.VMEM((L, D), F32),
            pltpu.VMEM((L, D), F32),
            pltpu.VMEM((NP, L // 4, HD), U32),
            pltpu.VMEM((NT, L, 128), F32),
            pltpu.VMEM((NT, HALO + L, 128), F32),
            pltpu.VMEM((NT, HALO + L, 128), F32),
            pltpu.VMEM((2, NT, HALO, 128), F32),
            pltpu.VMEM((2, NT, HALO, 128), F32),
            pltpu.VMEM((2, L, 128), F32),
            pltpu.VMEM((NT // 2, NP, L // 4, 128), U32),
            pltpu.VMEM((2, L, 128), F32),
            pltpu.VMEM((2, L, 128), F32),
            pltpu.VMEM((2, 64, L), U32),
            pltpu.VMEM((2 * NT, 128, 128), F32),
            pltpu.VMEM((2 * NT, 8, 128), F32),
            pltpu.VMEM((H, 8, 128), F32),
            pltpu.VMEM((128, 256), F32),
            pltpu.SemaphoreType.DMA((15,)),
        ],
        compiler_params=pltpu.CompilerParams(
            dimension_semantics=("arbitrary", "arbitrary"),
            vmem_limit_bytes=110 * 2**20,
            flags={k: True for k in os.environ.get('FL', '').split(',') if k} or None),
        name="interleave",
    )(A_x.reshape(S, D), B_beta.reshape(1, H), A_wqkv, A_wo, B_wq, B_wk, B_wv, B_wo)
    return out.reshape(1, S, D)
```

```python
import functools
import math
import os

import jax
import jax.numpy as jnp
import numpy as np
from jax import lax
from jax.experimental import pallas as pl
from jax.experimental.pallas import tpu as pltpu

S, D, H, DH = 2048, 1024, 32, 32
NSEG = 4
L = S // NSEG
W, DIL = 8, 2
HALO = 16
NT = D // 128
HD = D // 2
SPLIT = int(os.environ.get('SPLIT', 2))
GATE = int(os.environ.get('GATE', 3))
SLACK = int(os.environ.get('SLACK', 4))
FIRST = int(os.environ.get('FIRST', 7))
PITCH = int(os.environ.get('PITCH', 17))
WROWS = 16 * PITCH
RC = 256
NCH = L // RC
LOG2E = math.log2(math.e)
QSCALE = DH ** -0.5 * LOG2E
NEG = -1e9 * LOG2E
F32, BF16, U32 = jnp.float32, jnp.bfloat16, jnp.uint32
STRASSEN = int(os.environ.get("STR", 1))
NP = 7 if STRASSEN else 4


def _dot(a, b):
    return jnp.dot(a, b, preferred_element_type=F32)


def _dot_nt(a, b):
    return lax.dot_general(a, b, (((1,), (1,)), ((), ())), preferred_element_type=F32)


def _pack(x):
    return pltpu.bitcast(x.astype(BF16), U32)


def _unpack(x):
    return pltpu.bitcast(x, BF16)


def _lhs_blocks(a11, a12, a21, a22):
    if STRASSEN:
        return [a11 + a22, a21 + a22, a11, a22, a11 + a12, a21 - a11, a12 - a22]
    return [a11, a12, a21, a22]


def _rhs_blocks(b11, b12, b21, b22):
    if STRASSEN:
        return [b11 + b22, b11, b12 - b22, b21 - b11, b22, b11 + b12, b21 + b22]
    return [b11, b12, b21, b22]


def _whole(fn):
    def prod(a, b):
        y = fn(a, b)
        yield
        return y
    return prod


def _tiled(lhs, rhs, nk, nn, dot, tick):
    def prod(a, b):
        acc = [None] * nn
        cnt = 0
        for n in range(nn):
            for k in range(nk):
                t = dot(lhs(a, k), rhs(b, k, n))
                acc[n] = t if k == 0 else acc[n] + t
                cnt += 1
                if cnt % 4 == 0:
                    tick(t)
                    yield
        return jnp.concatenate(acc, axis=1)
    return prod


def _block_matmul(prod, done):
    if STRASSEN:
        p3 = yield from prod(2, 2)
        p5 = yield from prod(4, 4)
        done(0, 1, p3 + p5)
        p2 = yield from prod(1, 1)
        p4 = yield from prod(3, 3)
        done(1, 0, p2 + p4)
        u, v = p4 - p5, p3 - p2
        p1 = yield from prod(0, 0)
        u, v = u + p1, v + p1
        p7 = yield from prod(6, 6)
        done(0, 0, u + p7)
        p6 = yield from prod(5, 5)
        done(1, 1, v + p6)
    else:
        for i in range(2):
            for j in range(2):
                t = yield from prod(2 * i, j)
                u = yield from prod(2 * i + 1, 2 + j)
                done(i, j, t + u)


def _run(gen, n=None):
    k = 0
    while n is None or k < n:
        if next(gen, "end") == "end":
            break
        k += 1


def _chain(*gens):
    for g in gens:
        yield from g


def _layernorm(x):
    m = jnp.mean(x, axis=-1, keepdims=True)
    xc = x - m
    v = jnp.mean(xc * xc, axis=-1, keepdims=True)
    return xc * lax.rsqrt(v + 1e-5)


def _phi(t):
    return jnp.where(t > 0, t + 1.0, jnp.exp(t))


def _kernel(x_hbm, beta_ref, wqkv_hbm, woa_hbm, wq_hbm, wk_hbm, wv_hbm, wob_hbm, out_ref,
            x_ref, raw, wa, woa, wqk, wvt, wob,
            xs, xa, xb, qb, kb, vb, kc, vc, of, oc, bq, bk, bv, mt, zs, gate, cmask, sems):
    seg = pl.program_id(0)
    rep = pl.program_id(1)

    def row_blocks(xn):
        return _lhs_blocks(xn[:128, :HD], xn[:128, HD:], xn[128:, :HD], xn[128:, HD:])

    def norm_blocks(ch):
        return row_blocks(_layernorm(xs[ch * RC:(ch + 1) * RC, :]))

    first_step = (seg == 0) & (rep == 0)
    c1 = 256

    def early_copy(i):
        m, j = divmod(i, 2)
        if m < 3:
            c0 = (1, 0, 2)[m] * D + j * HD
            return pltpu.make_async_copy(wqkv_hbm.at[:, pl.ds(c0, HD)], raw.at[m, :, pl.ds(j * HD, HD)], sems.at[i])
        return pltpu.make_async_copy(woa_hbm.at[pl.ds(j * HD, HD)], raw.at[3, pl.ds(j * HD, HD)], sems.at[i])

    pair0 = [pltpu.make_async_copy(s.at[:, pl.ds(0, c1)], raw.at[4 + i, :, pl.ds(0, c1)], sems.at[8 + i])
             for i, s in enumerate((wq_hbm, wk_hbm, wv_hbm))]
    late = [pltpu.make_async_copy(s.at[:, pl.ds(c1, D - c1)], raw.at[4 + i, :, pl.ds(c1, D - c1)], sems.at[11 + i])
            for i, s in enumerate((wq_hbm, wk_hbm, wv_hbm))]
    late.append(pltpu.make_async_copy(wob_hbm, raw.at[7], sems.at[14]))

    def selector(head_major):
        row = lax.broadcasted_iota(jnp.int32, (128, 128), 0)
        col = lax.broadcasted_iota(jnp.int32, (128, 128), 1)
        if not head_major:
            row = (((row >> 5) & 1) * 2 + (row & 1)) * DH + (row >> 6) * 16 + ((row >> 1) & 15)
        return jnp.where(row == col, 1.0, 0.0).astype(BF16)

    def packed_blocks(b11, b12, b21, b22):
        quad = (b11, b12, b21, b22)
        vals = [_unpack(b).astype(F32) for b in quad]
        out = []
        for blk in _rhs_blocks(*vals):
            same = [i for i, v in enumerate(vals) if v is blk]
            out.append(quad[same[0]] if same else _pack(blk))
        return out

    def raw_u32(m, rows, cols):
        return pltpu.bitcast(raw[m, rows, cols], U32)

    def prep_pair(t, carry):
        p = t // 2
        c0 = pl.multiple_of(p * 256, 256)
        for jj in range(2):
            j = (t % 2) * 2 + jj
            r0 = pl.multiple_of(j * 128, 128)
            y = _dot_nt(selector(True), jnp.concatenate(
                [raw[6, pl.ds(kh * HD + r0, 128), pl.ds(c0 + e * 128, 128)] for kh in range(2) for e in range(2)],
                axis=0))
            for i, v in enumerate(_rhs_blocks(*[y[:, c:c + 128] for c in range(0, HD, 128)])):
                wvt[p, i, :, pl.ds(r0, 128)] = _pack(v)
            for m in range(2):
                top = raw_u32(4 + m, pl.ds(r0, 128), pl.ds(c0, 256))
                bot = raw_u32(4 + m, pl.ds(HD + r0, 128), pl.ds(c0, 256))
                for i, v in enumerate(packed_blocks(top[:, :128], top[:, 128:], bot[:, :128], bot[:, 128:])):
                    wqk[p, i, pl.ds(pl.multiple_of(j * 64, 64), 64), m * 128:(m + 1) * 128] = v
        return carry

    def arrive(piece, lo, hi):
        for i in range(lo, hi):
            @pl.when(piece == i)
            def _():
                early_copy(i).wait()
                if i == 0:
                    early_copy(1).start()
                if i == 1:
                    for n in range(2, 6):
                        early_copy(n).start()

    def scatter(dst, t, blocks):
        for i, v in enumerate(blocks):
            v = _pack(v)
            for c in range(NT // 2):
                for hp in range(2):
                    dst(i, c)[pl.ds(t * 2 + hp, 16, stride=PITCH), :] = v[hp * 16:(hp + 1) * 16, c * 128:(c + 1) * 128]

    def perm_cols(u, carry):
        m = u // 2
        arrive(u, 0, 6)
        for tt in range(4):
            t = (u % 2) * 4 + tt
            c0 = pl.multiple_of(t * 128, 128)
            top = _dot_nt(selector(False), raw[m, 0:HD, pl.ds(c0, 128)])
            bot = _dot_nt(selector(False), raw[m, HD:D, pl.ds(c0, 128)])
            scatter(lambda i, c: wa.at[m, i, c], t, _rhs_blocks(top[:64], top[64:], bot[:64], bot[64:]))
        return carry

    def perm_rows(u, carry):
        arrive(6 + u, 6, 8)
        for tt in range(4):
            t = u * 4 + tt
            y = _dot(selector(False), raw[3, pl.ds(pl.multiple_of(t * 128, 128), 128), :])
            scatter(lambda i, c: woa.at[i, c], t, _rhs_blocks(y[:64, :HD], y[:64, HD:], y[64:, :HD], y[64:, HD:]))
        return carry

    def x_copy(s):
        return pltpu.make_async_copy(x_hbm.at[pl.ds(pl.multiple_of(s * L, L), L)], x_ref, sems.at[15])

    @pl.when(first_step)
    def _prologue():
        early_copy(0).start()
        x_copy(0).start()
        kc[...] = jnp.zeros(kc.shape, F32)
        vc[...] = jnp.zeros(vc.shape, F32)
        mt[...] = jnp.zeros(mt.shape, F32)
        zs[...] = jnp.zeros(zs.shape, F32)
        g_all = jax.nn.sigmoid(beta_ref[...].astype(F32))
        lane_h = lax.broadcasted_iota(jnp.int32, (1, H), 1)
        for h in range(H):
            gh = jnp.sum(jnp.where(lane_h == h, g_all, 0.0), axis=1, keepdims=True)
            gate[h] = jnp.broadcast_to(gh, (8, 128))
        kk = lax.broadcasted_iota(jnp.int32, (128, 256), 0)
        qq = lax.broadcasted_iota(jnp.int32, (128, 256), 1)
        qq = jnp.where(qq < 128, qq ^ 64, qq - 128)
        cmask[...] = jnp.where(qq < kk, NEG, 0.0).astype(F32)

        perm_cols(0, 0)
        x_copy(0).wait()

        def load_x(j, carry):
            r0 = pl.multiple_of(j * 64, 64)
            x0 = x_ref[pl.ds(r0, 64), :].astype(F32)
            xs[pl.ds(r0, 64), :] = x0
            xa[pl.ds(r0, 64), :] = _layernorm(x0)
            xs[pl.ds(RC + r0, 64), :] = x_ref[pl.ds(RC + r0, 64), :].astype(F32)
            return carry
        lax.fori_loop(0, RC // 64, load_x, 0)
        perm_cols(1, 0)

    fetch_next = (rep == 1) & (seg < NSEG - 1)
    pl.when(fetch_next)(lambda: x_copy(seg + 1).start())

    def _mid_weights():
        for c in [early_copy(6), early_copy(7)] + pair0:
            c.start()
        lax.fori_loop(2, 6, perm_cols, 0)

        lax.fori_loop(0, 2, perm_rows, 0)
        for c in late:
            c.start()
        for c in pair0:
            c.wait()
        lax.fori_loop(0, 2, prep_pair, 0)

    def _late_weights():
        for c in late:
            c.wait()
        lax.fori_loop(2, NT, prep_pair, 0)

        def comb_ob(t, carry):
            p, j = t // 2, t % 2
            r0 = pl.multiple_of(p * 256 + j * 64, 64)
            top = raw_u32(7, pl.ds(r0, 64), slice(None))
            bot = raw_u32(7, pl.ds(r0 + 128, 64), slice(None))
            for i, v in enumerate(packed_blocks(top[:, :HD], top[:, HD:], bot[:, :HD], bot[:, HD:])):
                wob[i, pl.ds(pl.multiple_of(t * 32, 32), 32), :] = v
            return carry
        lax.fori_loop(0, 8, comb_ob, 0)

    for c in range(NT):
        kb[c, 0:HALO, :] = kc[rep, c]
        vb[c, 0:HALO, :] = vc[rep, c]

    ticks = []

    def tick(y):
        ticks.extend(y[0:8, c:c + 128] for c in range(0, y.shape[1], 128))
        return y

    def after(t, x):
        return x if t < 0 else jnp.where(cmask[0:8, 0:128] > 1.0, ticks[min(t, len(ticks) - 1)], x)

    def before(deps, a):
        if not deps:
            return a
        head = a[0:8, 0:128]
        for d in deps:
            head = jnp.where(cmask[0:8, 0:128] > 1.0, d, head)
        top = jnp.concatenate([head, a[0:8, 128:]], axis=1)
        return jnp.concatenate([top, a[8:]], axis=0)

    def permuted(ref):
        return _unpack(jnp.concatenate([jnp.concatenate(
            [ref[c, d * PITCH:d * PITCH + 16, :] for d in range(16)], axis=0) for c in range(NT // 2)], axis=1))

    def a_proj(ch, m, lhs):
        dst, off = ((kb, HALO), (qb, 0), (vb, HALO))[m]

        def done(i, j, y):
            r0 = off + ch * RC + i * 128
            if m == 1:
                y = y * QSCALE
            for c in range(NT // 2):
                dst[j * NT // 2 + c, r0:r0 + 128, :] = y[:, c * 128:(c + 1) * 128]
        return _block_matmul(
            _whole(lambda a, b: tick(_dot_nt(lhs(a).astype(BF16), permuted(wa.at[m, b])))), done)

    def a_probs(r0, t):
        accs = [None] * W
        for c in range(NT):
            qc = after(t, qb[c, r0:r0 + 8, :])
            for w in range(W):
                o0 = HALO + r0 - DIL * w
                u = qc * kb[c, o0:o0 + 8, :]
                accs[w] = u if c == 0 else accs[w] + u
        ls = []
        for w in range(W):
            acc = accs[w]
            acc = acc + pltpu.roll(acc, 64, 1)
            acc = acc + pltpu.roll(acc, 32, 1)
            if r0 < DIL * w:
                pos = seg * L + r0 + lax.broadcasted_iota(jnp.int32, (8, 128), 0)
                acc = jnp.where(pos >= DIL * w, acc, NEG)
            ls.append(acc)
        mx = functools.reduce(jnp.maximum, ls)
        es = [jnp.exp2(l - mx) for l in ls]
        inv = pl.reciprocal(functools.reduce(jnp.add, es), full_range=False)
        return es, inv

    def a_mix(r0, es, inv):
        ps = [e * inv for e in es]
        outs = []
        for c in range(NT):
            acc = None
            for w in range(W):
                o0 = HALO + r0 - DIL * w
                u = ps[w] * vb[c, o0:o0 + 8, :]
                acc = u if acc is None else acc + u
            outs.append(acc)
        return jnp.concatenate(outs, axis=1)

    def a_attn_chunk(ch, t0, dt0, t1, dt1):
        n = RC // 8
        rows = [None] * n
        for i in range(n):
            r = i // 2 + (i % 2) * (n // 2)
            es, inv = a_probs(ch * RC + r * 8, int(t0 + i * dt0))
            rows[r] = a_mix(ch * RC + r * 8, es, after(int(t1 + i * dt1), inv))
        return rows

    def add_rows(ch):
        def done(i, j, y):
            r0 = ch * RC + i * 128
            xs[r0:r0 + 128, j * HD:(j + 1) * HD] += y
        return done

    def a_out(ch, lhs):
        return _block_matmul(_whole(lambda a, b: tick(_dot(lhs(a).astype(BF16), permuted(woa.at[b])))), add_rows(ch))

    def tile(i):
        return slice(i * 128, (i + 1) * 128)

    def b_proj_qk(p, ch, lhs=None):
        def done(i, j, y):
            r0 = ch * RC + i * 128
            bq[j, r0:r0 + 128, :] = y[:, :128]
            bk[j, r0:r0 + 128, :] = y[:, 128:]
        if lhs is not None:
            return _block_matmul(_whole(lambda a, b: tick(_dot(lhs[a].astype(BF16), _unpack(wqk[p, b])))), done)
        return _block_matmul(_tiled(
            lambda a, k: _unpack(xb[a, ch * 64:(ch + 1) * 64, tile(k)]),
            lambda b, k, n: _unpack(wqk[p, b, k * 64:(k + 1) * 64, tile(n)]), 4, 2, _dot, tick), done)

    def b_proj_v(p):
        def done(i, j, y):
            for ch in range(NCH):
                c0 = ch * RC + i * 128
                bv[j, :, c0:c0 + 128] = _pack(y[:, tile(ch)])
        return _block_matmul(_tiled(
            lambda a, k: a, lambda b, k, n: (b, k, n), 4, NCH,
            lambda a, t: _dot_nt(_unpack(wvt[p, t[0], :, tile(t[1])]),
                                 _unpack(xb[a, t[2] * 64:(t[2] + 1) * 64, tile(t[1])])), tick), done)

    def finish_rows(ch):
        def done(i, j, y):
            idx = (slice(ch * RC + i * 128, ch * RC + (i + 1) * 128), slice(j * HD, (j + 1) * HD))
            xnew = xs[idx] + y
            out_ref[idx] = xnew.astype(BF16)
            xs[idx] = jnp.where(rep == 0, xnew, x_ref[idx].astype(F32))
        return done

    def b_out(ch, p0, p1):
        def prod(a, b):
            acc = None
            for p in range(p0, p1):
                t = _dot(_unpack(oc[p, a, ch * 64:(ch + 1) * 64, :]), _unpack(wob[b, p * 64:(p + 1) * 64, :]))
                acc = t if acc is None else acc + t
                tick(t[:, 0:128])
                yield
            return acc
        return _block_matmul(prod, finish_rows(ch) if p1 == NT // 2 else add_rows(ch))

    lane = lax.broadcasted_iota(jnp.int32, (1, 128), 1) // DH

    def head_queries(q, j):
        qj = q[tile(j), :]
        qh = [qj * jnp.where(lane == h, QSCALE, 0.0) for h in range(4)]
        return [(t[:64], t[64:]) for t in qh]

    def corner(q, k, j):
        qm = jnp.concatenate([hi for _, hi in head_queries(q, j)], axis=0)
        return _dot_nt(k[j * 128 + 64:(j + 1) * 128].astype(BF16), qm.astype(BF16))

    def scores(q, k, j, cor):
        nk = 128 * j + 64
        qm = jnp.concatenate([part for h, (lo, hi) in enumerate(head_queries(q, j))
                              for part in ((lo, hi) if h % 2 else (hi, lo))], axis=0)
        st = _dot_nt(k[0:nk].astype(BF16), qm.astype(BF16))
        for i in range(j + 1):
            tick(st[i * 128:i * 128 + 8, 0:128])
        diag = jnp.concatenate([st[nk - 64:], jnp.concatenate([cor[:, tile(h // 2)] for h in range(4)], axis=1)],
                               axis=0)
        diag = diag + jnp.concatenate([cmask[...]] * 2, axis=1)
        return diag if j == 0 else jnp.concatenate([st[:nk - 64], diag], axis=0)

    def memory(g, q):
        pq = _phi(q).astype(BF16)
        zrow = lax.broadcasted_iota(jnp.int32, (16, 128), 0)
        zl = jnp.where(zrow == lane, jnp.broadcast_to(zs[rep * NT + g, 0:1, :], (16, 128)), 0.0)
        lhs = jnp.concatenate([mt[rep * NT + g], zl], axis=0).astype(BF16)
        return _dot_nt(lhs, pq)

    def update(g, k, vt):
        pk = _phi(k)
        upd = functools.reduce(jnp.add, [
            _dot(_unpack(vt[:, i * 128:(i + 1) * 128]), pk[i * 128:(i + 1) * 128].astype(BF16)) for i in range(L // 128)])
        rr = lax.broadcasted_iota(jnp.int32, (128, 128), 0) // DH
        mt[rep * NT + g] += jnp.where(rr == lane, upd, 0.0)
        zs[rep * NT + g] += jnp.sum(pk, axis=0, keepdims=True)

    def attend(g, e, j, st, nd, vt):
        mx = jnp.broadcast_to(jnp.max(st, axis=0, keepdims=True), (8, 512))
        pv, l = [None] * 4, None
        for i in range(j + 1):
            mi = jnp.concatenate([after(len(ticks) - GATE, mx[:, tile(h)]) for h in range(4)], axis=1)
            p3 = jnp.exp2(st[tile(i)].reshape(16, 8, 512) - mi)
            p = p3.reshape(128, 512)
            li = jnp.sum(p3, axis=0)
            l = li if i == 0 else l + li
            for h in range(4):
                t = _dot(_unpack(vt[h * 16:(h + 1) * 16, tile(i)]), p[:, tile(h)].astype(BF16))
                pv[h] = t if i == 0 else pv[h] + t
            if i < j:
                yield
        l = jnp.sum(l, axis=0, keepdims=True)
        rows = []
        for h in range(4):
            gh = gate[g * 4 + h][0:1, :]
            num = nd[h * DH:(h + 1) * DH, tile(j)]
            den = nd[128 + h:129 + h, tile(j)] + 1e-6
            loc = pv[h] * ((1.0 - gh) * pl.reciprocal(l[:, tile(h)], full_range=False))
            rows.append(num * (gh / den) + (loc if h % 2 else pltpu.roll(loc, 64, 1)))
        of[e, tile(j), :] = jnp.concatenate(rows, axis=0).T
        yield

    def b_out_blocks(p, ch):
        r0 = ch * RC
        blocks = _lhs_blocks(of[0, r0:r0 + 128, :], of[1, r0:r0 + 128, :],
                             of[0, r0 + 128:r0 + 256, :], of[1, r0 + 128:r0 + 256, :])
        for i, b in enumerate(blocks):
            oc[p, i, ch * 64:(ch + 1) * 64, :] = _pack(b)

    def due_rows(blocks, counts, lhs):
        counts, seen = iter(counts), [0]

        def held(a):
            n = next(counts)
            deps = [b[r * 8:r * 8 + 8, c:c + 128] for r in range(seen[0], seen[0] + n)
                    for b in blocks[-2:] for c in range(0, HD, 128)]
            seen[0] += n
            return before(deps, lhs[a])
        return held

    xn1 = _layernorm(xs[RC:L, :])
    xa[RC:L, :] = xn1
    a_in = [row_blocks(xa[0:RC, :]), row_blocks(xn1)]
    _run(a_proj(0, 0, due_rows(a_in[1], [int(v) for v in os.environ.get("DUEK", "0,2,2,3,3,3,3").split(",")], a_in[0])))
    _run(a_proj(1, 0, lambda a: a_in[1][a]))
    pl.when(first_step)(_mid_weights)
    del ticks[:]
    a_in = [row_blocks(xa[ch * RC:(ch + 1) * RC, :]) for ch in range(NCH)]
    with jax.named_scope("sc_A"):
        tm = (7 if STRASSEN else 8) * 4
        P = [float(v) for v in os.environ.get("PACE", "1,0.85,2.86,0.75,2,0.85,3.86,0.1").split(",")]
        for ch, m in [divmod(int(c), 3) for c in os.environ.get("ORD", "1425")]:
            _run(a_proj(ch, m, lambda a, ch=ch: a_in[ch][a]))
        o0 = row_blocks(jnp.concatenate(a_attn_chunk(0, P[0] * tm, P[1], P[2] * tm, P[3]), axis=0))
        rows1 = a_attn_chunk(1, P[4] * tm, P[5], P[6] * tm, P[7])
        o1 = row_blocks(jnp.concatenate(rows1, axis=0))
        _run(a_out(0, due_rows(o1, [int(v) for v in os.environ.get("DUE", "0,1,2,2,3,3,3").split(",")], o0)))
        x0 = norm_blocks(0)
        first = b_proj_qk(0, 0, x0)
        _run(first, FIRST)
        t0 = len(ticks)
        _run(a_out(1, lambda a: o1[a]))
        _run(first)
        x1 = norm_blocks(1)
        t1 = len(ticks)
        _run(b_proj_qk(0, 1, x1))
        for ch, (blocks, t, dt) in enumerate(((x0, t0, 3), (x1, t1, 1))):
            for i, blk in enumerate(blocks):
                for r in range(0, 128, 32):
                    g = jnp.concatenate([ticks[t + i * dt]] * 4, axis=0)
                    g = jnp.concatenate([g] * 4, axis=1)
                    nv = jnp.concatenate([cmask[0:32, 0:128]] * 4, axis=1) > 1.0
                    xb[i, ch * 64 + r // 2:ch * 64 + r // 2 + 16, :] = _pack(jnp.where(nv, g, blk[r:r + 32]))
        _run(b_proj_v(0))
        for c in range(NT):
            kc[rep, c] = kb[c, L:L + HALO, :]
            vc[rep, c] = vb[c, L:L + HALO, :]

    npair = NT // 2

    def b_pair(p, last):
        del ticks[:]
        qs = [bq[e] for e in range(2)]
        ks = [bk[e] for e in range(2)]
        vts = [bv[e] for e in range(2)]
        if last:
            fill = _chain(b_out(0, 0, p), b_out(1, 0, SPLIT)) if SPLIT else b_out(0, 0, p)
            plan = os.environ.get("PLANL", "f s0 s1 n f p s2 p f p s3 f p f p f p f f p f p f p f p f u f "
                                  "/ s0 s1 n f p f s2 p f p o s3 f p f p f p f x p f x p f x p f x p o f x u f x F X")
            tail = b_out(0, p, p + 1)
        else:
            fill = _chain(b_proj_qk(p + 1, 0), b_proj_qk(p + 1, 1), b_proj_v(p + 1))
            plan = os.environ.get("PLAN", "f s3 f f s2 f n p f p f p f f p s1 p f f p f p f s0 f p f f p f u f f p "
                                  "/ s3 f s2 n f p f p f p f p f f s1 p f p f p o s0 f f p f p f u f p o F")
        for e, steps in enumerate(plan.split("/")):
            g = 2 * p + e
            q, k, vt = qs[e], ks[e], vts[e]
            todo, cur, nd, seen, cors = [], None, None, [], {}
            for op in steps.split():
                if op == "f":
                    _run(fill, 1)
                elif op == "F":
                    _run(fill)
                elif op == "x":
                    _run(tail, 1)
                elif op == "X":
                    _run(tail)
                    xa[0:RC, :] = _layernorm(xs[0:RC, :])
                elif op[0] == "s":
                    j = int(op[1])
                    if j not in cors:
                        cors.update({i: corner(q, k, i) for i in (j, j ^ 1)})
                    todo.append((j, scores(q, k, j, cors[j])))
                elif op == "n":
                    nd = memory(g, q)
                elif op == "u":
                    update(g, k, vt)
                elif op == "o":
                    if e:
                        b_out_blocks(p, seen[-1] // 2)
                else:
                    if cur is None or next(cur, "end") == "end":
                        j, st = todo.pop(0)
                        seen.append(j)
                        cur = attend(g, e, j, st, nd, vt)
                        next(cur)
            assert not todo and next(cur, "end") == "end"

    pl.when(first_step)(_late_weights)
    pl.when(fetch_next)(lambda: x_copy(seg + 1).wait())
    with jax.named_scope("sc_Bloop"):
        lax.fori_loop(0, npair - 1, lambda p, c: (b_pair(p, False), c)[1], 0)
    with jax.named_scope("sc_Blast"):
        b_pair(npair - 1, True)
        _run(b_out(1, SPLIT, npair))


@jax.jit
def pallas_interleave_layers__sliding_local_dilated__memory_aug_infini_attn__prompt_kernel(
        A_x, A_wqkv, A_wo, B_x, B_wq, B_wk, B_wv, B_wo, B_beta):
    del B_x
    hbm = pl.BlockSpec(memory_space=pl.ANY)
    out = pl.pallas_call(
        _kernel,
        grid=(NSEG, 2),
        in_specs=[hbm,
                  pl.BlockSpec((1, H), lambda s, r: (0, 0)),
                  hbm, hbm, hbm, hbm, hbm, hbm],
        out_specs=pl.BlockSpec((L, D), lambda s, r: (s, 0)),
        out_shape=jax.ShapeDtypeStruct((S, D), BF16),
        scratch_shapes=[
            pltpu.VMEM((L, D), BF16),
            pltpu.VMEM((8, D, D), BF16),
            pltpu.VMEM((3, NP, NT // 2, WROWS, 128), U32),
            pltpu.VMEM((NP, NT // 2, WROWS, 128), U32),
            pltpu.VMEM((NT // 2, NP, HD // 2, 256), U32),
            pltpu.VMEM((NT // 2, NP, 64, HD), U32),
            pltpu.VMEM((NP, HD // 2, HD), U32),
            pltpu.VMEM((L, D), F32),
            pltpu.VMEM((L, D), F32),
            pltpu.VMEM((NP, L // 4, HD), U32),
            pltpu.VMEM((NT, L, 128), F32),
            pltpu.VMEM((NT, HALO + L, 128), F32),
            pltpu.VMEM((NT, HALO + L, 128), F32),
            pltpu.VMEM((2, NT, HALO, 128), F32),
            pltpu.VMEM((2, NT, HALO, 128), F32),
            pltpu.VMEM((2, L, 128), F32),
            pltpu.VMEM((NT // 2, NP, L // 4, 128), U32),
            pltpu.VMEM((2, L, 128), F32),
            pltpu.VMEM((2, L, 128), F32),
            pltpu.VMEM((2, 64, L), U32),
            pltpu.VMEM((2 * NT, 128, 128), F32),
            pltpu.VMEM((2 * NT, 8, 128), F32),
            pltpu.VMEM((H, 8, 128), F32),
            pltpu.VMEM((128, 256), F32),
            pltpu.SemaphoreType.DMA((16,)),
        ],
        compiler_params=pltpu.CompilerParams(
            dimension_semantics=("arbitrary", "arbitrary"),
            vmem_limit_bytes=110 * 2**20,
            flags={k: True for k in os.environ.get('FL', '').split(',') if k} or None),
        name="interleave",
    )(A_x.reshape(S, D), B_beta.reshape(1, H), A_wqkv, A_wo, B_wq, B_wk, B_wv, B_wo)
    return out.reshape(1, S, D)
```

```python
import functools
import math

import jax
import jax.numpy as jnp
from jax import lax
from jax.experimental import pallas as pl
from jax.experimental.pallas import tpu as pltpu

S, D, H, DH = 2048, 1024, 32, 32
NSEG = 4
L = S // NSEG
W, DIL = 8, 2
HALO = 16
NT = D // 128
NPAIR = NT // 2
HD = D // 2
RC = 256
NCH = L // RC
NP = 7
PITCH = 17
WROWS = 16 * PITCH + 16
LOG2E = math.log2(math.e)
QSCALE = DH ** -0.5 * LOG2E
NEG = -1e9 * LOG2E
F32, BF16, U32 = jnp.float32, jnp.bfloat16, jnp.uint32

TUNE = dict(
    pace=((24, 1.05, 80, 0.75), (52, 1.1, 108, 0.1)),
    due_norm=(0, 2, 2, 3, 3, 3, 3),
    due_probs=(0, 0, 0, 0, 0, 0, 0, 0, 3, 4, 4, 4, 4, 4, 4, 4, 4, 4, 4, 4, 4, 4, 3, 3, 3, 0, 0, 0),
    due_mix0=(0, 0, 2, 6, 7, 6, 9),
    due_mix1=(0, 0, 3, 3, 4, 2, 3),
    due_norm0=(0, 1, 2, 2, 3, 3, 5),
    due_norm1=(0, 0, 2, 1, 4, 4, 2),
    keep=((10, 2), (0, 1)),
    gate=3,
    split=2,
    plan="f s3 f f s2 f n p f p f p f f p s1 p f f p f p f s0 f p f f p f u f f p "
         "/ s3 f s2 n f p f p f p f p f f s1 p f p f p o s0 f f p f p f u f p o F",
    plan_last="f s0 s1 n f p s2 p f p s3 f p f p f p f p f p f p f f p f u "
              "/ s0 s1 f n f p s2 p f p o s3 f p f p p f x f p x p f f x p f x p o f x x u F X",
)


def _dot(a, b):
    return jnp.dot(a, b, preferred_element_type=F32)


def _dot_nt(a, b):
    return lax.dot_general(a, b, (((1,), (1,)), ((), ())), preferred_element_type=F32)


def _pack(x):
    return pltpu.bitcast(x.astype(BF16), U32)


def _unpack(x):
    return pltpu.bitcast(x, BF16)


def _tile(i):
    return slice(i * 128, (i + 1) * 128)


def _lhs_blocks(a11, a12, a21, a22):
    return [a11 + a22, a21 + a22, a11, a22, a11 + a12, a21 - a11, a12 - a22]


def _rhs_blocks(b11, b12, b21, b22):
    return [b11 + b22, b11, b12 - b22, b21 - b11, b22, b11 + b12, b21 + b22]


def _row_blocks(x):
    return _lhs_blocks(x[:128, :HD], x[:128, HD:], x[128:, :HD], x[128:, HD:])


def _block_matmul(prod, done):
    p3 = yield from prod(2)
    p5 = yield from prod(4)
    done(0, 1, p3 + p5)
    p2 = yield from prod(1)
    p4 = yield from prod(3)
    done(1, 0, p2 + p4)
    u, v = p4 - p5, p3 - p2
    p1 = yield from prod(0)
    u, v = u + p1, v + p1
    p7 = yield from prod(6)
    done(0, 0, u + p7)
    p6 = yield from prod(5)
    done(1, 1, v + p6)


def _whole(fn):
    def prod(i):
        y = fn(i)
        yield
        return y
    return prod


def _tiled(dot, nk, nn, tick):
    def prod(i):
        acc = [None] * nn
        for n in range(nn):
            for k in range(nk):
                t = dot(i, k, n)
                acc[n] = t if k == 0 else acc[n] + t
            tick(t)
            yield
        return jnp.concatenate(acc, axis=1)
    return prod


def _run(gen, n=None):
    k = 0
    while (n is None or k < n) and next(gen, "end") != "end":
        k += 1


def _chain(*gens):
    for g in gens:
        yield from g


def _layernorm(x):
    m = jnp.mean(x, axis=-1, keepdims=True)
    xc = x - m
    v = jnp.mean(xc * xc, axis=-1, keepdims=True)
    return xc * lax.rsqrt(v + 1e-5)


def _phi(t):
    return jnp.where(t > 0, t + 1.0, jnp.exp(t))


def _kernel(x_hbm, beta_ref, wqkv_hbm, woa_hbm, wq_hbm, wk_hbm, wv_hbm, wob_hbm, out_ref,
            xin, raw_a, raw_ao, raw_b, raw_bo, wa, woa, wqk, wvt, wob,
            xs, xa, xb, qb, kb, vb, kc, vc, of, oc, bq, bk, bv, mt, zs, gate, cmask, sems):
    seg = pl.program_id(0)
    rep = pl.program_id(1)
    first_step = (seg == 0) & (rep == 0)

    def window_copy(i):
        m, j = divmod(i, 2)
        if m < 3:
            c0 = (1, 0, 2)[m] * D + j * HD
            return pltpu.make_async_copy(wqkv_hbm.at[:, pl.ds(c0, HD)], raw_a.at[i], sems.at[i])
        return pltpu.make_async_copy(woa_hbm.at[pl.ds(j * HD, HD)], raw_ao.at[j], sems.at[i])

    def pair_copies(p):
        return [pltpu.make_async_copy(w.at[:, pl.ds(p * 256, 256)], raw_b.at[m, p], sems.at[8 + 3 * p + m])
                for m, w in enumerate((wq_hbm, wk_hbm, wv_hbm))]

    def late_copies():
        return ([c for p in range(1, NPAIR) for c in pair_copies(p)]
                + [pltpu.make_async_copy(wob_hbm, raw_bo, sems.at[20])])

    def x_copy(s):
        return pltpu.make_async_copy(x_hbm.at[pl.ds(pl.multiple_of(s * L, L), L)], xin, sems.at[21])

    def selector(reorder):
        row = lax.broadcasted_iota(jnp.int32, (128, 128), 0)
        col = lax.broadcasted_iota(jnp.int32, (128, 128), 1)
        if reorder:
            row = (((row >> 5) & 1) * 2 + (row & 1)) * DH + (row >> 6) * 16 + ((row >> 1) & 15)
        return jnp.where(row == col, 1.0, 0.0).astype(BF16)

    def packed_blocks(*quad):
        quad = [pltpu.bitcast(b, U32) for b in quad]
        vals = [_unpack(b).astype(F32) for b in quad]
        out = []
        for blk in _rhs_blocks(*vals):
            same = [i for i, v in enumerate(vals) if v is blk]
            out.append(quad[same[0]] if same else _pack(blk))
        return out

    def arrive(piece, lo, hi):
        for i in range(lo, hi):
            @pl.when(piece == i)
            def _():
                window_copy(i).wait()
                for n in {0: (1,), 1: (2, 3, 4, 5)}.get(i, ()):
                    window_copy(n).start()

    def scatter(dst, t, blocks):
        for i, v in enumerate(blocks):
            v = _pack(v)
            for c in range(NPAIR):
                for hp in range(2):
                    dst(i, c)[pl.ds(t * 2 + hp, 16, stride=PITCH), :] = v[hp * 16:(hp + 1) * 16, _tile(c)]

    def prep_window_in(piece, carry):
        arrive(piece, 0, 6)
        for t in range(4):
            top = _dot_nt(selector(True), raw_a[piece, 0:HD, _tile(t)])
            bot = _dot_nt(selector(True), raw_a[piece, HD:D, _tile(t)])
            scatter(lambda i, c: wa.at[piece // 2, i, c], (piece % 2) * 4 + t,
                    _rhs_blocks(top[:64], top[64:], bot[:64], bot[64:]))
        return carry

    def prep_window_out(j, carry):
        arrive(6 + j, 6, 8)
        for t in range(4):
            y = _dot(selector(True), raw_ao[j, _tile(t), :])
            scatter(lambda i, c: woa.at[i, c], j * 4 + t,
                    _rhs_blocks(y[:64, :HD], y[:64, HD:], y[64:, :HD], y[64:, HD:]))
        return carry

    def prep_pair(t, carry):
        p = t // 2
        for jj in range(2):
            j = (t % 2) * 2 + jj
            top = pl.ds(pl.multiple_of(j * 128, 128), 128)
            bot = pl.ds(pl.multiple_of(HD + j * 128, 128), 128)
            y = _dot_nt(selector(False), jnp.concatenate(
                [raw_b[2, p, rows, _tile(e)] for rows in (top, bot) for e in range(2)], axis=0))
            for i, v in enumerate(_rhs_blocks(*[y[:, _tile(c)] for c in range(4)])):
                wvt[p, i, :, top] = _pack(v)
            for m in range(2):
                quad = [raw_b[m, p, rows, _tile(e)] for rows in (top, bot) for e in range(2)]
                for i, v in enumerate(packed_blocks(*quad)):
                    wqk[p, i, pl.ds(pl.multiple_of(j * 64, 64), 64), _tile(m)] = v
        return carry

    def prep_memory_out(t, carry):
        r0 = (t // 2) * 256 + (t % 2) * 64
        quad = [raw_bo[pl.ds(pl.multiple_of(r0 + e * 128, 64), 64), c:c + HD] for e in range(2) for c in (0, HD)]
        for i, v in enumerate(packed_blocks(*quad)):
            wob[i, pl.ds(pl.multiple_of(t * 32, 32), 32), :] = v
        return carry

    @pl.when(first_step)
    def _start():
        window_copy(0).start()
        x_copy(0).start()
        kc[...] = jnp.zeros(kc.shape, F32)
        vc[...] = jnp.zeros(vc.shape, F32)
        mt[...] = jnp.zeros(mt.shape, F32)
        zs[...] = jnp.zeros(zs.shape, F32)
        g_all = jax.nn.sigmoid(beta_ref[...].astype(F32))
        head = lax.broadcasted_iota(jnp.int32, (1, H), 1)
        for h in range(H):
            gate[h] = jnp.broadcast_to(jnp.sum(jnp.where(head == h, g_all, 0.0), axis=1, keepdims=True), (8, 128))
        kk = lax.broadcasted_iota(jnp.int32, (128, 256), 0)
        qq = lax.broadcasted_iota(jnp.int32, (128, 256), 1)
        qq = jnp.where(qq < 128, qq ^ 64, qq - 128)
        cmask[...] = jnp.where(qq < kk, NEG, 0.0).astype(F32)
        prep_window_in(0, 0)
        x_copy(0).wait()

        def load_rows(j, carry):
            rows = pl.ds(pl.multiple_of(j * 64, 64), 64)
            later = pl.ds(pl.multiple_of(RC + j * 64, 64), 64)
            x0 = xin[rows, :].astype(F32)
            xs[rows, :] = x0
            xa[rows, :] = _layernorm(x0)
            xs[later, :] = xin[later, :].astype(F32)
            return carry
        lax.fori_loop(0, RC // 64, load_rows, 0)
        prep_window_in(1, 0)

    def _more_weights():
        for c in [window_copy(6), window_copy(7)] + pair_copies(0):
            c.start()
        lax.fori_loop(2, 6, prep_window_in, 0)
        lax.fori_loop(0, 2, prep_window_out, 0)
        for c in late_copies():
            c.start()
        for c in pair_copies(0):
            c.wait()
        lax.fori_loop(0, 2, prep_pair, 0)

    def _last_weights():
        for c in late_copies():
            c.wait()
        lax.fori_loop(2, NT, prep_pair, 0)
        lax.fori_loop(0, 8, prep_memory_out, 0)

    ticks = []

    def tick(y):
        ticks.extend(y[0:8, c:c + 128] for c in range(0, y.shape[1], 128))
        return y

    def never(rows, tiles=1):
        return jnp.concatenate([cmask[0:rows, 0:128]] * tiles, axis=1) > 1.0

    def after(t, x):
        return x if t < 0 else jnp.where(never(8), ticks[min(t, len(ticks) - 1)], x)

    def before(deps, a):
        if not deps:
            return a
        head = jnp.where(never(8), functools.reduce(jnp.maximum, deps), a[0:8, 0:128])
        return jnp.concatenate([jnp.concatenate([head, a[0:8, 128:]], axis=1), a[8:]], axis=0)

    def held_for(blocks, counts, lhs):
        counts, seen = iter(counts), [0]

        def held(i):
            n = next(counts)
            deps = [b[r * 8:r * 8 + 8, _tile(c)] for r in range(seen[0], seen[0] + n)
                    for b in blocks[-2:] for c in range(NPAIR)]
            seen[0] += n
            return before(deps, lhs[i])
        return held

    def reordered(ref):
        return _unpack(jnp.concatenate([jnp.concatenate(
            [ref[c, d * PITCH:d * PITCH + 16, :] for d in range(16)], axis=0) for c in range(NPAIR)], axis=1))

    def window_in(ch, m, lhs):
        dst, off = ((kb, HALO), (qb, 0), (vb, HALO))[m]

        def done(i, j, y):
            r0 = off + ch * RC + i * 128
            if m == 1:
                y = y * QSCALE
            for c in range(NPAIR):
                dst[j * NPAIR + c, r0:r0 + 128, :] = y[:, _tile(c)]
        return _block_matmul(
            _whole(lambda i: tick(_dot_nt(lhs(i).astype(BF16), reordered(wa.at[m, i])))), done)

    def taps(ref, c, r0, w):
        o0 = HALO + r0 - DIL * w
        return ref[c, o0:o0 + 8, :]

    def row_group(i):
        return i // 2 + (i % 2) * (RC // 16)

    @functools.cache
    def window_probs(ch, i):
        r0 = ch * RC + row_group(i) * 8
        t = int(TUNE["pace"][ch][0] + i * TUNE["pace"][ch][1])
        qs = [after(t, qb[c, r0:r0 + 8, :]) for c in range(NT)]
        logits = []
        for w in range(W):
            acc = functools.reduce(jnp.add, [qs[c] * taps(kb, c, r0, w) for c in range(NT)])
            acc = acc + pltpu.roll(acc, 64, 1)
            acc = acc + pltpu.roll(acc, 32, 1)
            if r0 < DIL * w:
                pos = seg * L + r0 + lax.broadcasted_iota(jnp.int32, (8, 128), 0)
                acc = jnp.where(pos >= DIL * w, acc, NEG)
            logits.append(acc)
        mx = functools.reduce(jnp.maximum, logits)
        es = [jnp.exp2(v - mx) for v in logits]
        return es, 1.0 / functools.reduce(jnp.add, es)

    @functools.cache
    def window_rows(ch, i):
        r0 = ch * RC + row_group(i) * 8
        es, inv = window_probs(ch, i)
        inv = after(int(TUNE["pace"][ch][2] + i * TUNE["pace"][ch][3]), inv)
        ps = [e * inv for e in es]
        return jnp.concatenate(
            [functools.reduce(jnp.add, [ps[w] * taps(vb, c, r0, w) for w in range(W)]) for c in range(NT)], axis=1)

    def window_blocks(ch):
        rows = [None] * (RC // 8)
        for i in range(RC // 8):
            rows[row_group(i)] = window_rows(ch, i)
        return _row_blocks(jnp.concatenate(rows, axis=0))

    def add_rows(ch):
        def done(i, j, y):
            r0 = ch * RC + i * 128
            xs[r0:r0 + 128, j * HD:(j + 1) * HD] += y
        return done

    def window_out(ch, lhs):
        return _block_matmul(
            _whole(lambda i: tick(_dot(lhs(i).astype(BF16), reordered(woa.at[i])))), add_rows(ch))

    def memory_qk(p, ch, lhs=None):
        def done(i, j, y):
            r0 = ch * RC + i * 128
            bq[j, r0:r0 + 128, :] = y[:, :128]
            bk[j, r0:r0 + 128, :] = y[:, 128:]
        if lhs is not None:
            return _block_matmul(_whole(lambda i: tick(_dot(lhs(i).astype(BF16), _unpack(wqk[p, i])))), done)
        return _block_matmul(_tiled(
            lambda i, k, n: _dot(_unpack(xb[i, ch * 64:(ch + 1) * 64, _tile(k)]),
                                 _unpack(wqk[p, i, k * 64:(k + 1) * 64, _tile(n)])), 4, 2, tick), done)

    def memory_v(p):
        def done(i, j, y):
            for ch in range(NCH):
                c0 = ch * RC + i * 128
                bv[j, :, c0:c0 + 128] = _pack(y[:, _tile(ch)])
        return _block_matmul(_tiled(
            lambda i, k, n: _dot_nt(_unpack(wvt[p, i, :, _tile(k)]),
                                    _unpack(xb[i, n * 64:(n + 1) * 64, _tile(k)])), 4, NCH, tick), done)

    def finish_rows(ch):
        def done(i, j, y):
            idx = (slice(ch * RC + i * 128, ch * RC + (i + 1) * 128), slice(j * HD, (j + 1) * HD))
            xnew = xs[idx] + y
            out_ref[idx] = xnew.astype(BF16)
            xs[idx] = jnp.where(rep == 0, xnew, xin[idx].astype(F32))
        return done

    def memory_out(ch, p0, p1):
        def prod(i):
            acc = None
            for p in range(p0, p1):
                t = _dot(_unpack(oc[p, i, ch * 64:(ch + 1) * 64, :]), _unpack(wob[i, p * 64:(p + 1) * 64, :]))
                acc = t if acc is None else acc + t
                tick(t[:, 0:128])
                yield
            return acc
        return _block_matmul(prod, finish_rows(ch) if p1 == NPAIR else add_rows(ch))

    lane_head = lax.broadcasted_iota(jnp.int32, (1, 128), 1) // DH

    def head_queries(q, j):
        qh = [q[_tile(j), :] * jnp.where(lane_head == h, QSCALE, 0.0) for h in range(4)]
        return [(t[:64], t[64:]) for t in qh]

    def corner(q, k, j):
        qm = jnp.concatenate([hi for _, hi in head_queries(q, j)], axis=0)
        return _dot_nt(k[j * 128 + 64:(j + 1) * 128].astype(BF16), qm.astype(BF16))

    def scores(q, k, j, cor):
        nk = 128 * j + 64
        qm = jnp.concatenate([part for h, (lo, hi) in enumerate(head_queries(q, j))
                              for part in ((lo, hi) if h % 2 else (hi, lo))], axis=0)
        st = _dot_nt(k[0:nk].astype(BF16), qm.astype(BF16))
        for i in range(j + 1):
            tick(st[i * 128:i * 128 + 8, 0:128])
        diag = jnp.concatenate(
            [st[nk - 64:], jnp.concatenate([cor[:, _tile(h // 2)] for h in range(4)], axis=1)], axis=0)
        diag = diag + jnp.concatenate([cmask[...]] * 2, axis=1)
        return diag if j == 0 else jnp.concatenate([st[:nk - 64], diag], axis=0)

    def memory_read(g, q):
        zrow = lax.broadcasted_iota(jnp.int32, (16, 128), 0)
        zl = jnp.where(zrow == lane_head, jnp.broadcast_to(zs[rep * NT + g, 0:1, :], (16, 128)), 0.0)
        return _dot_nt(jnp.concatenate([mt[rep * NT + g], zl], axis=0).astype(BF16), _phi(q).astype(BF16))

    def memory_update(g, k, vt):
        pk = _phi(k)
        upd = functools.reduce(jnp.add, [
            _dot(_unpack(vt[:, _tile(i)]), pk[_tile(i)].astype(BF16)) for i in range(L // 128)])
        row_head = lax.broadcasted_iota(jnp.int32, (128, 128), 0) // DH
        mt[rep * NT + g] += jnp.where(row_head == lane_head, upd, 0.0)
        zs[rep * NT + g] += jnp.sum(pk, axis=0, keepdims=True)

    def attend(g, e, j, st, nd, vt):
        mx = jnp.broadcast_to(jnp.max(st, axis=0, keepdims=True), (8, 512))
        pv, l = [None] * 4, None
        for i in range(j + 1):
            mi = jnp.concatenate([after(len(ticks) - TUNE["gate"], mx[:, _tile(h)]) for h in range(4)], axis=1)
            p3 = jnp.exp2(st[_tile(i)].reshape(16, 8, 512) - mi)
            p = p3.reshape(128, 512)
            li = jnp.sum(p3, axis=0)
            l = li if i == 0 else l + li
            for h in range(4):
                t = _dot(_unpack(vt[h * 16:(h + 1) * 16, _tile(i)]), p[:, _tile(h)].astype(BF16))
                pv[h] = t if i == 0 else pv[h] + t
            if i < j:
                yield
        l = jnp.sum(l, axis=0, keepdims=True)
        rows = []
        for h in range(4):
            gh = gate[g * 4 + h][0:1, :]
            num = nd[h * DH:(h + 1) * DH, _tile(j)]
            den = nd[128 + h:129 + h, _tile(j)] + 1e-6
            loc = pv[h] * ((1.0 - gh) / l[:, _tile(h)])
            rows.append(num * (gh / den) + (loc if h % 2 else pltpu.roll(loc, 64, 1)))
        of[e, _tile(j), :] = jnp.concatenate(rows, axis=0).T
        yield

    def keep_output(p, ch):
        r0 = ch * RC
        blocks = _lhs_blocks(of[0, r0:r0 + 128, :], of[1, r0:r0 + 128, :],
                             of[0, r0 + 128:r0 + 256, :], of[1, r0 + 128:r0 + 256, :])
        for i, b in enumerate(blocks):
            oc[p, i, ch * 64:(ch + 1) * 64, :] = _pack(b)

    def memory_pair(p, last):
        del ticks[:]
        qs = [bq[e] for e in range(2)]
        ks = [bk[e] for e in range(2)]
        vts = [bv[e] for e in range(2)]
        if last:
            fill = _chain(memory_out(0, 0, p), memory_out(1, 0, TUNE["split"]))
            tail = memory_out(0, p, NPAIR)
        else:
            fill = _chain(memory_qk(p + 1, 0), memory_qk(p + 1, 1), memory_v(p + 1))
        for e, steps in enumerate(TUNE["plan_last" if last else "plan"].split("/")):
            g = 2 * p + e
            q, k, vt = qs[e], ks[e], vts[e]
            todo, cur, nd, seen, corners = [], None, None, [], {}
            for op in steps.split():
                if op == "f":
                    _run(fill, 1)
                elif op == "F":
                    _run(fill)
                elif op == "x":
                    _run(tail, 1)
                elif op == "X":
                    _run(tail)
                    xa[0:RC, :] = _layernorm(xs[0:RC, :])
                elif op[0] == "s":
                    j = int(op[1])
                    if j not in corners:
                        corners.update({i: corner(q, k, i) for i in (j, j ^ 1)})
                    todo.append((j, scores(q, k, j, corners[j])))
                elif op == "n":
                    nd = memory_read(g, q)
                elif op == "u":
                    memory_update(g, k, vt)
                elif op == "o":
                    keep_output(p, seen[-1] // 2)
                elif cur is None or next(cur, "end") == "end":
                    j, st = todo.pop(0)
                    seen.append(j)
                    cur = attend(g, e, j, st, nd, vt)
                    next(cur)
            assert len(seen) == L // 128 and next(cur, "end") == "end"
        return 0

    fetch_next = (rep == 1) & (seg < NSEG - 1)
    pl.when(fetch_next)(lambda: x_copy(seg + 1).start())

    def keys_stage():
        for c in range(NT):
            kb[c, 0:HALO, :] = kc[rep, c]
            vb[c, 0:HALO, :] = vc[rep, c]
        xn1 = _layernorm(xs[RC:L, :])
        xa[RC:L, :] = xn1
        in0, in1 = _row_blocks(xa[0:RC, :]), _row_blocks(xn1)
        _run(window_in(0, 0, held_for(in1, TUNE["due_norm"], in0)))
        _run(window_in(1, 0, lambda i: in1[i]))

    def window_stage():
        del ticks[:]
        a_in = [_row_blocks(xa[ch * RC:(ch + 1) * RC, :]) for ch in range(NCH)]
        due_probs, due_mix = iter(TUNE["due_probs"]), iter((0,) * (3 * NP) + TUNE["due_mix0"])
        seen = [0, 0]

        def held(ch, i):
            n, n2 = next(due_probs), next(due_mix)
            deps = [window_probs(*divmod(r, RC // 8))[1] for r in range(seen[0], seen[0] + n)]
            deps += [window_rows(0, r)[:, _tile(c)] for r in range(seen[1], seen[1] + n2) for c in range(NT)]
            seen[0] += n
            seen[1] += n2
            return before(deps, a_in[ch][i])
        for ch, m in ((0, 1), (1, 1), (0, 2), (1, 2)):
            _run(window_in(ch, m, functools.partial(held, ch)))
        o0, o1 = window_blocks(0), window_blocks(1)
        _run(window_out(0, held_for(o1, TUNE["due_mix1"], o0)))
        x0 = _row_blocks(_layernorm(xs[0:RC, :]))
        t0 = len(ticks)
        _run(window_out(1, held_for(x0, TUNE["due_norm0"], o1)))
        x1 = _row_blocks(_layernorm(xs[RC:L, :]))
        _run(memory_qk(0, 0, held_for(x1, TUNE["due_norm1"], x0)))
        t1 = len(ticks)
        _run(memory_qk(0, 1, lambda i: x1[i]))
        for ch, (blocks, t) in enumerate(((x0, t0), (x1, t1))):
            start, step = TUNE["keep"][ch]
            for i, blk in enumerate(blocks):
                dep = jnp.concatenate([jnp.concatenate([ticks[t + start + i * step]] * 4, axis=0)] * 4, axis=1)
                for r in range(0, 128, 32):
                    xb[i, ch * 64 + r // 2:ch * 64 + r // 2 + 16, :] = _pack(
                        jnp.where(never(32, 4), dep, blk[r:r + 32]))
        _run(memory_v(0))
        for c in range(NT):
            kc[rep, c] = kb[c, L:L + HALO, :]
            vc[rep, c] = vb[c, L:L + HALO, :]

    def last_stage():
        memory_pair(NPAIR - 1, True)
        _run(memory_out(1, TUNE["split"], NPAIR))

    keys_stage()
    pl.when(first_step)(_more_weights)
    window_stage()
    pl.when(first_step)(_last_weights)
    pl.when(fetch_next)(lambda: x_copy(seg + 1).wait())
    lax.fori_loop(0, NPAIR - 1, lambda p, carry: memory_pair(p, False), 0)
    last_stage()


@jax.jit
def pallas_interleave_layers__sliding_local_dilated__memory_aug_infini_attn__prompt_kernel(
        A_x, A_wqkv, A_wo, B_x, B_wq, B_wk, B_wv, B_wo, B_beta):
    del B_x
    hbm = pl.BlockSpec(memory_space=pl.ANY)
    out = pl.pallas_call(
        _kernel,
        grid=(NSEG, 2),
        in_specs=[hbm, pl.BlockSpec((1, H), lambda s, r: (0, 0)), hbm, hbm, hbm, hbm, hbm, hbm],
        out_specs=pl.BlockSpec((L, D), lambda s, r: (s, 0)),
        out_shape=jax.ShapeDtypeStruct((S, D), BF16),
        scratch_shapes=[
            pltpu.VMEM((L, D), BF16),
            pltpu.VMEM((6, D, HD), BF16),
            pltpu.VMEM((2, HD, D), BF16),
            pltpu.VMEM((3, NPAIR, D, 256), BF16),
            pltpu.VMEM((D, D), BF16),
            pltpu.VMEM((3, NP, NPAIR, WROWS, 128), U32),
            pltpu.VMEM((NP, NPAIR, WROWS, 128), U32),
            pltpu.VMEM((NPAIR, NP, HD // 2, 256), U32),
            pltpu.VMEM((NPAIR, NP, 64, HD), U32),
            pltpu.VMEM((NP, HD // 2, HD), U32),
            pltpu.VMEM((L, D), F32),
            pltpu.VMEM((L, D), F32),
            pltpu.VMEM((NP, L // 4, HD), U32),
            pltpu.VMEM((NT, L, 128), F32),
            pltpu.VMEM((NT, HALO + L, 128), F32),
            pltpu.VMEM((NT, HALO + L, 128), F32),
            pltpu.VMEM((2, NT, HALO, 128), F32),
            pltpu.VMEM((2, NT, HALO, 128), F32),
            pltpu.VMEM((2, L, 128), F32),
            pltpu.VMEM((NPAIR, NP, L // 4, 128), U32),
            pltpu.VMEM((2, L, 128), F32),
            pltpu.VMEM((2, L, 128), F32),
            pltpu.VMEM((2, 64, L), U32),
            pltpu.VMEM((2 * NT, 128, 128), F32),
            pltpu.VMEM((2 * NT, 8, 128), F32),
            pltpu.VMEM((H, 8, 128), F32),
            pltpu.VMEM((128, 256), F32),
            pltpu.SemaphoreType.DMA((22,)),
        ],
        compiler_params=pltpu.CompilerParams(
            dimension_semantics=("arbitrary", "arbitrary"),
            vmem_limit_bytes=110 * 2**20),
        name="interleave",
    )(A_x.reshape(S, D), B_beta.reshape(1, H), A_wqkv, A_wo, B_wq, B_wk, B_wv, B_wo)
    return out.reshape(1, S, D)
```

```python
import functools
import math

import jax
import jax.numpy as jnp
from jax import lax
from jax.experimental import pallas as pl
from jax.experimental.pallas import tpu as pltpu

S, D, H, DH = 2048, 1024, 32, 32
NSEG = 4
L = S // NSEG
W, DIL = 8, 2
HALO = 16
NT = D // 128
NPAIR = NT // 2
HD = D // 2
RC = 256
NCH = L // RC
NP = 7
PITCH = 17
WROWS = 16 * PITCH + 16
LOG2E = math.log2(math.e)
QSCALE = DH ** -0.5 * LOG2E
NEG = -1e9 * LOG2E
F32, BF16, U32 = jnp.float32, jnp.bfloat16, jnp.uint32

TUNE = dict(
    pace=((24, 1.05, 80, 0.75), (52, 1.1, 108, 0.1)),
    due_norm=(0, 2, 2, 3, 3, 3, 3),
    due_probs=(0, 0, 0, 0, 0, 0, 0, 0, 3, 4, 4, 4, 4, 4, 4, 4, 4, 4, 4, 4, 4, 4, 3, 3, 3, 0, 0, 0),
    due_mix0=(0, 0, 2, 6, 7, 6, 9),
    due_mix1=(0, 0, 3, 3, 4, 2, 3),
    due_norm0=(0, 1, 2, 2, 3, 3, 5),
    due_norm1=(0, 0, 2, 1, 4, 4, 2),
    keep=((10, 2), (0, 1)),
    split=2,
    plan="f s3 f f s2 f n p3 f p3 f p3 f f p3 s1 p3 f f p3 f s0 p3 f f p3 f f p4 f u f f p3 "
         "/ f s3 s2 n f p3 f p3 f p3 f f p4 f f s1 p3 f p3 f p3 o s0 f f p3 f p3 f u f p3 o F",
    plan_last="f s0 s1 n p4 s2 f p3 f p3 s3 f p3 f p3 f p2 f p3 f p3 f p3 f f p3 f u "
              "/ s0 s1 f n f p3 s2 p3 f p3 o s3 f p4 f p3 p2 f x f p3 x p3 f f x p4 x p3 o f x f x u F X",
)


def _dot(a, b):
    return jnp.dot(a, b, preferred_element_type=F32)


def _dot_nt(a, b):
    return lax.dot_general(a, b, (((1,), (1,)), ((), ())), preferred_element_type=F32)


def _pack(x):
    return pltpu.bitcast(x.astype(BF16), U32)


def _unpack(x):
    return pltpu.bitcast(x, BF16)


def _tile(i):
    return slice(i * 128, (i + 1) * 128)


def _lhs_blocks(a11, a12, a21, a22):
    return [a11 + a22, a21 + a22, a11, a22, a11 + a12, a21 - a11, a12 - a22]


def _rhs_blocks(b11, b12, b21, b22):
    return [b11 + b22, b11, b12 - b22, b21 - b11, b22, b11 + b12, b21 + b22]


def _row_blocks(x):
    return _lhs_blocks(x[:128, :HD], x[:128, HD:], x[128:, :HD], x[128:, HD:])


def _block_matmul(prod, done):
    p3 = yield from prod(2)
    p5 = yield from prod(4)
    done(0, 1, p3 + p5)
    p2 = yield from prod(1)
    p4 = yield from prod(3)
    done(1, 0, p2 + p4)
    u, v = p4 - p5, p3 - p2
    p1 = yield from prod(0)
    u, v = u + p1, v + p1
    p7 = yield from prod(6)
    done(0, 0, u + p7)
    p6 = yield from prod(5)
    done(1, 1, v + p6)


def _whole(fn):
    def prod(i):
        y = fn(i)
        yield
        return y
    return prod


def _tiled(dot, nk, nn, tick):
    def prod(i):
        acc = [None] * nn
        for n in range(nn):
            for k in range(nk):
                t = dot(i, k, n)
                acc[n] = t if k == 0 else acc[n] + t
            tick(t)
            yield
        return jnp.concatenate(acc, axis=1)
    return prod


def _run(gen, n=None):
    k = 0
    while (n is None or k < n) and next(gen, "end") != "end":
        k += 1


def _chain(*gens):
    for g in gens:
        yield from g


def _layernorm(x):
    m = jnp.mean(x, axis=-1, keepdims=True)
    xc = x - m
    v = jnp.mean(xc * xc, axis=-1, keepdims=True)
    return xc * lax.rsqrt(v + 1e-5)


def _phi(t):
    return jnp.where(t > 0, t + 1.0, jnp.exp(t))


def _kernel(x_hbm, beta_ref, wqkv_hbm, woa_hbm, wq_hbm, wk_hbm, wv_hbm, wob_hbm, out_hbm,
            xin, xout, raw_a, raw_ao, raw_b, raw_bo, wa, woa, wqk, wvt, wob,
            xs, xa, xb, qb, kb, vb, kc, vc, of, oc, bq, bk, bv, mt, zs, gate, cmask, sems):
    seg = pl.program_id(0)
    rep = pl.program_id(1)
    first_step = (seg == 0) & (rep == 0)

    def window_copy(i):
        m, j = divmod(i, 2)
        if m < 3:
            c0 = (1, 0, 2)[m] * D + j * HD
            return pltpu.make_async_copy(wqkv_hbm.at[:, pl.ds(c0, HD)], raw_a.at[i], sems.at[i])
        return pltpu.make_async_copy(woa_hbm.at[pl.ds(j * HD, HD)], raw_ao.at[j], sems.at[i])

    def pair_copies(p):
        return [pltpu.make_async_copy(w.at[:, pl.ds(p * 256, 256)], raw_b.at[m, p], sems.at[8 + 3 * p + m])
                for m, w in enumerate((wq_hbm, wk_hbm, wv_hbm))]

    def late_copies():
        return ([c for p in range(1, NPAIR) for c in pair_copies(p)]
                + [pltpu.make_async_copy(wob_hbm, raw_bo, sems.at[20])])

    def x_copy(s):
        return pltpu.make_async_copy(x_hbm.at[pl.ds(pl.multiple_of(s * L, L), L)], xin, sems.at[21])

    def out_copy(s, ch, i, j):
        rows = pl.ds(pl.multiple_of(s * L + ch * RC + i * 128, 128), 128)
        n = ch * 4 + i * 2 + j
        return pltpu.make_async_copy(xout.at[n], out_hbm.at[rows, pl.ds(j * HD, HD)], sems.at[22 + n])

    def wait_out(s):
        for n in range(4 * NCH):
            out_copy(s, n // 4, n // 2 % 2, n % 2).wait()

    def selector(reorder):
        row = lax.broadcasted_iota(jnp.int32, (128, 128), 0)
        col = lax.broadcasted_iota(jnp.int32, (128, 128), 1)
        if reorder:
            row = (((row >> 5) & 1) * 2 + (row & 1)) * DH + (row >> 6) * 16 + ((row >> 1) & 15)
        return jnp.where(row == col, 1.0, 0.0).astype(BF16)

    def packed_blocks(*quad):
        quad = [pltpu.bitcast(b, U32) for b in quad]
        vals = [_unpack(b).astype(F32) for b in quad]
        out = []
        for blk in _rhs_blocks(*vals):
            same = [i for i, v in enumerate(vals) if v is blk]
            out.append(quad[same[0]] if same else _pack(blk))
        return out

    def arrive(piece, lo, hi):
        for i in range(lo, hi):
            @pl.when(piece == i)
            def _():
                window_copy(i).wait()
                for n in {0: (1,), 1: (2, 3, 4, 5)}.get(i, ()):
                    window_copy(n).start()

    def scatter(dst, t, blocks):
        for i, v in enumerate(blocks):
            v = _pack(v)
            for c in range(NPAIR):
                for hp in range(2):
                    dst(i, c)[pl.ds(t * 2 + hp, 16, stride=PITCH), :] = v[hp * 16:(hp + 1) * 16, _tile(c)]

    def prep_window_in(piece, carry):
        arrive(piece, 0, 6)
        for t in range(4):
            top = _dot_nt(selector(True), raw_a[piece, 0:HD, _tile(t)])
            bot = _dot_nt(selector(True), raw_a[piece, HD:D, _tile(t)])
            scatter(lambda i, c: wa.at[piece // 2, i, c], (piece % 2) * 4 + t,
                    _rhs_blocks(top[:64], top[64:], bot[:64], bot[64:]))
        return carry

    def prep_window_out(j, carry):
        arrive(6 + j, 6, 8)
        for t in range(4):
            y = _dot(selector(True), raw_ao[j, _tile(t), :])
            scatter(lambda i, c: woa.at[i, c], j * 4 + t,
                    _rhs_blocks(y[:64, :HD], y[:64, HD:], y[64:, :HD], y[64:, HD:]))
        return carry

    def prep_pair(t, carry):
        p = t // 2
        for jj in range(2):
            j = (t % 2) * 2 + jj
            top = pl.ds(pl.multiple_of(j * 128, 128), 128)
            bot = pl.ds(pl.multiple_of(HD + j * 128, 128), 128)
            y = _dot_nt(selector(False), jnp.concatenate(
                [raw_b[2, p, rows, _tile(e)] for rows in (top, bot) for e in range(2)], axis=0))
            for i, v in enumerate(_rhs_blocks(*[y[:, _tile(c)] for c in range(4)])):
                wvt[p, i, :, top] = _pack(v)
            for m in range(2):
                quad = [raw_b[m, p, rows, _tile(e)] for rows in (top, bot) for e in range(2)]
                for i, v in enumerate(packed_blocks(*quad)):
                    wqk[p, i, pl.ds(pl.multiple_of(j * 64, 64), 64), _tile(m)] = v
        return carry

    def prep_memory_out(t, carry):
        r0 = (t // 2) * 256 + (t % 2) * 64
        quad = [raw_bo[pl.ds(pl.multiple_of(r0 + e * 128, 64), 64), c:c + HD] for e in range(2) for c in (0, HD)]
        for i, v in enumerate(packed_blocks(*quad)):
            wob[i, pl.ds(pl.multiple_of(t * 32, 32), 32), :] = v
        return carry

    @pl.when(first_step)
    def _start():
        window_copy(0).start()
        x_copy(0).start()
        kc[...] = jnp.zeros(kc.shape, F32)
        vc[...] = jnp.zeros(vc.shape, F32)
        mt[...] = jnp.zeros(mt.shape, F32)
        zs[...] = jnp.zeros(zs.shape, F32)
        g_all = jax.nn.sigmoid(beta_ref[...].astype(F32))
        head = lax.broadcasted_iota(jnp.int32, (1, H), 1)
        for h in range(H):
            gate[h] = jnp.broadcast_to(jnp.sum(jnp.where(head == h, g_all, 0.0), axis=1, keepdims=True), (8, 128))
        kk = lax.broadcasted_iota(jnp.int32, (128, 256), 0)
        qq = lax.broadcasted_iota(jnp.int32, (128, 256), 1)
        qq = jnp.where(qq < 128, qq ^ 64, qq - 128)
        cmask[...] = jnp.where(qq < kk, NEG, 0.0).astype(F32)
        prep_window_in(0, 0)
        x_copy(0).wait()

        def load_rows(j, carry):
            rows = pl.ds(pl.multiple_of(j * 64, 64), 64)
            later = pl.ds(pl.multiple_of(RC + j * 64, 64), 64)
            x0 = xin[rows, :].astype(F32)
            xs[rows, :] = x0
            xa[rows, :] = _layernorm(x0)
            xs[later, :] = xin[later, :].astype(F32)
            return carry
        lax.fori_loop(0, RC // 64, load_rows, 0)
        prep_window_in(1, 0)

    def _more_weights():
        for c in [window_copy(6), window_copy(7)] + pair_copies(0):
            c.start()
        lax.fori_loop(2, 6, prep_window_in, 0)
        lax.fori_loop(0, 2, prep_window_out, 0)
        for c in late_copies():
            c.start()
        for c in pair_copies(0):
            c.wait()
        lax.fori_loop(0, 2, prep_pair, 0)

    def _last_weights():
        for c in late_copies():
            c.wait()
        lax.fori_loop(2, NT, prep_pair, 0)
        lax.fori_loop(0, 8, prep_memory_out, 0)

    ticks = []

    def tick(y):
        ticks.extend(y[0:8, c:c + 128] for c in range(0, y.shape[1], 128))
        return y

    def never(rows, tiles=1):
        return jnp.concatenate([cmask[0:rows, 0:128]] * tiles, axis=1) > 1.0

    def after(t, x):
        return x if t < 0 else jnp.where(never(8), ticks[min(t, len(ticks) - 1)], x)

    def before(deps, a):
        if not deps:
            return a
        head = jnp.where(never(8), functools.reduce(jnp.maximum, deps), a[0:8, 0:128])
        return jnp.concatenate([jnp.concatenate([head, a[0:8, 128:]], axis=1), a[8:]], axis=0)

    def held_for(blocks, counts, lhs):
        counts, seen = iter(counts), [0]

        def held(i):
            n = next(counts)
            deps = [b[r * 8:r * 8 + 8, _tile(c)] for r in range(seen[0], seen[0] + n)
                    for b in blocks[-2:] for c in range(NPAIR)]
            seen[0] += n
            return before(deps, lhs[i])
        return held

    def reordered(ref):
        return _unpack(jnp.concatenate([jnp.concatenate(
            [ref[c, d * PITCH:d * PITCH + 16, :] for d in range(16)], axis=0) for c in range(NPAIR)], axis=1))

    def window_in(ch, m, lhs):
        dst, off = ((kb, HALO), (qb, 0), (vb, HALO))[m]

        def done(i, j, y):
            r0 = off + ch * RC + i * 128
            if m == 1:
                y = y * QSCALE
            for c in range(NPAIR):
                dst[j * NPAIR + c, r0:r0 + 128, :] = y[:, _tile(c)]
        return _block_matmul(
            _whole(lambda i: tick(_dot_nt(lhs(i).astype(BF16), reordered(wa.at[m, i])))), done)

    def taps(ref, c, r0, w):
        o0 = HALO + r0 - DIL * w
        return ref[c, o0:o0 + 8, :]

    def row_group(i):
        return i // 2 + (i % 2) * (RC // 16)

    @functools.cache
    def window_probs(ch, i):
        r0 = ch * RC + row_group(i) * 8
        t = int(TUNE["pace"][ch][0] + i * TUNE["pace"][ch][1])
        qs = [after(t, qb[c, r0:r0 + 8, :]) for c in range(NT)]
        logits = []
        for w in range(W):
            acc = functools.reduce(jnp.add, [qs[c] * taps(kb, c, r0, w) for c in range(NT)])
            acc = acc + pltpu.roll(acc, 64, 1)
            acc = acc + pltpu.roll(acc, 32, 1)
            if r0 < DIL * w:
                pos = seg * L + r0 + lax.broadcasted_iota(jnp.int32, (8, 128), 0)
                acc = jnp.where(pos >= DIL * w, acc, NEG)
            logits.append(acc)
        mx = functools.reduce(jnp.maximum, logits)
        es = [jnp.exp2(v - mx) for v in logits]
        return es, 1.0 / functools.reduce(jnp.add, es)

    @functools.cache
    def window_rows(ch, i):
        r0 = ch * RC + row_group(i) * 8
        es, inv = window_probs(ch, i)
        inv = after(int(TUNE["pace"][ch][2] + i * TUNE["pace"][ch][3]), inv)
        ps = [e * inv for e in es]
        return jnp.concatenate(
            [functools.reduce(jnp.add, [ps[w] * taps(vb, c, r0, w) for w in range(W)]) for c in range(NT)], axis=1)

    def window_blocks(ch):
        rows = [None] * (RC // 8)
        for i in range(RC // 8):
            rows[row_group(i)] = window_rows(ch, i)
        return _row_blocks(jnp.concatenate(rows, axis=0))

    def add_rows(ch):
        def done(i, j, y):
            r0 = ch * RC + i * 128
            xs[r0:r0 + 128, j * HD:(j + 1) * HD] += y
        return done

    def window_out(ch, lhs):
        return _block_matmul(
            _whole(lambda i: tick(_dot(lhs(i).astype(BF16), reordered(woa.at[i])))), add_rows(ch))

    def memory_qk(p, ch, lhs=None):
        def done(i, j, y):
            r0 = ch * RC + i * 128
            bq[j, r0:r0 + 128, :] = y[:, :128]
            bk[j, r0:r0 + 128, :] = y[:, 128:]
        if lhs is not None:
            return _block_matmul(_whole(lambda i: tick(_dot(lhs(i).astype(BF16), _unpack(wqk[p, i])))), done)
        return _block_matmul(_tiled(
            lambda i, k, n: _dot(_unpack(xb[i, ch * 64:(ch + 1) * 64, _tile(k)]),
                                 _unpack(wqk[p, i, k * 64:(k + 1) * 64, _tile(n)])), 4, 2, tick), done)

    def memory_v(p):
        def done(i, j, y):
            for ch in range(NCH):
                c0 = ch * RC + i * 128
                bv[j, :, c0:c0 + 128] = _pack(y[:, _tile(ch)])
        return _block_matmul(_tiled(
            lambda i, k, n: _dot_nt(_unpack(wvt[p, i, :, _tile(k)]),
                                    _unpack(xb[i, n * 64:(n + 1) * 64, _tile(k)])), 4, NCH, tick), done)

    def finish_rows(ch):
        def done(i, j, y):
            idx = (slice(ch * RC + i * 128, ch * RC + (i + 1) * 128), slice(j * HD, (j + 1) * HD))
            xnew = xs[idx] + y
            xout[ch * 4 + i * 2 + j] = xnew.astype(BF16)
            out_copy(seg, ch, i, j).start()
            xs[idx] = jnp.where(rep == 0, xnew, xin[idx].astype(F32))
        return done

    def memory_out(ch, p0, p1):
        def prod(i):
            acc = None
            for p in range(p0, p1):
                t = _dot(_unpack(oc[p, i, ch * 64:(ch + 1) * 64, :]), _unpack(wob[i, p * 64:(p + 1) * 64, :]))
                acc = t if acc is None else acc + t
                tick(t[:, 0:128])
                yield
            return acc
        return _block_matmul(prod, finish_rows(ch) if p1 == NPAIR else add_rows(ch))

    lane_head = lax.broadcasted_iota(jnp.int32, (1, 128), 1) // DH

    def head_queries(q, j):
        qh = [q[_tile(j), :] * jnp.where(lane_head == h, QSCALE, 0.0) for h in range(4)]
        return [(t[:64], t[64:]) for t in qh]

    def corner(q, k, j):
        qm = jnp.concatenate([hi for _, hi in head_queries(q, j)], axis=0)
        return _dot_nt(k[j * 128 + 64:(j + 1) * 128].astype(BF16), qm.astype(BF16))

    def scores(q, k, j, cor):
        nk = 128 * j + 64
        qm = jnp.concatenate([part for h, (lo, hi) in enumerate(head_queries(q, j))
                              for part in ((lo, hi) if h % 2 else (hi, lo))], axis=0)
        st = _dot_nt(k[0:nk].astype(BF16), qm.astype(BF16))
        for i in range(j + 1):
            tick(st[i * 128:i * 128 + 8, 0:128])
        diag = jnp.concatenate(
            [st[nk - 64:], jnp.concatenate([cor[:, _tile(h // 2)] for h in range(4)], axis=1)], axis=0)
        diag = diag + jnp.concatenate([cmask[...]] * 2, axis=1)
        return diag if j == 0 else jnp.concatenate([st[:nk - 64], diag], axis=0)

    def memory_read(g, q):
        zrow = lax.broadcasted_iota(jnp.int32, (16, 128), 0)
        zl = jnp.where(zrow == lane_head, jnp.broadcast_to(zs[rep * NT + g, 0:1, :], (16, 128)), 0.0)
        return _dot_nt(jnp.concatenate([mt[rep * NT + g], zl], axis=0).astype(BF16), _phi(q).astype(BF16))

    def memory_update(g, k, vt):
        pk = _phi(k)
        upd = functools.reduce(jnp.add, [
            _dot(_unpack(vt[:, _tile(i)]), pk[_tile(i)].astype(BF16)) for i in range(L // 128)])
        row_head = lax.broadcasted_iota(jnp.int32, (128, 128), 0) // DH
        mt[rep * NT + g] += jnp.where(row_head == lane_head, upd, 0.0)
        zs[rep * NT + g] += jnp.sum(pk, axis=0, keepdims=True)

    def attend(g, e, j, st, nd, vt, lag):
        mx = jnp.broadcast_to(jnp.max(st, axis=0, keepdims=True), (8, 512))
        pv, l = [None] * 4, None
        for i in range(j + 1):
            mi = jnp.concatenate([after(len(ticks) - lag[0], mx[:, _tile(h)]) for h in range(4)], axis=1)
            p3 = jnp.exp2(st[_tile(i)].reshape(16, 8, 512) - mi)
            p = p3.reshape(128, 512)
            li = jnp.sum(p3, axis=0)
            l = li if i == 0 else l + li
            for h in range(4):
                t = _dot(_unpack(vt[h * 16:(h + 1) * 16, _tile(i)]), p[:, _tile(h)].astype(BF16))
                pv[h] = t if i == 0 else pv[h] + t
            if i < j:
                yield
        l = jnp.sum(l, axis=0, keepdims=True)
        rows = []
        for h in range(4):
            gh = gate[g * 4 + h][0:1, :]
            num = nd[h * DH:(h + 1) * DH, _tile(j)]
            den = nd[128 + h:129 + h, _tile(j)] + 1e-6
            loc = pv[h] * ((1.0 - gh) / l[:, _tile(h)])
            rows.append(num * (gh / den) + (loc if h % 2 else pltpu.roll(loc, 64, 1)))
        of[e, _tile(j), :] = jnp.concatenate(rows, axis=0).T
        yield

    def keep_output(p, ch):
        r0 = ch * RC
        blocks = _lhs_blocks(of[0, r0:r0 + 128, :], of[1, r0:r0 + 128, :],
                             of[0, r0 + 128:r0 + 256, :], of[1, r0 + 128:r0 + 256, :])
        for i, b in enumerate(blocks):
            oc[p, i, ch * 64:(ch + 1) * 64, :] = _pack(b)

    def memory_pair(p, last):
        del ticks[:]
        qs = [bq[e] for e in range(2)]
        ks = [bk[e] for e in range(2)]
        vts = [bv[e] for e in range(2)]
        if last:
            fill = _chain(memory_out(0, 0, p), memory_out(1, 0, TUNE["split"]))
            tail = memory_out(0, p, NPAIR)
        else:
            fill = _chain(memory_qk(p + 1, 0), memory_qk(p + 1, 1), memory_v(p + 1))
        for e, steps in enumerate(TUNE["plan_last" if last else "plan"].split("/")):
            g = 2 * p + e
            q, k, vt = qs[e], ks[e], vts[e]
            todo, cur, nd, seen, corners, lag = [], None, None, [], {}, [0]
            for op in steps.split():
                if op == "f":
                    _run(fill, 1)
                elif op == "F":
                    _run(fill)
                elif op == "x":
                    _run(tail, 1)
                elif op == "X":
                    _run(tail)
                    xa[0:RC, :] = _layernorm(xs[0:RC, :])
                elif op[0] == "s":
                    j = int(op[1])
                    if j not in corners:
                        corners.update({i: corner(q, k, i) for i in (j, j ^ 1)})
                    todo.append((j, scores(q, k, j, corners[j])))
                elif op == "n":
                    nd = memory_read(g, q)
                elif op == "u":
                    memory_update(g, k, vt)
                elif op == "o":
                    keep_output(p, seen[-1] // 2)
                else:
                    lag[0] = int(op[1])
                    if cur is None or next(cur, "end") == "end":
                        j, st = todo.pop(0)
                        seen.append(j)
                        cur = attend(g, e, j, st, nd, vt, lag)
                        next(cur)
            assert len(seen) == L // 128 and next(cur, "end") == "end"
        return 0

    fetch_next = (rep == 1) & (seg < NSEG - 1)
    pl.when(fetch_next)(lambda: x_copy(seg + 1).start())

    def keys_stage():
        for c in range(NT):
            kb[c, 0:HALO, :] = kc[rep, c]
            vb[c, 0:HALO, :] = vc[rep, c]
        xn1 = _layernorm(xs[RC:L, :])
        xa[RC:L, :] = xn1
        in0, in1 = _row_blocks(xa[0:RC, :]), _row_blocks(xn1)
        _run(window_in(0, 0, held_for(in1, TUNE["due_norm"], in0)))
        _run(window_in(1, 0, lambda i: in1[i]))

    def window_stage():
        del ticks[:]
        a_in = [_row_blocks(xa[ch * RC:(ch + 1) * RC, :]) for ch in range(NCH)]
        due_probs, due_mix = iter(TUNE["due_probs"]), iter((0,) * (3 * NP) + TUNE["due_mix0"])
        seen = [0, 0]

        def held(ch, i):
            n, n2 = next(due_probs), next(due_mix)
            deps = [window_probs(*divmod(r, RC // 8))[1] for r in range(seen[0], seen[0] + n)]
            deps += [window_rows(0, r)[:, _tile(c)] for r in range(seen[1], seen[1] + n2) for c in range(NT)]
            seen[0] += n
            seen[1] += n2
            return before(deps, a_in[ch][i])
        for ch, m in ((0, 1), (1, 1), (0, 2), (1, 2)):
            _run(window_in(ch, m, functools.partial(held, ch)))
        o0, o1 = window_blocks(0), window_blocks(1)
        _run(window_out(0, held_for(o1, TUNE["due_mix1"], o0)))
        x0 = _row_blocks(_layernorm(xs[0:RC, :]))
        t0 = len(ticks)
        _run(window_out(1, held_for(x0, TUNE["due_norm0"], o1)))
        x1 = _row_blocks(_layernorm(xs[RC:L, :]))
        _run(memory_qk(0, 0, held_for(x1, TUNE["due_norm1"], x0)))
        t1 = len(ticks)
        _run(memory_qk(0, 1, lambda i: x1[i]))
        for ch, (blocks, t) in enumerate(((x0, t0), (x1, t1))):
            start, step = TUNE["keep"][ch]
            for i, blk in enumerate(blocks):
                dep = jnp.concatenate([jnp.concatenate([ticks[t + start + i * step]] * 4, axis=0)] * 4, axis=1)
                for r in range(0, 128, 32):
                    xb[i, ch * 64 + r // 2:ch * 64 + r // 2 + 16, :] = _pack(
                        jnp.where(never(32, 4), dep, blk[r:r + 32]))
        _run(memory_v(0))
        for c in range(NT):
            kc[rep, c] = kb[c, L:L + HALO, :]
            vc[rep, c] = vb[c, L:L + HALO, :]

    def last_stage():
        memory_pair(NPAIR - 1, True)
        _run(memory_out(1, TUNE["split"], NPAIR))

    keys_stage()
    pl.when(first_step)(_more_weights)
    window_stage()
    pl.when(first_step)(_last_weights)
    pl.when(jnp.logical_not(first_step))(lambda: wait_out(seg - 1 + rep))
    pl.when(fetch_next)(lambda: x_copy(seg + 1).wait())
    lax.fori_loop(0, NPAIR - 1, lambda p, carry: memory_pair(p, False), 0)
    last_stage()
    pl.when((seg == NSEG - 1) & (rep == 1))(lambda: wait_out(seg))


@jax.jit
def pallas_interleave_layers__sliding_local_dilated__memory_aug_infini_attn__prompt_kernel(
        A_x, A_wqkv, A_wo, B_x, B_wq, B_wk, B_wv, B_wo, B_beta):
    del B_x
    hbm = pl.BlockSpec(memory_space=pl.ANY)
    out = pl.pallas_call(
        _kernel,
        grid=(NSEG, 2),
        in_specs=[hbm, pl.BlockSpec((1, H), lambda s, r: (0, 0)), hbm, hbm, hbm, hbm, hbm, hbm],
        out_specs=hbm,
        out_shape=jax.ShapeDtypeStruct((S, D), BF16),
        scratch_shapes=[
            pltpu.VMEM((L, D), BF16),
            pltpu.VMEM((4 * NCH, 128, HD), BF16),
            pltpu.VMEM((6, D, HD), BF16),
            pltpu.VMEM((2, HD, D), BF16),
            pltpu.VMEM((3, NPAIR, D, 256), BF16),
            pltpu.VMEM((D, D), BF16),
            pltpu.VMEM((3, NP, NPAIR, WROWS, 128), U32),
            pltpu.VMEM((NP, NPAIR, WROWS, 128), U32),
            pltpu.VMEM((NPAIR, NP, HD // 2, 256), U32),
            pltpu.VMEM((NPAIR, NP, 64, HD), U32),
            pltpu.VMEM((NP, HD // 2, HD), U32),
            pltpu.VMEM((L, D), F32),
            pltpu.VMEM((L, D), F32),
            pltpu.VMEM((NP, L // 4, HD), U32),
            pltpu.VMEM((NT, L, 128), F32),
            pltpu.VMEM((NT, HALO + L, 128), F32),
            pltpu.VMEM((NT, HALO + L, 128), F32),
            pltpu.VMEM((2, NT, HALO, 128), F32),
            pltpu.VMEM((2, NT, HALO, 128), F32),
            pltpu.VMEM((2, L, 128), F32),
            pltpu.VMEM((NPAIR, NP, L // 4, 128), U32),
            pltpu.VMEM((2, L, 128), F32),
            pltpu.VMEM((2, L, 128), F32),
            pltpu.VMEM((2, 64, L), U32),
            pltpu.VMEM((2 * NT, 128, 128), F32),
            pltpu.VMEM((2 * NT, 8, 128), F32),
            pltpu.VMEM((H, 8, 128), F32),
            pltpu.VMEM((128, 256), F32),
            pltpu.SemaphoreType.DMA((30,)),
        ],
        compiler_params=pltpu.CompilerParams(
            dimension_semantics=("arbitrary", "arbitrary"),
            vmem_limit_bytes=110 * 2**20),
        name="interleave",
    )(A_x.reshape(S, D), B_beta.reshape(1, H), A_wqkv, A_wo, B_wq, B_wk, B_wv, B_wo)
    return out.reshape(1, S, D)
```

```python
import functools
import math

import jax
import jax.numpy as jnp
from jax import lax
from jax.experimental import pallas as pl
from jax.experimental.pallas import tpu as pltpu

S, D, H, DH = 2048, 1024, 32, 32
NSEG = 4
L = S // NSEG
W, DIL = 8, 2
HALO = 16
NT = D // 128
NPAIR = NT // 2
HD = D // 2
RC = 256
NCH = L // RC
NP = 7
PITCH = 17
WROWS = 16 * PITCH + 16
LOG2E = math.log2(math.e)
QSCALE = DH ** -0.5 * LOG2E
NEG = -1e9 * LOG2E
F32, BF16, U32 = jnp.float32, jnp.bfloat16, jnp.uint32

TUNE = dict(
    pace=((24, 1.05, 80, 0.75), (56, 1.1, 108, 0.1)),
    due_norm=(0, 2, 2, 3, 3, 3, 3),
    due_probs=(0, 0, 0, 0, 0, 0, 0, 0, 3, 3, 4, 5, 4, 4, 4, 4, 4, 4, 4, 4, 4, 4, 3, 3, 3, 0, 0, 0),
    due_mix0=(0, 1, 2, 5, 7, 6, 9),
    due_mix1=(0, 0, 3, 3, 1, 5, 3),
    due_norm0=(0, 1, 2, 2, 3, 3, 5),
    due_norm1=(0, 0, 2, 1, 4, 4, 2),
    keep=((10, 2), (0, 1)),
    split=2,
    plan="f s3 f f s2 f n p3 f p3 f p3 f f p3 s1 p3 f f p3 f s0 p3 f f p3 f f p4 f u f f p3 "
         "/ f s3 s2 n f p3 f p3 f p3 f f p4 f f s1 p3 f p3 f p3 o s0 f f p3 f p3 f u f p3 o F",
    plan_last="f s0 s1 n p4 s2 f p3 f p3 s3 f p3 f p3 f p2 f p3 f p3 f p3 f f p3 f u "
              "/ s0 s1 f n f p3 s2 p3 f p3 o s3 f p4 f p3 p2 f x f p3 x p3 f f x p4 x p3 o f x f x u F X",
)


def _dot(a, b):
    return jnp.dot(a, b, preferred_element_type=F32)


def _dot_nt(a, b):
    return lax.dot_general(a, b, (((1,), (1,)), ((), ())), preferred_element_type=F32)


def _pack(x):
    return pltpu.bitcast(x.astype(BF16), U32)


def _unpack(x):
    return pltpu.bitcast(x, BF16)


def _tile(i):
    return slice(i * 128, (i + 1) * 128)


def _lhs_blocks(a11, a12, a21, a22):
    return [a11 + a22, a21 + a22, a11, a22, a11 + a12, a21 - a11, a12 - a22]


def _rhs_blocks(b11, b12, b21, b22):
    return [b11 + b22, b11, b12 - b22, b21 - b11, b22, b11 + b12, b21 + b22]


def _row_blocks(x):
    return _lhs_blocks(x[:128, :HD], x[:128, HD:], x[128:, :HD], x[128:, HD:])


def _block_matmul(prod, done):
    p3 = yield from prod(2)
    p5 = yield from prod(4)
    done(0, 1, p3 + p5)
    p2 = yield from prod(1)
    p4 = yield from prod(3)
    done(1, 0, p2 + p4)
    u, v = p4 - p5, p3 - p2
    p1 = yield from prod(0)
    u, v = u + p1, v + p1
    p7 = yield from prod(6)
    done(0, 0, u + p7)
    p6 = yield from prod(5)
    done(1, 1, v + p6)


def _whole(fn):
    def prod(i):
        y = fn(i)
        yield
        return y
    return prod


def _tiled(dot, nk, nn, tick):
    def prod(i):
        acc = [None] * nn
        for n in range(nn):
            for k in range(nk):
                t = dot(i, k, n)
                acc[n] = t if k == 0 else acc[n] + t
            tick(t)
            yield
        return jnp.concatenate(acc, axis=1)
    return prod


def _run(gen, n=None):
    k = 0
    while (n is None or k < n) and next(gen, "end") != "end":
        k += 1


def _chain(*gens):
    for g in gens:
        yield from g


def _layernorm(x):
    m = jnp.mean(x, axis=-1, keepdims=True)
    xc = x - m
    v = jnp.mean(xc * xc, axis=-1, keepdims=True)
    return xc * lax.rsqrt(v + 1e-5)


def _phi(t):
    return jnp.where(t > 0, t + 1.0, jnp.exp(t))


def _kernel(x_hbm, beta_ref, wqkv_hbm, woa_hbm, wq_hbm, wk_hbm, wv_hbm, wob_hbm, out_hbm,
            xin, xout, raw_a, raw_ao, raw_b, raw_bo, wa, woa, wqk, wvt, wob,
            xs, xa, xb, qb, kb, vb, kc, vc, of, oc, bq, bk, bv, mt, zs, gate, cmask, sems):
    seg = pl.program_id(0)
    rep = pl.program_id(1)
    first_step = (seg == 0) & (rep == 0)

    def window_copy(i):
        m, j = divmod(i, 2)
        if m < 3:
            c0 = (1, 0, 2)[m] * D + j * HD
            return pltpu.make_async_copy(wqkv_hbm.at[:, pl.ds(c0, HD)], raw_a.at[i], sems.at[i])
        return pltpu.make_async_copy(woa_hbm.at[pl.ds(j * HD, HD)], raw_ao.at[j], sems.at[i])

    def pair_copies(p):
        return [pltpu.make_async_copy(w.at[:, pl.ds(p * 256, 256)], raw_b.at[m, p], sems.at[8 + 3 * p + m])
                for m, w in enumerate((wq_hbm, wk_hbm, wv_hbm))]

    def late_copies():
        return ([c for p in range(1, NPAIR) for c in pair_copies(p)]
                + [pltpu.make_async_copy(wob_hbm, raw_bo, sems.at[20])])

    def x_copy(s):
        return pltpu.make_async_copy(x_hbm.at[pl.ds(pl.multiple_of(s * L, L), L)], xin, sems.at[21])

    def out_copy(s, ch, i, j):
        rows = pl.ds(pl.multiple_of(s * L + ch * RC + i * 128, 128), 128)
        n = ch * 4 + i * 2 + j
        return pltpu.make_async_copy(xout.at[n], out_hbm.at[rows, pl.ds(j * HD, HD)], sems.at[22 + n])

    def wait_out(s):
        for n in range(4 * NCH):
            out_copy(s, n // 4, n // 2 % 2, n % 2).wait()

    def selector(reorder):
        row = lax.broadcasted_iota(jnp.int32, (128, 128), 0)
        col = lax.broadcasted_iota(jnp.int32, (128, 128), 1)
        if reorder:
            row = (((row >> 5) & 1) * 2 + (row & 1)) * DH + (row >> 6) * 16 + ((row >> 1) & 15)
        return jnp.where(row == col, 1.0, 0.0).astype(BF16)

    def packed_blocks(*quad):
        quad = [pltpu.bitcast(b, U32) for b in quad]
        vals = [_unpack(b).astype(F32) for b in quad]
        out = []
        for blk in _rhs_blocks(*vals):
            same = [i for i, v in enumerate(vals) if v is blk]
            out.append(quad[same[0]] if same else _pack(blk))
        return out

    def arrive(piece, lo, hi):
        for i in range(lo, hi):
            @pl.when(piece == i)
            def _():
                window_copy(i).wait()
                for n in {0: (1,), 1: (2, 3, 4, 5)}.get(i, ()):
                    window_copy(n).start()

    def scatter(dst, t, blocks):
        for i, v in enumerate(blocks):
            v = _pack(v)
            for c in range(NPAIR):
                for hp in range(2):
                    dst(i, c)[pl.ds(t * 2 + hp, 16, stride=PITCH), :] = v[hp * 16:(hp + 1) * 16, _tile(c)]

    def prep_window_in(piece, carry):
        arrive(piece, 0, 6)
        for t in range(4):
            top = _dot_nt(selector(True), raw_a[piece, 0:HD, _tile(t)])
            bot = _dot_nt(selector(True), raw_a[piece, HD:D, _tile(t)])
            scatter(lambda i, c: wa.at[piece // 2, i, c], (piece % 2) * 4 + t,
                    _rhs_blocks(top[:64], top[64:], bot[:64], bot[64:]))
        return carry

    def prep_window_out(j, carry):
        arrive(6 + j, 6, 8)
        for t in range(4):
            y = _dot(selector(True), raw_ao[j, _tile(t), :])
            scatter(lambda i, c: woa.at[i, c], j * 4 + t,
                    _rhs_blocks(y[:64, :HD], y[:64, HD:], y[64:, :HD], y[64:, HD:]))
        return carry

    def prep_pair(p, carry):
        quad = [_dot_nt(selector(False), raw_b[2, p, kh * HD:(kh + 1) * HD, _tile(e)])
                for kh in range(2) for e in range(2)]
        for i, v in enumerate(_rhs_blocks(*quad)):
            wvt[p, i] = _pack(v)

        def rows_qk(j, c):
            for m in range(2):
                quad = [raw_b[m, p, pl.ds(pl.multiple_of(kh * HD + j * 64, 64), 64), _tile(e)]
                        for kh in range(2) for e in range(2)]
                for i, v in enumerate(packed_blocks(*quad)):
                    wqk[p, i, pl.ds(pl.multiple_of(j * 32, 32), 32), _tile(m)] = v
            return c
        return lax.fori_loop(0, HD // 64, rows_qk, carry)

    def prep_memory_out(t, carry):
        r0 = (t // 4) * 256 + (t % 4) * 32
        quad = [raw_bo[pl.ds(pl.multiple_of(r0 + e * 128, 32), 32), c:c + HD] for e in range(2) for c in (0, HD)]
        for i, v in enumerate(packed_blocks(*quad)):
            wob[i, pl.ds(pl.multiple_of(t * 16, 16), 16), :] = v
        return carry

    @pl.when(first_step)
    def _start():
        window_copy(0).start()
        x_copy(0).start()
        kc[...] = jnp.zeros(kc.shape, F32)
        vc[...] = jnp.zeros(vc.shape, F32)
        mt[...] = jnp.zeros(mt.shape, F32)
        zs[...] = jnp.zeros(zs.shape, F32)
        g_all = jax.nn.sigmoid(beta_ref[...].astype(F32))
        head = lax.broadcasted_iota(jnp.int32, (1, H), 1)
        for h in range(H):
            gate[h] = jnp.broadcast_to(jnp.sum(jnp.where(head == h, g_all, 0.0), axis=1, keepdims=True), (8, 128))
        kk = lax.broadcasted_iota(jnp.int32, (128, 256), 0)
        qq = lax.broadcasted_iota(jnp.int32, (128, 256), 1)
        qq = jnp.where(qq < 128, qq ^ 64, qq - 128)
        cmask[...] = jnp.where(qq < kk, NEG, 0.0).astype(F32)
        prep_window_in(0, 0)
        x_copy(0).wait()

        def load_rows(j, carry):
            rows = pl.ds(pl.multiple_of(j * 64, 64), 64)
            later = pl.ds(pl.multiple_of(RC + j * 64, 64), 64)
            x0 = xin[rows, :].astype(F32)
            xs[rows, :] = x0
            xa[rows, :] = _layernorm(x0)
            xs[later, :] = xin[later, :].astype(F32)
            return carry
        lax.fori_loop(0, RC // 64, load_rows, 0)
        prep_window_in(1, 0)

    def _more_weights():
        for c in [window_copy(6), window_copy(7)] + pair_copies(0):
            c.start()
        lax.fori_loop(2, 6, prep_window_in, 0)
        lax.fori_loop(0, 2, prep_window_out, 0)
        for c in late_copies():
            c.start()
        for c in pair_copies(0):
            c.wait()
        prep_pair(0, 0)

    def _last_weights():
        for c in late_copies():
            c.wait()
        lax.fori_loop(1, NPAIR, prep_pair, 0)
        lax.fori_loop(0, HD // 32, prep_memory_out, 0)

    ticks = []

    def tick(y):
        ticks.extend(y[0:8, c:c + 128] for c in range(0, y.shape[1], 128))
        return y

    def never(rows, tiles=1):
        return jnp.concatenate([cmask[0:rows, 0:128]] * tiles, axis=1) > 1.0

    def after(t, x):
        return x if t < 0 else jnp.where(never(8), ticks[min(t, len(ticks) - 1)], x)

    def before(deps, a):
        if not deps:
            return a
        head = jnp.where(never(8), functools.reduce(jnp.maximum, deps), a[0:8, 0:128])
        return jnp.concatenate([jnp.concatenate([head, a[0:8, 128:]], axis=1), a[8:]], axis=0)

    def held_for(blocks, counts, lhs):
        counts, seen = iter(counts), [0]

        def held(i):
            n = next(counts)
            deps = [b[r * 8:r * 8 + 8, _tile(c)] for r in range(seen[0], seen[0] + n)
                    for b in blocks[-2:] for c in range(NPAIR)]
            seen[0] += n
            return before(deps, lhs[i])
        return held

    def reordered(ref):
        return _unpack(jnp.concatenate([jnp.concatenate(
            [ref[c, d * PITCH:d * PITCH + 16, :] for d in range(16)], axis=0) for c in range(NPAIR)], axis=1))

    def window_in(ch, m, lhs):
        dst, off = ((kb, HALO), (qb, 0), (vb, HALO))[m]

        def done(i, j, y):
            r0 = off + ch * RC + i * 128
            if m == 1:
                y = y * QSCALE
            for c in range(NPAIR):
                dst[j * NPAIR + c, r0:r0 + 128, :] = y[:, _tile(c)]
        return _block_matmul(
            _whole(lambda i: tick(_dot_nt(lhs(i).astype(BF16), reordered(wa.at[m, i])))), done)

    def taps(ref, c, r0, w):
        o0 = HALO + r0 - DIL * w
        return ref[c, o0:o0 + 8, :]

    def row_group(i):
        return i // 2 + (i % 2) * (RC // 16)

    @functools.cache
    def window_probs(ch, i):
        r0 = ch * RC + row_group(i) * 8
        t = int(TUNE["pace"][ch][0] + i * TUNE["pace"][ch][1])
        qs = [after(t, qb[c, r0:r0 + 8, :]) for c in range(NT)]
        logits = []
        for w in range(W):
            acc = functools.reduce(jnp.add, [qs[c] * taps(kb, c, r0, w) for c in range(NT)])
            acc = acc + pltpu.roll(acc, 64, 1)
            acc = acc + pltpu.roll(acc, 32, 1)
            if r0 < DIL * w:
                pos = seg * L + r0 + lax.broadcasted_iota(jnp.int32, (8, 128), 0)
                acc = jnp.where(pos >= DIL * w, acc, NEG)
            logits.append(acc)
        mx = functools.reduce(jnp.maximum, logits)
        es = [jnp.exp2(v - mx) for v in logits]
        return es, 1.0 / functools.reduce(jnp.add, es)

    @functools.cache
    def window_rows(ch, i):
        r0 = ch * RC + row_group(i) * 8
        es, inv = window_probs(ch, i)
        inv = after(int(TUNE["pace"][ch][2] + i * TUNE["pace"][ch][3]), inv)
        ps = [e * inv for e in es]
        return jnp.concatenate(
            [functools.reduce(jnp.add, [ps[w] * taps(vb, c, r0, w) for w in range(W)]) for c in range(NT)], axis=1)

    def window_blocks(ch):
        rows = [None] * (RC // 8)
        for i in range(RC // 8):
            rows[row_group(i)] = window_rows(ch, i)
        return _row_blocks(jnp.concatenate(rows, axis=0))

    def add_rows(ch):
        def done(i, j, y):
            r0 = ch * RC + i * 128
            xs[r0:r0 + 128, j * HD:(j + 1) * HD] += y
        return done

    def window_out(ch, lhs):
        return _block_matmul(
            _whole(lambda i: tick(_dot(lhs(i).astype(BF16), reordered(woa.at[i])))), add_rows(ch))

    def memory_qk(p, ch, lhs=None):
        def done(i, j, y):
            r0 = ch * RC + i * 128
            bq[j, r0:r0 + 128, :] = y[:, :128]
            bk[j, r0:r0 + 128, :] = y[:, 128:]
        if lhs is not None:
            return _block_matmul(_whole(lambda i: tick(_dot(lhs(i).astype(BF16), _unpack(wqk[p, i])))), done)
        return _block_matmul(_tiled(
            lambda i, k, n: _dot(_unpack(xb[i, ch * 64:(ch + 1) * 64, _tile(k)]),
                                 _unpack(wqk[p, i, k * 64:(k + 1) * 64, _tile(n)])), 4, 2, tick), done)

    def memory_v(p):
        def done(i, j, y):
            for ch in range(NCH):
                c0 = ch * RC + i * 128
                bv[j, :, c0:c0 + 128] = _pack(y[:, _tile(ch)])
        return _block_matmul(_tiled(
            lambda i, k, n: _dot_nt(_unpack(wvt[p, i, :, _tile(k)]),
                                    _unpack(xb[i, n * 64:(n + 1) * 64, _tile(k)])), 4, NCH, tick), done)

    def finish_rows(ch):
        def done(i, j, y):
            idx = (slice(ch * RC + i * 128, ch * RC + (i + 1) * 128), slice(j * HD, (j + 1) * HD))
            xnew = xs[idx] + y
            xout[ch * 4 + i * 2 + j] = xnew.astype(BF16)
            out_copy(seg, ch, i, j).start()
            xs[idx] = jnp.where(rep == 0, xnew, xin[idx].astype(F32))
        return done

    def memory_out(ch, p0, p1):
        def prod(i):
            acc = None
            for p in range(p0, p1):
                t = _dot(_unpack(oc[p, i, ch * 64:(ch + 1) * 64, :]), _unpack(wob[i, p * 64:(p + 1) * 64, :]))
                acc = t if acc is None else acc + t
                tick(t[:, 0:128])
                yield
            return acc
        return _block_matmul(prod, finish_rows(ch) if p1 == NPAIR else add_rows(ch))

    lane_head = lax.broadcasted_iota(jnp.int32, (1, 128), 1) // DH

    def head_queries(q, j):
        qh = [q[_tile(j), :] * jnp.where(lane_head == h, QSCALE, 0.0) for h in range(4)]
        return [(t[:64], t[64:]) for t in qh]

    def corner(q, k, j):
        qm = jnp.concatenate([hi for _, hi in head_queries(q, j)], axis=0)
        return _dot_nt(k[j * 128 + 64:(j + 1) * 128].astype(BF16), qm.astype(BF16))

    def scores(q, k, j, cor):
        nk = 128 * j + 64
        qm = jnp.concatenate([part for h, (lo, hi) in enumerate(head_queries(q, j))
                              for part in ((lo, hi) if h % 2 else (hi, lo))], axis=0)
        st = _dot_nt(k[0:nk].astype(BF16), qm.astype(BF16))
        for i in range(j + 1):
            tick(st[i * 128:i * 128 + 8, 0:128])
        diag = jnp.concatenate(
            [st[nk - 64:], jnp.concatenate([cor[:, _tile(h // 2)] for h in range(4)], axis=1)], axis=0)
        diag = diag + jnp.concatenate([cmask[...]] * 2, axis=1)
        return diag if j == 0 else jnp.concatenate([st[:nk - 64], diag], axis=0)

    def memory_read(g, q):
        zrow = lax.broadcasted_iota(jnp.int32, (16, 128), 0)
        zl = jnp.where(zrow == lane_head, jnp.broadcast_to(zs[rep * NT + g, 0:1, :], (16, 128)), 0.0)
        return _dot_nt(jnp.concatenate([mt[rep * NT + g], zl], axis=0).astype(BF16), _phi(q).astype(BF16))

    def memory_update(g, k, vt):
        pk = _phi(k)
        upd = functools.reduce(jnp.add, [
            _dot(_unpack(vt[:, _tile(i)]), pk[_tile(i)].astype(BF16)) for i in range(L // 128)])
        row_head = lax.broadcasted_iota(jnp.int32, (128, 128), 0) // DH
        mt[rep * NT + g] += jnp.where(row_head == lane_head, upd, 0.0)
        zs[rep * NT + g] += jnp.sum(pk, axis=0, keepdims=True)

    def attend(g, e, j, st, nd, vt, lag):
        mx = jnp.broadcast_to(jnp.max(st, axis=0, keepdims=True), (8, 512))
        pv, l = [None] * 4, None
        for i in range(j + 1):
            mi = jnp.concatenate([after(len(ticks) - lag[0], mx[:, _tile(h)]) for h in range(4)], axis=1)
            p3 = jnp.exp2(st[_tile(i)].reshape(16, 8, 512) - mi)
            p = p3.reshape(128, 512)
            li = jnp.sum(p3, axis=0)
            l = li if i == 0 else l + li
            for h in range(4):
                t = _dot(_unpack(vt[h * 16:(h + 1) * 16, _tile(i)]), p[:, _tile(h)].astype(BF16))
                pv[h] = t if i == 0 else pv[h] + t
            if i < j:
                yield
        l = jnp.sum(l, axis=0, keepdims=True)
        rows = []
        for h in range(4):
            gh = gate[g * 4 + h][0:1, :]
            num = nd[h * DH:(h + 1) * DH, _tile(j)]
            den = nd[128 + h:129 + h, _tile(j)] + 1e-6
            loc = pv[h] * ((1.0 - gh) / l[:, _tile(h)])
            rows.append(num * (gh / den) + (loc if h % 2 else pltpu.roll(loc, 64, 1)))
        of[e, _tile(j), :] = jnp.concatenate(rows, axis=0).T
        yield

    def keep_output(p, ch):
        r0 = ch * RC
        blocks = _lhs_blocks(of[0, r0:r0 + 128, :], of[1, r0:r0 + 128, :],
                             of[0, r0 + 128:r0 + 256, :], of[1, r0 + 128:r0 + 256, :])
        for i, b in enumerate(blocks):
            oc[p, i, ch * 64:(ch + 1) * 64, :] = _pack(b)

    def memory_pair(p, last):
        del ticks[:]
        qs = [bq[e] for e in range(2)]
        ks = [bk[e] for e in range(2)]
        vts = [bv[e] for e in range(2)]
        if last:
            fill = _chain(memory_out(0, 0, p), memory_out(1, 0, TUNE["split"]))
            tail = memory_out(0, p, NPAIR)
        else:
            fill = _chain(memory_qk(p + 1, 0), memory_qk(p + 1, 1), memory_v(p + 1))
        for e, steps in enumerate(TUNE["plan_last" if last else "plan"].split("/")):
            g = 2 * p + e
            q, k, vt = qs[e], ks[e], vts[e]
            todo, cur, nd, seen, corners, lag = [], None, None, [], {}, [0]
            for op in steps.split():
                if op == "f":
                    _run(fill, 1)
                elif op == "F":
                    _run(fill)
                elif op == "x":
                    _run(tail, 1)
                elif op == "X":
                    _run(tail)
                    xa[0:RC, :] = _layernorm(xs[0:RC, :])
                elif op[0] == "s":
                    j = int(op[1])
                    if j not in corners:
                        corners.update({i: corner(q, k, i) for i in (j, j ^ 1)})
                    todo.append((j, scores(q, k, j, corners[j])))
                elif op == "n":
                    nd = memory_read(g, q)
                elif op == "u":
                    memory_update(g, k, vt)
                elif op == "o":
                    keep_output(p, seen[-1] // 2)
                else:
                    lag[0] = int(op[1])
                    if cur is None or next(cur, "end") == "end":
                        j, st = todo.pop(0)
                        seen.append(j)
                        cur = attend(g, e, j, st, nd, vt, lag)
                        next(cur)
            assert len(seen) == L // 128 and next(cur, "end") == "end"
        return 0

    fetch_next = (rep == 1) & (seg < NSEG - 1)
    pl.when(fetch_next)(lambda: x_copy(seg + 1).start())

    def keys_stage():
        for c in range(NT):
            kb[c, 0:HALO, :] = kc[rep, c]
            vb[c, 0:HALO, :] = vc[rep, c]
        xn1 = _layernorm(xs[RC:L, :])
        xa[RC:L, :] = xn1
        in0, in1 = _row_blocks(xa[0:RC, :]), _row_blocks(xn1)
        _run(window_in(0, 0, held_for(in1, TUNE["due_norm"], in0)))
        _run(window_in(1, 0, lambda i: in1[i]))

    def window_stage():
        del ticks[:]
        a_in = [_row_blocks(xa[ch * RC:(ch + 1) * RC, :]) for ch in range(NCH)]
        due_probs, due_mix = iter(TUNE["due_probs"]), iter((0,) * (3 * NP) + TUNE["due_mix0"])
        seen = [0, 0]

        def held(ch, i):
            n, n2 = next(due_probs), next(due_mix)
            deps = [window_probs(*divmod(r, RC // 8))[1] for r in range(seen[0], seen[0] + n)]
            deps += [window_rows(0, r)[:, _tile(c)] for r in range(seen[1], seen[1] + n2) for c in range(NT)]
            seen[0] += n
            seen[1] += n2
            return before(deps, a_in[ch][i])
        for ch, m in ((0, 1), (1, 1), (0, 2), (1, 2)):
            _run(window_in(ch, m, functools.partial(held, ch)))
        o0, o1 = window_blocks(0), window_blocks(1)
        _run(window_out(0, held_for(o1, TUNE["due_mix1"], o0)))
        x0 = _row_blocks(_layernorm(xs[0:RC, :]))
        t0 = len(ticks)
        _run(window_out(1, held_for(x0, TUNE["due_norm0"], o1)))
        x1 = _row_blocks(_layernorm(xs[RC:L, :]))
        _run(memory_qk(0, 0, held_for(x1, TUNE["due_norm1"], x0)))
        t1 = len(ticks)
        _run(memory_qk(0, 1, lambda i: x1[i]))
        for ch, (blocks, t) in enumerate(((x0, t0), (x1, t1))):
            start, step = TUNE["keep"][ch]
            for i, blk in enumerate(blocks):
                dep = jnp.concatenate([jnp.concatenate([ticks[t + start + i * step]] * 4, axis=0)] * 4, axis=1)
                for r in range(0, 128, 32):
                    xb[i, ch * 64 + r // 2:ch * 64 + r // 2 + 16, :] = _pack(
                        jnp.where(never(32, 4), dep, blk[r:r + 32]))
        _run(memory_v(0))
        for c in range(NT):
            kc[rep, c] = kb[c, L:L + HALO, :]
            vc[rep, c] = vb[c, L:L + HALO, :]

    def last_stage():
        memory_pair(NPAIR - 1, True)
        _run(memory_out(1, TUNE["split"], NPAIR))

    keys_stage()
    pl.when(first_step)(_more_weights)
    window_stage()
    pl.when(first_step)(_last_weights)
    pl.when(jnp.logical_not(first_step))(lambda: wait_out(seg - 1 + rep))
    pl.when(fetch_next)(lambda: x_copy(seg + 1).wait())
    lax.fori_loop(0, NPAIR - 1, lambda p, carry: memory_pair(p, False), 0)
    last_stage()
    pl.when((seg == NSEG - 1) & (rep == 1))(lambda: wait_out(seg))


@jax.jit
def pallas_interleave_layers__sliding_local_dilated__memory_aug_infini_attn__prompt_kernel(
        A_x, A_wqkv, A_wo, B_x, B_wq, B_wk, B_wv, B_wo, B_beta):
    del B_x
    hbm = pl.BlockSpec(memory_space=pl.ANY)
    out = pl.pallas_call(
        _kernel,
        grid=(NSEG, 2),
        in_specs=[hbm, pl.BlockSpec((1, H), lambda s, r: (0, 0)), hbm, hbm, hbm, hbm, hbm, hbm],
        out_specs=hbm,
        out_shape=jax.ShapeDtypeStruct((S, D), BF16),
        scratch_shapes=[
            pltpu.VMEM((L, D), BF16),
            pltpu.VMEM((4 * NCH, 128, HD), BF16),
            pltpu.VMEM((6, D, HD), BF16),
            pltpu.VMEM((2, HD, D), BF16),
            pltpu.VMEM((3, NPAIR, D, 256), BF16),
            pltpu.VMEM((D, D), BF16),
            pltpu.VMEM((3, NP, NPAIR, WROWS, 128), U32),
            pltpu.VMEM((NP, NPAIR, WROWS, 128), U32),
            pltpu.VMEM((NPAIR, NP, HD // 2, 256), U32),
            pltpu.VMEM((NPAIR, NP, 64, HD), U32),
            pltpu.VMEM((NP, HD // 2, HD), U32),
            pltpu.VMEM((L, D), F32),
            pltpu.VMEM((L, D), F32),
            pltpu.VMEM((NP, L // 4, HD), U32),
            pltpu.VMEM((NT, L, 128), F32),
            pltpu.VMEM((NT, HALO + L, 128), F32),
            pltpu.VMEM((NT, HALO + L, 128), F32),
            pltpu.VMEM((2, NT, HALO, 128), F32),
            pltpu.VMEM((2, NT, HALO, 128), F32),
            pltpu.VMEM((2, L, 128), F32),
            pltpu.VMEM((NPAIR, NP, L // 4, 128), U32),
            pltpu.VMEM((2, L, 128), F32),
            pltpu.VMEM((2, L, 128), F32),
            pltpu.VMEM((2, 64, L), U32),
            pltpu.VMEM((2 * NT, 128, 128), F32),
            pltpu.VMEM((2 * NT, 8, 128), F32),
            pltpu.VMEM((H, 8, 128), F32),
            pltpu.VMEM((128, 256), F32),
            pltpu.SemaphoreType.DMA((30,)),
        ],
        compiler_params=pltpu.CompilerParams(
            dimension_semantics=("arbitrary", "arbitrary"),
            vmem_limit_bytes=110 * 2**20),
        name="interleave",
    )(A_x.reshape(S, D), B_beta.reshape(1, H), A_wqkv, A_wo, B_wq, B_wk, B_wv, B_wo)
    return out.reshape(1, S, D)
```

```python
import functools
import math

import jax
import jax.numpy as jnp
from jax import lax
from jax.experimental import pallas as pl
from jax.experimental.pallas import tpu as pltpu

S, D, H, DH = 2048, 1024, 32, 32
NSEG = 4
L = S // NSEG
W, DIL = 8, 2
HALO = 16
NT = D // 128
NPAIR = NT // 2
HD = D // 2
RC = 256
NCH = L // RC
NP = 7
PITCH = 17
WROWS = 16 * PITCH + 16
LOG2E = math.log2(math.e)
QSCALE = DH ** -0.5 * LOG2E
NEG = -1e9 * LOG2E
F32, BF16, U32 = jnp.float32, jnp.bfloat16, jnp.uint32

TUNE = dict(
    pace=((24, 1.05, 80, 0.75), (56, 1.1, 108, 0.1)),
    due_norm=(0, 2, 3, 4, 2, 2, 3),
    due_probs=(0, 0, 0, 0, 0, 0, 0, 0, 3, 3, 4, 5, 4, 4, 4, 4, 4, 4, 4, 4, 4, 4, 3, 3, 3, 0, 0, 0),
    due_mix0=(0, 1, 2, 5, 7, 6, 9),
    due_mix1=(0, 0, 3, 3, 1, 5, 3),
    due_norm0=(0, 1, 2, 2, 3, 3, 5),
    due_norm1=(0, 0, 2, 1, 4, 4, 2),
    due_next=(0, 0, 1, 5, 1, 2, 10, 1, 2, 2, 0, 5, 3, 0),
    keep=((10, 2), (0, 1)),
    split=2,
    plan="f f s3 f s2 f n f p3 f p3 f p3 f f p3 s1 p3 f f p3 f s0 p3 f f p3 f f p4 f u f f p3 "
         "/ f s3 s2 n f p3 f p2 f p3 f f p4 f f s1 p3 f p3 f p2 o s0 f p3 f f p3 u f p2 f o F",
    plan_last="f s0 s1 n p4 s2 f p3 f p3 s3 f p3 f p3 p2 f f p3 f p3 f p3 f f p4 f u "
              "/ s0 s1 f n f p3 s2 p3 f p3 o s3 f p4 f p3 p2 f x f p3 x p3 f f x p4 x p3 o f x f x u F X",
)


def _dot(a, b):
    return jnp.dot(a, b, preferred_element_type=F32)


def _dot_nt(a, b):
    return lax.dot_general(a, b, (((1,), (1,)), ((), ())), preferred_element_type=F32)


def _pack(x):
    return pltpu.bitcast(x.astype(BF16), U32)


def _unpack(x):
    return pltpu.bitcast(x, BF16)


def _tile(i):
    return slice(i * 128, (i + 1) * 128)


def _lhs_blocks(a11, a12, a21, a22):
    return [a11 + a22, a21 + a22, a11, a22, a11 + a12, a21 - a11, a12 - a22]


def _rhs_blocks(b11, b12, b21, b22):
    return [b11 + b22, b11, b12 - b22, b21 - b11, b22, b11 + b12, b21 + b22]


def _row_blocks(x):
    return _lhs_blocks(x[:128, :HD], x[:128, HD:], x[128:, :HD], x[128:, HD:])


def _block_matmul(prod, done):
    p3 = yield from prod(2)
    p5 = yield from prod(4)
    done(0, 1, p3 + p5)
    p2 = yield from prod(1)
    p4 = yield from prod(3)
    done(1, 0, p2 + p4)
    u, v = p4 - p5, p3 - p2
    p1 = yield from prod(0)
    u, v = u + p1, v + p1
    p7 = yield from prod(6)
    done(0, 0, u + p7)
    p6 = yield from prod(5)
    done(1, 1, v + p6)


def _whole(fn):
    def prod(i):
        y = fn(i)
        yield
        return y
    return prod


def _tiled(dot, nk, nn, tick):
    def prod(i):
        acc = [None] * nn
        for n in range(nn):
            for k in range(nk):
                t = dot(i, k, n)
                acc[n] = t if k == 0 else acc[n] + t
            tick(t)
            yield
        return jnp.concatenate(acc, axis=1)
    return prod


def _run(gen, n=None):
    k = 0
    while (n is None or k < n) and next(gen, "end") != "end":
        k += 1


def _chain(*gens):
    for g in gens:
        yield from g


def _layernorm(x):
    m = jnp.mean(x, axis=-1, keepdims=True)
    xc = x - m
    v = jnp.mean(xc * xc, axis=-1, keepdims=True)
    return xc * lax.rsqrt(v + 1e-5)


def _phi(t):
    return jnp.where(t > 0, t + 1.0, jnp.exp(t))


def _kernel(x_hbm, beta_ref, wqkv_hbm, woa_hbm, wq_hbm, wk_hbm, wv_hbm, wob_hbm, out_hbm,
            xin, xout, raw_a, raw_ao, raw_b, raw_bo, wa, woa, wqk, wvt, wob,
            xs, xa, xb, qb, kb, vb, kc, vc, of, oc, bq, bk, bv, mt, zs, gate, cmask, sems):
    seg = pl.program_id(0)
    rep = pl.program_id(1)
    first_step = (seg == 0) & (rep == 0)

    def window_copy(i):
        m, j = divmod(i, 2)
        if m < 3:
            c0 = (1, 0, 2)[m] * D + j * HD
            return pltpu.make_async_copy(wqkv_hbm.at[:, pl.ds(c0, HD)], raw_a.at[i], sems.at[i])
        return pltpu.make_async_copy(woa_hbm.at[pl.ds(j * HD, HD)], raw_ao.at[j], sems.at[i])

    def pair_copies(p):
        return [pltpu.make_async_copy(w.at[:, pl.ds(p * 256, 256)], raw_b.at[m, p], sems.at[8 + 3 * p + m])
                for m, w in enumerate((wq_hbm, wk_hbm, wv_hbm))]

    def late_copies():
        return ([c for p in range(1, NPAIR) for c in pair_copies(p)]
                + [pltpu.make_async_copy(wob_hbm, raw_bo, sems.at[20])])

    def x_copy(s):
        return pltpu.make_async_copy(x_hbm.at[pl.ds(pl.multiple_of(s * L, L), L)], xin, sems.at[21])

    def out_copy(s, ch, i, j):
        rows = pl.ds(pl.multiple_of(s * L + ch * RC + i * 128, 128), 128)
        n = ch * 4 + i * 2 + j
        return pltpu.make_async_copy(xout.at[n], out_hbm.at[rows, pl.ds(j * HD, HD)], sems.at[22 + n])

    def wait_out(s):
        for n in range(4 * NCH):
            out_copy(s, n // 4, n // 2 % 2, n % 2).wait()

    def selector(reorder):
        row = lax.broadcasted_iota(jnp.int32, (128, 128), 0)
        col = lax.broadcasted_iota(jnp.int32, (128, 128), 1)
        if reorder:
            row = (((row >> 5) & 1) * 2 + (row & 1)) * DH + (row >> 6) * 16 + ((row >> 1) & 15)
        return jnp.where(row == col, 1.0, 0.0).astype(BF16)

    def packed_blocks(*quad):
        quad = [pltpu.bitcast(b, U32) for b in quad]
        vals = [_unpack(b).astype(F32) for b in quad]
        out = []
        for blk in _rhs_blocks(*vals):
            same = [i for i, v in enumerate(vals) if v is blk]
            out.append(quad[same[0]] if same else _pack(blk))
        return out

    def arrive(piece, lo, hi):
        for i in range(lo, hi):
            @pl.when(piece == i)
            def _():
                window_copy(i).wait()
                for n in {0: (1,), 1: (2, 3, 4, 5)}.get(i, ()):
                    window_copy(n).start()

    def scatter(dst, t, blocks):
        for i, v in enumerate(blocks):
            v = _pack(v)
            for c in range(NPAIR):
                for hp in range(2):
                    dst(i, c)[pl.ds(t * 2 + hp, 16, stride=PITCH), :] = v[hp * 16:(hp + 1) * 16, _tile(c)]

    def prep_window_in(piece, carry):
        arrive(piece, 0, 6)
        for t in range(4):
            top = _dot_nt(selector(True), raw_a[piece, 0:HD, _tile(t)])
            bot = _dot_nt(selector(True), raw_a[piece, HD:D, _tile(t)])
            scatter(lambda i, c: wa.at[piece // 2, i, c], (piece % 2) * 4 + t,
                    _rhs_blocks(top[:64], top[64:], bot[:64], bot[64:]))
        return carry

    def prep_window_out(j, carry):
        arrive(6 + j, 6, 8)
        for t in range(4):
            y = _dot(selector(True), raw_ao[j, _tile(t), :])
            scatter(lambda i, c: woa.at[i, c], j * 4 + t,
                    _rhs_blocks(y[:64, :HD], y[:64, HD:], y[64:, :HD], y[64:, HD:]))
        return carry

    def prep_pair(p, carry):
        quad = [_dot_nt(selector(False), raw_b[2, p, kh * HD:(kh + 1) * HD, _tile(e)])
                for kh in range(2) for e in range(2)]
        for i, v in enumerate(_rhs_blocks(*quad)):
            wvt[p, i] = _pack(v)

        def rows_qk(j, c):
            for m in range(2):
                quad = [raw_b[m, p, pl.ds(pl.multiple_of(kh * HD + j * 64, 64), 64), _tile(e)]
                        for kh in range(2) for e in range(2)]
                for i, v in enumerate(packed_blocks(*quad)):
                    wqk[p, i, pl.ds(pl.multiple_of(j * 32, 32), 32), _tile(m)] = v
            return c
        return lax.fori_loop(0, HD // 64, rows_qk, carry)

    def prep_memory_out(t, carry):
        r0 = (t // 4) * 256 + (t % 4) * 32
        quad = [raw_bo[pl.ds(pl.multiple_of(r0 + e * 128, 32), 32), c:c + HD] for e in range(2) for c in (0, HD)]
        for i, v in enumerate(packed_blocks(*quad)):
            wob[i, pl.ds(pl.multiple_of(t * 16, 16), 16), :] = v
        return carry

    @pl.when(first_step)
    def _start():
        window_copy(0).start()
        x_copy(0).start()
        kc[...] = jnp.zeros(kc.shape, F32)
        vc[...] = jnp.zeros(vc.shape, F32)
        mt[...] = jnp.zeros(mt.shape, F32)
        zs[...] = jnp.zeros(zs.shape, F32)
        g_all = jax.nn.sigmoid(beta_ref[...].astype(F32))
        head = lax.broadcasted_iota(jnp.int32, (1, H), 1)
        for h in range(H):
            gate[h] = jnp.broadcast_to(jnp.sum(jnp.where(head == h, g_all, 0.0), axis=1, keepdims=True), (8, 128))
        kk = lax.broadcasted_iota(jnp.int32, (128, 256), 0)
        qq = lax.broadcasted_iota(jnp.int32, (128, 256), 1)
        qq = jnp.where(qq < 128, qq ^ 64, qq - 128)
        cmask[...] = jnp.where(qq < kk, NEG, 0.0).astype(F32)
        prep_window_in(0, 0)
        x_copy(0).wait()

        def load_rows(j, carry):
            rows = pl.ds(pl.multiple_of(j * 64, 64), 64)
            later = pl.ds(pl.multiple_of(RC + j * 64, 64), 64)
            x0 = xin[rows, :].astype(F32)
            xs[rows, :] = x0
            xa[rows, :] = _layernorm(x0)
            xs[later, :] = xin[later, :].astype(F32)
            return carry
        lax.fori_loop(0, RC // 64, load_rows, 0)
        prep_window_in(1, 0)

    def _more_weights():
        for c in [window_copy(6), window_copy(7)] + pair_copies(0):
            c.start()
        lax.fori_loop(2, 6, prep_window_in, 0)
        lax.fori_loop(0, 2, prep_window_out, 0)
        for c in late_copies():
            c.start()
        for c in pair_copies(0):
            c.wait()
        prep_pair(0, 0)

    def _last_weights():
        for c in late_copies():
            c.wait()
        lax.fori_loop(1, NPAIR, prep_pair, 0)
        lax.fori_loop(0, HD // 32, prep_memory_out, 0)

    ticks = []

    def tick(y):
        ticks.extend(y[0:8, c:c + 128] for c in range(0, y.shape[1], 128))
        return y

    def never(rows, tiles=1):
        return jnp.concatenate([cmask[0:rows, 0:128]] * tiles, axis=1) > 1.0

    def after(t, x):
        return x if t < 0 else jnp.where(never(8), ticks[min(t, len(ticks) - 1)], x)

    def before(deps, a):
        if not deps:
            return a
        dep = functools.reduce(jnp.maximum, deps)
        head = jnp.where(never(8), dep if a.dtype == F32 else pltpu.bitcast(dep, a.dtype), a[0:8, 0:128])
        if a.shape[1] > 128:
            head = jnp.concatenate([head, a[0:8, 128:]], axis=1)
        return jnp.concatenate([head, a[8:]], axis=0)

    def held_for(blocks, counts, lhs):
        counts, seen = iter(counts), [0]

        def held(i):
            n = next(counts)
            deps = [b[r * 8:r * 8 + 8, _tile(c)] for r in range(seen[0], seen[0] + n)
                    for b in blocks[-2:] for c in range(NPAIR)]
            seen[0] += n
            return before(deps, lhs[i])
        return held

    def reordered(ref):
        return _unpack(jnp.concatenate([jnp.concatenate(
            [ref[c, d * PITCH:d * PITCH + 16, :] for d in range(16)], axis=0) for c in range(NPAIR)], axis=1))

    def window_in(ch, m, lhs):
        dst, off = ((kb, HALO), (qb, 0), (vb, HALO))[m]

        def done(i, j, y):
            r0 = off + ch * RC + i * 128
            if m == 1:
                y = y * QSCALE
            for c in range(NPAIR):
                dst[j * NPAIR + c, r0:r0 + 128, :] = y[:, _tile(c)]
        return _block_matmul(
            _whole(lambda i: tick(_dot_nt(lhs(i).astype(BF16), reordered(wa.at[m, i])))), done)

    def taps(ref, c, r0, w):
        o0 = HALO + r0 - DIL * w
        return ref[c, o0:o0 + 8, :]

    def row_group(i):
        return i // 2 + (i % 2) * (RC // 16)

    @functools.cache
    def window_probs(ch, i):
        r0 = ch * RC + row_group(i) * 8
        t = int(TUNE["pace"][ch][0] + i * TUNE["pace"][ch][1])
        qs = [after(t, qb[c, r0:r0 + 8, :]) for c in range(NT)]
        logits = []
        for w in range(W):
            acc = functools.reduce(jnp.add, [qs[c] * taps(kb, c, r0, w) for c in range(NT)])
            acc = acc + pltpu.roll(acc, 64, 1)
            acc = acc + pltpu.roll(acc, 32, 1)
            if r0 < DIL * w:
                pos = seg * L + r0 + lax.broadcasted_iota(jnp.int32, (8, 128), 0)
                acc = jnp.where(pos >= DIL * w, acc, NEG)
            logits.append(acc)
        mx = functools.reduce(jnp.maximum, logits)
        es = [jnp.exp2(v - mx) for v in logits]
        return es, 1.0 / functools.reduce(jnp.add, es)

    @functools.cache
    def window_rows(ch, i):
        r0 = ch * RC + row_group(i) * 8
        es, inv = window_probs(ch, i)
        inv = after(int(TUNE["pace"][ch][2] + i * TUNE["pace"][ch][3]), inv)
        ps = [e * inv for e in es]
        return jnp.concatenate(
            [functools.reduce(jnp.add, [ps[w] * taps(vb, c, r0, w) for w in range(W)]) for c in range(NT)], axis=1)

    def window_blocks(ch):
        rows = [None] * (RC // 8)
        for i in range(RC // 8):
            rows[row_group(i)] = window_rows(ch, i)
        return _row_blocks(jnp.concatenate(rows, axis=0))

    def add_rows(ch):
        def done(i, j, y):
            r0 = ch * RC + i * 128
            xs[r0:r0 + 128, j * HD:(j + 1) * HD] += y
        return done

    def window_out(ch, lhs):
        return _block_matmul(
            _whole(lambda i: tick(_dot(lhs(i).astype(BF16), reordered(woa.at[i])))), add_rows(ch))

    def memory_qk(p, ch, lhs=None):
        def done(i, j, y):
            r0 = ch * RC + i * 128
            bq[p % 2 * 2 + j, r0:r0 + 128, :] = y[:, :128]
            bk[p % 2 * 2 + j, r0:r0 + 128, :] = y[:, 128:]
        if lhs is not None:
            return _block_matmul(_whole(lambda i: tick(_dot(lhs(i).astype(BF16), _unpack(wqk[p, i])))), done)
        return _block_matmul(_tiled(
            lambda i, k, n: _dot(_unpack(xb[i, ch * 64:(ch + 1) * 64, _tile(k)]),
                                 _unpack(wqk[p, i, k * 64:(k + 1) * 64, _tile(n)])), 4, 2, tick), done)

    def memory_v(p):
        def done(i, j, y):
            for ch in range(NCH):
                c0 = ch * RC + i * 128
                bv[p % 2 * 2 + j, :, c0:c0 + 128] = _pack(y[:, _tile(ch)])
        return _block_matmul(_tiled(
            lambda i, k, n: _dot_nt(_unpack(wvt[p, i, :, _tile(k)]),
                                    _unpack(xb[i, n * 64:(n + 1) * 64, _tile(k)])), 4, NCH, tick), done)

    def finish_rows(ch):
        def done(i, j, y):
            idx = (slice(ch * RC + i * 128, ch * RC + (i + 1) * 128), slice(j * HD, (j + 1) * HD))
            xnew = xs[idx] + y
            xout[ch * 4 + i * 2 + j] = xnew.astype(BF16)
            out_copy(seg, ch, i, j).start()
            xs[idx] = jnp.where(rep == 0, xnew, xin[idx].astype(F32))
        return done

    def memory_out(ch, p0, p1, hold=lambda a: a):
        def prod(i):
            acc = None
            for p in range(p0, p1):
                t = _dot(_unpack(hold(oc[p, i, ch * 64:(ch + 1) * 64, :])), _unpack(wob[i, p * 64:(p + 1) * 64, :]))
                acc = t if acc is None else acc + t
                tick(t[:, 0:128])
                yield
            return acc
        return _block_matmul(prod, finish_rows(ch) if p1 == NPAIR else add_rows(ch))

    lane_head = lax.broadcasted_iota(jnp.int32, (1, 128), 1) // DH

    def head_queries(q, j):
        qh = [q[_tile(j), :] * jnp.where(lane_head == h, QSCALE, 0.0) for h in range(4)]
        return [(t[:64], t[64:]) for t in qh]

    def corner(q, k, j):
        qm = jnp.concatenate([hi for _, hi in head_queries(q, j)], axis=0)
        return _dot_nt(k[j * 128 + 64:(j + 1) * 128, :].astype(BF16), qm.astype(BF16))

    def scores(q, k, j, cor):
        nk = 128 * j + 64
        qm = jnp.concatenate([part for h, (lo, hi) in enumerate(head_queries(q, j))
                              for part in ((lo, hi) if h % 2 else (hi, lo))], axis=0)
        st = _dot_nt(k[0:nk, :].astype(BF16), qm.astype(BF16))
        for i in range(j + 1):
            tick(st[i * 128:i * 128 + 8, 0:128])
        diag = jnp.concatenate(
            [st[nk - 64:], jnp.concatenate([cor[:, _tile(h // 2)] for h in range(4)], axis=1)], axis=0)
        diag = diag + jnp.concatenate([cmask[...]] * 2, axis=1)
        return diag if j == 0 else jnp.concatenate([st[:nk - 64], diag], axis=0)

    def memory_read(g, q):
        zrow = lax.broadcasted_iota(jnp.int32, (16, 128), 0)
        zl = jnp.where(zrow == lane_head, jnp.broadcast_to(zs[rep * NT + g, 0:1, :], (16, 128)), 0.0)
        return _dot_nt(jnp.concatenate([mt[rep * NT + g], zl], axis=0).astype(BF16), _phi(q[...]).astype(BF16))

    def memory_update(g, k, vt):
        pk = _phi(k[...])
        upd = functools.reduce(jnp.add, [
            _dot(_unpack(vt[:, _tile(i)]), pk[_tile(i)].astype(BF16)) for i in range(L // 128)])
        row_head = lax.broadcasted_iota(jnp.int32, (128, 128), 0) // DH
        mt[rep * NT + g] += jnp.where(row_head == lane_head, upd, 0.0)
        zs[rep * NT + g] += jnp.sum(pk, axis=0, keepdims=True)

    def attend(g, e, j, st, nd, vt, lag):
        mx = jnp.broadcast_to(jnp.max(st, axis=0, keepdims=True), (8, 512))
        pv, l = [None] * 4, None
        for i in range(j + 1):
            mi = jnp.concatenate([after(len(ticks) - lag[0], mx[:, _tile(h)]) for h in range(4)], axis=1)
            p3 = jnp.exp2(st[_tile(i)].reshape(16, 8, 512) - mi)
            p = p3.reshape(128, 512)
            li = jnp.sum(p3, axis=0)
            l = li if i == 0 else l + li
            for h in range(4):
                t = _dot(_unpack(vt[h * 16:(h + 1) * 16, _tile(i)]), p[:, _tile(h)].astype(BF16))
                pv[h] = t if i == 0 else pv[h] + t
            if i < j:
                yield
        l = jnp.sum(l, axis=0, keepdims=True)
        rows = []
        for h in range(4):
            gh = gate[g * 4 + h][0:1, :]
            num = nd[h * DH:(h + 1) * DH, _tile(j)]
            den = nd[128 + h:129 + h, _tile(j)] + 1e-6
            loc = pv[h] * ((1.0 - gh) / l[:, _tile(h)])
            rows.append(num * (gh / den) + (loc if h % 2 else pltpu.roll(loc, 64, 1)))
        of[e, _tile(j), :] = jnp.concatenate(rows, axis=0).T
        yield

    def keep_output(p, ch):
        r0 = ch * RC
        blocks = _lhs_blocks(of[0, r0:r0 + 128, :], of[1, r0:r0 + 128, :],
                             of[0, r0 + 128:r0 + 256, :], of[1, r0 + 128:r0 + 256, :])
        for i, b in enumerate(blocks):
            oc[p, i, ch * 64:(ch + 1) * 64, :] = _pack(b)

    def memory_pair(p, last):
        del ticks[:]
        if last:
            fill = _chain(memory_out(0, 0, p), memory_out(1, 0, TUNE["split"]))
            tail = memory_out(0, p, NPAIR)
        else:
            fill = _chain(memory_qk(p + 1, 0), memory_qk(p + 1, 1), memory_v(p + 1))
        for e, steps in enumerate(TUNE["plan_last" if last else "plan"].split("/")):
            g = 2 * p + e
            q, k, vt = (ref.at[p % 2 * 2 + e] for ref in (bq, bk, bv))
            todo, cur, nd, seen, corners, lag = [], None, None, [], {}, [0]
            for op in steps.split():
                if op == "f":
                    _run(fill, 1)
                elif op == "F":
                    _run(fill)
                elif op == "x":
                    _run(tail, 1)
                elif op == "X":
                    _run(tail)
                elif op[0] == "s":
                    j = int(op[1])
                    if j not in corners:
                        corners.update({i: corner(q, k, i) for i in (j, j ^ 1)})
                    todo.append((j, scores(q, k, j, corners[j])))
                elif op == "n":
                    nd = memory_read(g, q)
                elif op == "u":
                    memory_update(g, k, vt)
                elif op == "o":
                    keep_output(p, seen[-1] // 2)
                else:
                    lag[0] = int(op[1])
                    if cur is None or next(cur, "end") == "end":
                        j, st = todo.pop(0)
                        seen.append(j)
                        cur = attend(g, e, j, st, nd, vt, lag)
                        next(cur)
            assert len(seen) == L // 128 and next(cur, "end") == "end"
        return 0

    fetch_next = (rep == 1) & (seg < NSEG - 1)
    pl.when(fetch_next)(lambda: x_copy(seg + 1).start())

    def keys_stage():
        for c in range(NT):
            kb[c, 0:HALO, :] = kc[rep, c]
            vb[c, 0:HALO, :] = vc[rep, c]
        xn1 = _layernorm(xs[RC:L, :])
        xa[RC:L, :] = xn1
        in0, in1 = _row_blocks(xa[0:RC, :]), _row_blocks(xn1)
        _run(window_in(0, 0, held_for(in1, TUNE["due_norm"], in0)))
        _run(window_in(1, 0, lambda i: in1[i]))

    def window_stage():
        del ticks[:]
        a_in = [_row_blocks(xa[ch * RC:(ch + 1) * RC, :]) for ch in range(NCH)]
        due_probs, due_mix = iter(TUNE["due_probs"]), iter((0,) * (3 * NP) + TUNE["due_mix0"])
        seen = [0, 0]

        def held(ch, i):
            n, n2 = next(due_probs), next(due_mix)
            deps = [window_probs(*divmod(r, RC // 8))[1] for r in range(seen[0], seen[0] + n)]
            deps += [window_rows(0, r)[:, _tile(c)] for r in range(seen[1], seen[1] + n2) for c in range(NT)]
            seen[0] += n
            seen[1] += n2
            return before(deps, a_in[ch][i])
        for ch, m in ((0, 1), (1, 1), (0, 2), (1, 2)):
            _run(window_in(ch, m, functools.partial(held, ch)))
        o0, o1 = window_blocks(0), window_blocks(1)
        _run(window_out(0, held_for(o1, TUNE["due_mix1"], o0)))
        x0 = _row_blocks(_layernorm(xs[0:RC, :]))
        t0 = len(ticks)
        _run(window_out(1, held_for(x0, TUNE["due_norm0"], o1)))
        x1 = _row_blocks(_layernorm(xs[RC:L, :]))
        _run(memory_qk(0, 0, held_for(x1, TUNE["due_norm1"], x0)))
        t1 = len(ticks)
        _run(memory_qk(0, 1, lambda i: x1[i]))
        for ch, (blocks, t) in enumerate(((x0, t0), (x1, t1))):
            start, step = TUNE["keep"][ch]
            for i, blk in enumerate(blocks):
                dep = jnp.concatenate([jnp.concatenate([ticks[t + start + i * step]] * 4, axis=0)] * 4, axis=1)
                for r in range(0, 128, 32):
                    xb[i, ch * 64 + r // 2:ch * 64 + r // 2 + 16, :] = _pack(
                        jnp.where(never(32, 4), dep, blk[r:r + 32]))
        _run(memory_v(0))
        for c in range(NT):
            kc[rep, c] = kb[c, L:L + HALO, :]
            vc[rep, c] = vb[c, L:L + HALO, :]

    def last_stage():
        memory_pair(NPAIR - 1, True)
        xn0 = _layernorm(xs[0:RC, :])
        xa[0:RC, :] = xn0
        counts, seen = iter(TUNE["due_next"]), [0]

        def hold(a):
            n = next(counts)
            deps = [xn0[r * 8:r * 8 + 8, _tile(c)] for r in range(seen[0], seen[0] + n) for c in (0, NT - 1)]
            seen[0] += n
            return before(deps, a)
        _run(memory_out(1, TUNE["split"], NPAIR, hold))

    keys_stage()
    pl.when(first_step)(_more_weights)
    window_stage()
    pl.when(first_step)(_last_weights)
    pl.when(jnp.logical_not(first_step))(lambda: wait_out(seg - 1 + rep))
    pl.when(fetch_next)(lambda: x_copy(seg + 1).wait())
    lax.fori_loop(0, NPAIR - 1, lambda p, carry: memory_pair(p, False), 0)
    last_stage()
    pl.when((seg == NSEG - 1) & (rep == 1))(lambda: wait_out(seg))


@jax.jit
def pallas_interleave_layers__sliding_local_dilated__memory_aug_infini_attn__prompt_kernel(
        A_x, A_wqkv, A_wo, B_x, B_wq, B_wk, B_wv, B_wo, B_beta):
    del B_x
    hbm = pl.BlockSpec(memory_space=pl.ANY)
    out = pl.pallas_call(
        _kernel,
        grid=(NSEG, 2),
        in_specs=[hbm, pl.BlockSpec((1, H), lambda s, r: (0, 0)), hbm, hbm, hbm, hbm, hbm, hbm],
        out_specs=hbm,
        out_shape=jax.ShapeDtypeStruct((S, D), BF16),
        scratch_shapes=[
            pltpu.VMEM((L, D), BF16),
            pltpu.VMEM((4 * NCH, 128, HD), BF16),
            pltpu.VMEM((6, D, HD), BF16),
            pltpu.VMEM((2, HD, D), BF16),
            pltpu.VMEM((3, NPAIR, D, 256), BF16),
            pltpu.VMEM((D, D), BF16),
            pltpu.VMEM((3, NP, NPAIR, WROWS, 128), U32),
            pltpu.VMEM((NP, NPAIR, WROWS, 128), U32),
            pltpu.VMEM((NPAIR, NP, HD // 2, 256), U32),
            pltpu.VMEM((NPAIR, NP, 64, HD), U32),
            pltpu.VMEM((NP, HD // 2, HD), U32),
            pltpu.VMEM((L, D), F32),
            pltpu.VMEM((L, D), F32),
            pltpu.VMEM((NP, L // 4, HD), U32),
            pltpu.VMEM((NT, L, 128), F32),
            pltpu.VMEM((NT, HALO + L, 128), F32),
            pltpu.VMEM((NT, HALO + L, 128), F32),
            pltpu.VMEM((2, NT, HALO, 128), F32),
            pltpu.VMEM((2, NT, HALO, 128), F32),
            pltpu.VMEM((2, L, 128), F32),
            pltpu.VMEM((NPAIR, NP, L // 4, 128), U32),
            pltpu.VMEM((4, L, 128), F32),
            pltpu.VMEM((4, L, 128), F32),
            pltpu.VMEM((4, 64, L), U32),
            pltpu.VMEM((2 * NT, 128, 128), F32),
            pltpu.VMEM((2 * NT, 8, 128), F32),
            pltpu.VMEM((H, 8, 128), F32),
            pltpu.VMEM((128, 256), F32),
            pltpu.SemaphoreType.DMA((30,)),
        ],
        compiler_params=pltpu.CompilerParams(
            dimension_semantics=("arbitrary", "arbitrary"),
            vmem_limit_bytes=110 * 2**20),
        name="interleave",
    )(A_x.reshape(S, D), B_beta.reshape(1, H), A_wqkv, A_wo, B_wq, B_wk, B_wv, B_wo)
    return out.reshape(1, S, D)
```

```python
import functools
import math

import jax
import jax.numpy as jnp
from jax import lax
from jax.experimental import pallas as pl
from jax.experimental.pallas import tpu as pltpu

S, D, H, DH = 2048, 1024, 32, 32
NSEG = 4
L = S // NSEG
W, DIL = 8, 2
HALO = 16
NT = D // 128
NPAIR = NT // 2
HD = D // 2
RC = 256
NCH = L // RC
NP = 7
PITCH = 17
WROWS = 16 * PITCH + 16
LOG2E = math.log2(math.e)
QSCALE = DH ** -0.5 * LOG2E
NEG = -1e9 * LOG2E
F32, BF16, U32 = jnp.float32, jnp.bfloat16, jnp.uint32

TUNE = dict(
    pace=((24, 1.05, 80, 0.75), (56, 1.1, 110, 0.1)),
    due_norm=(0, 2, 3, 4, 2, 2, 3),
    due_probs=(0, 0, 0, 0, 0, 0, 0, 0, 3, 3, 4, 5, 4, 4, 4, 5, 3, 4, 4, 4, 4, 4, 3, 3, 3, 0, 0, 0),
    due_mix0=(0, 0, 1, 5, 7, 5, 10),
    due_mix1=(0, 0, 4, 3, 4, 4, 0),
    due_norm0=(0, 0, 1, 1, 3, 0, 1),
    due_next=(0, 0, 1, 5, 1, 2, 10, 1, 2, 2, 0, 5, 3, 0),
    split=2,
    plan="f f s3 f s2 f n f p3 f p3 f p3 f f p3 s1 p3 f f p3 f s0 p3 f f p3 f f p4 f u f f p3 "
         "/ f s3 s2 n f p3 f p2 f p3 f f p4 f f s1 p3 f p3 f p2 o s0 f p3 f f p3 u f p2 f o F",
    plan_last="f s0 s1 n p4 s2 f p3 f p3 s3 f p3 f p3 p2 f f p3 f p3 f p3 f f p4 f u "
              "/ s0 s1 f n f p3 s2 p3 f p3 o s3 f p4 f p3 p2 f x f p3 x p3 f f x p4 x p3 o f x f x u F X",
)


def _dot(a, b):
    return jnp.dot(a, b, preferred_element_type=F32)


def _dot_nt(a, b):
    return lax.dot_general(a, b, (((1,), (1,)), ((), ())), preferred_element_type=F32)


def _pack(x):
    return pltpu.bitcast(x.astype(BF16), U32)


def _unpack(x):
    return pltpu.bitcast(x, BF16)


def _tile(i):
    return slice(i * 128, (i + 1) * 128)


def _lhs_blocks(a11, a12, a21, a22):
    return [a11 + a22, a21 + a22, a11, a22, a11 + a12, a21 - a11, a12 - a22]


def _rhs_blocks(b11, b12, b21, b22):
    return [b11 + b22, b11, b12 - b22, b21 - b11, b22, b11 + b12, b21 + b22]


def _row_blocks(x):
    return _lhs_blocks(x[:128, :HD], x[:128, HD:], x[128:, :HD], x[128:, HD:])


def _block_matmul(prod, done):
    p3 = yield from prod(2)
    p5 = yield from prod(4)
    done(0, 1, p3 + p5)
    p2 = yield from prod(1)
    p4 = yield from prod(3)
    done(1, 0, p2 + p4)
    u, v = p4 - p5, p3 - p2
    p1 = yield from prod(0)
    u, v = u + p1, v + p1
    p7 = yield from prod(6)
    done(0, 0, u + p7)
    p6 = yield from prod(5)
    done(1, 1, v + p6)


def _whole(fn):
    def prod(i):
        y = fn(i)
        yield
        return y
    return prod


def _tiled(dot, nk, nn, tick):
    def prod(i):
        acc = [None] * nn
        for n in range(nn):
            for k in range(nk):
                t = dot(i, k, n)
                acc[n] = t if k == 0 else acc[n] + t
            tick(t)
            yield
        return jnp.concatenate(acc, axis=1)
    return prod


def _run(gen, n=None):
    k = 0
    while (n is None or k < n) and next(gen, "end") != "end":
        k += 1


def _chain(*gens):
    for g in gens:
        yield from g


def _layernorm(x):
    m = jnp.mean(x, axis=-1, keepdims=True)
    xc = x - m
    v = jnp.mean(xc * xc, axis=-1, keepdims=True)
    return xc * lax.rsqrt(v + 1e-5)


def _phi(t):
    return jnp.where(t > 0, t + 1.0, jnp.exp(t))


def _kernel(x_hbm, beta_ref, wqkv_hbm, woa_hbm, wq_hbm, wk_hbm, wv_hbm, wob_hbm, out_hbm,
            xin, xout, raw_a, raw_ao, raw_b, raw_bo, wa, woa, wqk, wvt, wob,
            xs, xa, xb, qb, kb, vb, kc, vc, of, oc, bq, bk, bv, mt, zs, gate, cmask, sems):
    seg = pl.program_id(0)
    rep = pl.program_id(1)
    first_step = (seg == 0) & (rep == 0)

    def window_copy(i):
        m, j = divmod(i, 2)
        if m < 3:
            c0 = (1, 0, 2)[m] * D + j * HD
            return pltpu.make_async_copy(wqkv_hbm.at[:, pl.ds(c0, HD)], raw_a.at[i], sems.at[i])
        return pltpu.make_async_copy(woa_hbm.at[pl.ds(j * HD, HD)], raw_ao.at[j], sems.at[i])

    def pair_copies(p):
        return [pltpu.make_async_copy(w.at[:, pl.ds(p * 256, 256)], raw_b.at[m, p], sems.at[8 + 3 * p + m])
                for m, w in enumerate((wq_hbm, wk_hbm, wv_hbm))]

    def late_copies():
        return ([c for p in range(1, NPAIR) for c in pair_copies(p)]
                + [pltpu.make_async_copy(wob_hbm, raw_bo, sems.at[20])])

    def x_copy(s):
        return pltpu.make_async_copy(x_hbm.at[pl.ds(pl.multiple_of(s * L, L), L)], xin, sems.at[21])

    def out_copy(s, ch, i, j):
        rows = pl.ds(pl.multiple_of(s * L + ch * RC + i * 128, 128), 128)
        n = ch * 4 + i * 2 + j
        return pltpu.make_async_copy(xout.at[n], out_hbm.at[rows, pl.ds(j * HD, HD)], sems.at[22 + n])

    def wait_out(s):
        for n in range(4 * NCH):
            out_copy(s, n // 4, n // 2 % 2, n % 2).wait()

    def selector(reorder):
        row = lax.broadcasted_iota(jnp.int32, (128, 128), 0)
        col = lax.broadcasted_iota(jnp.int32, (128, 128), 1)
        if reorder:
            row = (((row >> 5) & 1) * 2 + (row & 1)) * DH + (row >> 6) * 16 + ((row >> 1) & 15)
        return jnp.where(row == col, 1.0, 0.0).astype(BF16)

    def packed_blocks(*quad):
        quad = [pltpu.bitcast(b, U32) for b in quad]
        vals = [_unpack(b).astype(F32) for b in quad]
        out = []
        for blk in _rhs_blocks(*vals):
            same = [i for i, v in enumerate(vals) if v is blk]
            out.append(quad[same[0]] if same else _pack(blk))
        return out

    def arrive(piece, lo, hi):
        for i in range(lo, hi):
            @pl.when(piece == i)
            def _():
                window_copy(i).wait()
                for n in {0: (1,), 1: (2, 3, 4, 5)}.get(i, ()):
                    window_copy(n).start()

    def scatter(dst, t, blocks):
        for i, v in enumerate(blocks):
            v = _pack(v)
            for c in range(NPAIR):
                for hp in range(2):
                    dst(i, c)[pl.ds(t * 2 + hp, 16, stride=PITCH), :] = v[hp * 16:(hp + 1) * 16, _tile(c)]

    def prep_window_in(piece, carry):
        arrive(piece, 0, 6)
        for t in range(4):
            top = _dot_nt(selector(True), raw_a[piece, 0:HD, _tile(t)])
            bot = _dot_nt(selector(True), raw_a[piece, HD:D, _tile(t)])
            scatter(lambda i, c: wa.at[piece // 2, i, c], (piece % 2) * 4 + t,
                    _rhs_blocks(top[:64], top[64:], bot[:64], bot[64:]))
        return carry

    def prep_window_out(j, carry):
        arrive(6 + j, 6, 8)
        for t in range(4):
            y = _dot(selector(True), raw_ao[j, _tile(t), :])
            scatter(lambda i, c: woa.at[i, c], j * 4 + t,
                    _rhs_blocks(y[:64, :HD], y[:64, HD:], y[64:, :HD], y[64:, HD:]))
        return carry

    def prep_pair(p, carry):
        quad = [_dot_nt(selector(False), raw_b[2, p, kh * HD:(kh + 1) * HD, _tile(e)])
                for kh in range(2) for e in range(2)]
        for i, v in enumerate(_rhs_blocks(*quad)):
            wvt[p, i] = _pack(v)

        def rows_qk(j, c):
            for m in range(2):
                quad = [raw_b[m, p, pl.ds(pl.multiple_of(kh * HD + j * 64, 64), 64), _tile(e)]
                        for kh in range(2) for e in range(2)]
                for i, v in enumerate(packed_blocks(*quad)):
                    wqk[p, i, pl.ds(pl.multiple_of(j * 32, 32), 32), _tile(m)] = v
            return c
        return lax.fori_loop(0, HD // 64, rows_qk, carry)

    def prep_memory_out(t, carry):
        r0 = (t // 4) * 256 + (t % 4) * 32
        quad = [raw_bo[pl.ds(pl.multiple_of(r0 + e * 128, 32), 32), c:c + HD] for e in range(2) for c in (0, HD)]
        for i, v in enumerate(packed_blocks(*quad)):
            wob[i, pl.ds(pl.multiple_of(t * 16, 16), 16), :] = v
        return carry

    @pl.when(first_step)
    def _start():
        window_copy(0).start()
        x_copy(0).start()
        kc[...] = jnp.zeros(kc.shape, F32)
        vc[...] = jnp.zeros(vc.shape, F32)
        mt[...] = jnp.zeros(mt.shape, F32)
        zs[...] = jnp.zeros(zs.shape, F32)
        g_all = jax.nn.sigmoid(beta_ref[...].astype(F32))
        head = lax.broadcasted_iota(jnp.int32, (1, H), 1)
        for h in range(H):
            gate[h] = jnp.broadcast_to(jnp.sum(jnp.where(head == h, g_all, 0.0), axis=1, keepdims=True), (8, 128))
        kk = lax.broadcasted_iota(jnp.int32, (128, 256), 0)
        qq = lax.broadcasted_iota(jnp.int32, (128, 256), 1)
        qq = jnp.where(qq < 128, qq ^ 64, qq - 128)
        cmask[...] = jnp.where(qq < kk, NEG, 0.0).astype(F32)
        prep_window_in(0, 0)
        x_copy(0).wait()

        def load_rows(j, carry):
            rows = pl.ds(pl.multiple_of(j * 64, 64), 64)
            later = pl.ds(pl.multiple_of(RC + j * 64, 64), 64)
            x0 = xin[rows, :].astype(F32)
            xs[rows, :] = x0
            xa[rows, :] = _layernorm(x0)
            xs[later, :] = xin[later, :].astype(F32)
            return carry
        lax.fori_loop(0, RC // 64, load_rows, 0)
        prep_window_in(1, 0)

    def _more_weights():
        for c in [window_copy(6), window_copy(7)] + pair_copies(0):
            c.start()
        lax.fori_loop(2, 6, prep_window_in, 0)
        lax.fori_loop(0, 2, prep_window_out, 0)
        for c in late_copies():
            c.start()
        for c in pair_copies(0):
            c.wait()
        prep_pair(0, 0)

    def _last_weights():
        for c in late_copies():
            c.wait()
        lax.fori_loop(1, NPAIR, prep_pair, 0)
        lax.fori_loop(0, HD // 32, prep_memory_out, 0)

    ticks = []

    def tick(y):
        ticks.extend(y[0:8, c:c + 128] for c in range(0, y.shape[1], 128))
        return y

    def never():
        return cmask[0:8, 0:128] > 1.0

    def after(t, x):
        return x if t < 0 else jnp.where(never(), ticks[min(t, len(ticks) - 1)], x)

    def before(deps, a):
        if not deps:
            return a
        dep = functools.reduce(jnp.maximum, deps)
        head = jnp.where(never(), dep if a.dtype == F32 else pltpu.bitcast(dep, a.dtype), a[0:8, 0:128])
        if a.shape[1] > 128:
            head = jnp.concatenate([head, a[0:8, 128:]], axis=1)
        return jnp.concatenate([head, a[8:]], axis=0)

    def held_for(blocks, counts, lhs):
        counts, seen = iter(counts), [0]

        def held(i):
            n = next(counts)
            deps = [b[r * 8:r * 8 + 8, _tile(c)] for r in range(seen[0], seen[0] + n)
                    for b in blocks[-2:] for c in range(NPAIR)]
            seen[0] += n
            return before(deps, lhs[i])
        return held

    def reordered(ref):
        return _unpack(jnp.concatenate([jnp.concatenate(
            [ref[c, d * PITCH:d * PITCH + 16, :] for d in range(16)], axis=0) for c in range(NPAIR)], axis=1))

    def window_in(ch, m, lhs):
        dst, off = ((kb, HALO), (qb, 0), (vb, HALO))[m]

        def done(i, j, y):
            r0 = off + ch * RC + i * 128
            if m == 1:
                y = y * QSCALE
            for c in range(NPAIR):
                dst[j * NPAIR + c, r0:r0 + 128, :] = y[:, _tile(c)]
        return _block_matmul(
            _whole(lambda i: tick(_dot_nt(lhs(i).astype(BF16), reordered(wa.at[m, i])))), done)

    def taps(ref, c, r0, w):
        o0 = HALO + r0 - DIL * w
        return ref[c, o0:o0 + 8, :]

    def row_group(i):
        return i // 2 + (i % 2) * (RC // 16)

    @functools.cache
    def window_probs(ch, i):
        r0 = ch * RC + row_group(i) * 8
        t = int(TUNE["pace"][ch][0] + i * TUNE["pace"][ch][1])
        qs = [after(t, qb[c, r0:r0 + 8, :]) for c in range(NT)]
        logits = []
        for w in range(W):
            acc = functools.reduce(jnp.add, [qs[c] * taps(kb, c, r0, w) for c in range(NT)])
            acc = acc + pltpu.roll(acc, 64, 1)
            acc = acc + pltpu.roll(acc, 32, 1)
            if r0 < DIL * w:
                pos = seg * L + r0 + lax.broadcasted_iota(jnp.int32, (8, 128), 0)
                acc = jnp.where(pos >= DIL * w, acc, NEG)
            logits.append(acc)
        mx = functools.reduce(jnp.maximum, logits)
        es = [jnp.exp2(v - mx) for v in logits]
        return es, 1.0 / functools.reduce(jnp.add, es)

    @functools.cache
    def window_rows(ch, i):
        r0 = ch * RC + row_group(i) * 8
        es, inv = window_probs(ch, i)
        inv = after(int(TUNE["pace"][ch][2] + i * TUNE["pace"][ch][3]), inv)
        ps = [e * inv for e in es]
        return jnp.concatenate(
            [functools.reduce(jnp.add, [ps[w] * taps(vb, c, r0, w) for w in range(W)]) for c in range(NT)], axis=1)

    def window_blocks(ch):
        rows = [None] * (RC // 8)
        for i in range(RC // 8):
            rows[row_group(i)] = window_rows(ch, i)
        return _row_blocks(jnp.concatenate(rows, axis=0))

    def add_rows(ch):
        def done(i, j, y):
            r0 = ch * RC + i * 128
            xs[r0:r0 + 128, j * HD:(j + 1) * HD] += y
        return done

    def window_out(ch, lhs):
        return _block_matmul(
            _whole(lambda i: tick(_dot(lhs(i).astype(BF16), reordered(woa.at[i])))), add_rows(ch))

    def memory_qk(p, ch, lhs=None):
        def done(i, j, y):
            r0 = ch * RC + i * 128
            bq[p % 2 * 2 + j, r0:r0 + 128, :] = y[:, :128]
            bk[p % 2 * 2 + j, r0:r0 + 128, :] = y[:, 128:]
        if lhs is not None:
            return _block_matmul(_whole(lambda i: tick(_dot(_unpack(lhs[i]), _unpack(wqk[p, i])))), done)
        return _block_matmul(_tiled(
            lambda i, k, n: _dot(_unpack(xb[i, ch * 64:(ch + 1) * 64, _tile(k)]),
                                 _unpack(wqk[p, i, k * 64:(k + 1) * 64, _tile(n)])), 4, 2, tick), done)

    def memory_v(p):
        def done(i, j, y):
            for ch in range(NCH):
                c0 = ch * RC + i * 128
                bv[p % 2 * 2 + j, :, c0:c0 + 128] = _pack(y[:, _tile(ch)])
        return _block_matmul(_tiled(
            lambda i, k, n: _dot_nt(_unpack(wvt[p, i, :, _tile(k)]),
                                    _unpack(xb[i, n * 64:(n + 1) * 64, _tile(k)])), 4, NCH, tick), done)

    def finish_rows(ch):
        def done(i, j, y):
            idx = (slice(ch * RC + i * 128, ch * RC + (i + 1) * 128), slice(j * HD, (j + 1) * HD))
            xnew = xs[idx] + y
            xout[ch * 4 + i * 2 + j] = xnew.astype(BF16)
            out_copy(seg, ch, i, j).start()
            xs[idx] = jnp.where(rep == 0, xnew, xin[idx].astype(F32))
        return done

    def memory_out(ch, p0, p1, hold=lambda a: a):
        def prod(i):
            acc = None
            for p in range(p0, p1):
                t = _dot(_unpack(hold(oc[p, i, ch * 64:(ch + 1) * 64, :])), _unpack(wob[i, p * 64:(p + 1) * 64, :]))
                acc = t if acc is None else acc + t
                tick(t[:, 0:128])
                yield
            return acc
        return _block_matmul(prod, finish_rows(ch) if p1 == NPAIR else add_rows(ch))

    lane_head = lax.broadcasted_iota(jnp.int32, (1, 128), 1) // DH

    def head_queries(q, j):
        qh = [q[_tile(j), :] * jnp.where(lane_head == h, QSCALE, 0.0) for h in range(4)]
        return [(t[:64], t[64:]) for t in qh]

    def corner(q, k, j):
        qm = jnp.concatenate([hi for _, hi in head_queries(q, j)], axis=0)
        return _dot_nt(k[j * 128 + 64:(j + 1) * 128, :].astype(BF16), qm.astype(BF16))

    def scores(q, k, j, cor):
        nk = 128 * j + 64
        qm = jnp.concatenate([part for h, (lo, hi) in enumerate(head_queries(q, j))
                              for part in ((lo, hi) if h % 2 else (hi, lo))], axis=0)
        st = _dot_nt(k[0:nk, :].astype(BF16), qm.astype(BF16))
        for i in range(j + 1):
            tick(st[i * 128:i * 128 + 8, 0:128])
        diag = jnp.concatenate(
            [st[nk - 64:], jnp.concatenate([cor[:, _tile(h // 2)] for h in range(4)], axis=1)], axis=0)
        diag = diag + jnp.concatenate([cmask[...]] * 2, axis=1)
        return diag if j == 0 else jnp.concatenate([st[:nk - 64], diag], axis=0)

    def memory_read(g, q):
        zrow = lax.broadcasted_iota(jnp.int32, (16, 128), 0)
        zl = jnp.where(zrow == lane_head, jnp.broadcast_to(zs[rep * NT + g, 0:1, :], (16, 128)), 0.0)
        return _dot_nt(jnp.concatenate([mt[rep * NT + g], zl], axis=0).astype(BF16), _phi(q[...]).astype(BF16))

    def memory_update(g, k, vt):
        pk = _phi(k[...])
        upd = functools.reduce(jnp.add, [
            _dot(_unpack(vt[:, _tile(i)]), pk[_tile(i)].astype(BF16)) for i in range(L // 128)])
        row_head = lax.broadcasted_iota(jnp.int32, (128, 128), 0) // DH
        mt[rep * NT + g] += jnp.where(row_head == lane_head, upd, 0.0)
        zs[rep * NT + g] += jnp.sum(pk, axis=0, keepdims=True)

    def attend(g, e, j, st, nd, vt, lag):
        mx = jnp.broadcast_to(jnp.max(st, axis=0, keepdims=True), (8, 512))
        pv, l = [None] * 4, None
        for i in range(j + 1):
            mi = jnp.concatenate([after(len(ticks) - lag[0], mx[:, _tile(h)]) for h in range(4)], axis=1)
            p3 = jnp.exp2(st[_tile(i)].reshape(16, 8, 512) - mi)
            p = p3.reshape(128, 512)
            li = jnp.sum(p3, axis=0)
            l = li if i == 0 else l + li
            for h in range(4):
                t = _dot(_unpack(vt[h * 16:(h + 1) * 16, _tile(i)]), p[:, _tile(h)].astype(BF16))
                pv[h] = t if i == 0 else pv[h] + t
            if i < j:
                yield
        l = jnp.sum(l, axis=0, keepdims=True)
        rows = []
        for h in range(4):
            gh = gate[g * 4 + h][0:1, :]
            num = nd[h * DH:(h + 1) * DH, _tile(j)]
            den = nd[128 + h:129 + h, _tile(j)] + 1e-6
            loc = pv[h] * ((1.0 - gh) / l[:, _tile(h)])
            rows.append(num * (gh / den) + (loc if h % 2 else pltpu.roll(loc, 64, 1)))
        of[e, _tile(j), :] = jnp.concatenate(rows, axis=0).T
        yield

    def keep_output(p, ch):
        r0 = ch * RC
        blocks = _lhs_blocks(of[0, r0:r0 + 128, :], of[1, r0:r0 + 128, :],
                             of[0, r0 + 128:r0 + 256, :], of[1, r0 + 128:r0 + 256, :])
        for i, b in enumerate(blocks):
            oc[p, i, ch * 64:(ch + 1) * 64, :] = _pack(b)

    def memory_pair(p, last):
        del ticks[:]
        if last:
            fill = _chain(memory_out(0, 0, p), memory_out(1, 0, TUNE["split"]))
            tail = memory_out(0, p, NPAIR)
        else:
            fill = _chain(memory_qk(p + 1, 0), memory_qk(p + 1, 1), memory_v(p + 1))
        for e, steps in enumerate(TUNE["plan_last" if last else "plan"].split("/")):
            g = 2 * p + e
            q, k, vt = (ref.at[p % 2 * 2 + e] for ref in (bq, bk, bv))
            todo, cur, nd, seen, corners, lag = [], None, None, [], {}, [0]
            for op in steps.split():
                if op == "f":
                    _run(fill, 1)
                elif op == "F":
                    _run(fill)
                elif op == "x":
                    _run(tail, 1)
                elif op == "X":
                    _run(tail)
                elif op[0] == "s":
                    j = int(op[1])
                    if j not in corners:
                        corners.update({i: corner(q, k, i) for i in (j, j ^ 1)})
                    todo.append((j, scores(q, k, j, corners[j])))
                elif op == "n":
                    nd = memory_read(g, q)
                elif op == "u":
                    memory_update(g, k, vt)
                elif op == "o":
                    keep_output(p, seen[-1] // 2)
                else:
                    lag[0] = int(op[1])
                    if cur is None or next(cur, "end") == "end":
                        j, st = todo.pop(0)
                        seen.append(j)
                        cur = attend(g, e, j, st, nd, vt, lag)
                        next(cur)
            assert len(seen) == L // 128 and next(cur, "end") == "end"
        return 0

    fetch_next = (rep == 1) & (seg < NSEG - 1)
    pl.when(fetch_next)(lambda: x_copy(seg + 1).start())

    def keys_stage():
        for c in range(NT):
            kb[c, 0:HALO, :] = kc[rep, c]
            vb[c, 0:HALO, :] = vc[rep, c]
        xn1 = _layernorm(xs[RC:L, :])
        xa[RC:L, :] = xn1
        in0, in1 = _row_blocks(xa[0:RC, :]), _row_blocks(xn1)
        _run(window_in(0, 0, held_for(in1, TUNE["due_norm"], in0)))
        _run(window_in(1, 0, lambda i: in1[i]))

    def window_stage():
        del ticks[:]
        a_in = [_row_blocks(xa[ch * RC:(ch + 1) * RC, :]) for ch in range(NCH)]
        due_probs, due_mix = iter(TUNE["due_probs"]), iter((0,) * (3 * NP) + TUNE["due_mix0"])
        seen = [0, 0]

        def held(ch, i):
            n, n2 = next(due_probs), next(due_mix)
            deps = [window_probs(*divmod(r, RC // 8))[1] for r in range(seen[0], seen[0] + n)]
            deps += [window_rows(0, r)[:, _tile(c)] for r in range(seen[1], seen[1] + n2) for c in range(NT)]
            seen[0] += n
            seen[1] += n2
            return before(deps, a_in[ch][i])
        for ch, m in ((0, 1), (1, 1), (0, 2), (1, 2)):
            _run(window_in(ch, m, functools.partial(held, ch)))
        o0, o1 = window_blocks(0), window_blocks(1)
        _run(window_out(0, held_for(o1, TUNE["due_mix1"], o0)))

        def memory_in(ch):
            blocks = [_pack(b) for b in _row_blocks(_layernorm(xs[ch * RC:(ch + 1) * RC, :]))]
            for i, b in enumerate(blocks):
                xb[i, ch * 64:(ch + 1) * 64, :] = b
            return blocks
        x0 = memory_in(0)
        _run(window_out(1, held_for([pltpu.bitcast(b, F32) for b in x0], TUNE["due_norm0"], o1)))
        for ch, blocks in enumerate((x0, memory_in(1))):
            _run(memory_qk(0, ch, blocks))
        _run(memory_v(0))
        for c in range(NT):
            kc[rep, c] = kb[c, L:L + HALO, :]
            vc[rep, c] = vb[c, L:L + HALO, :]

    def last_stage():
        memory_pair(NPAIR - 1, True)
        xn0 = _layernorm(xs[0:RC, :])
        xa[0:RC, :] = xn0
        counts, seen = iter(TUNE["due_next"]), [0]

        def hold(a):
            n = next(counts)
            deps = [xn0[r * 8:r * 8 + 8, _tile(c)] for r in range(seen[0], seen[0] + n) for c in (0, NT - 1)]
            seen[0] += n
            return before(deps, a)
        _run(memory_out(1, TUNE["split"], NPAIR, hold))

    keys_stage()
    pl.when(first_step)(_more_weights)
    window_stage()
    pl.when(first_step)(_last_weights)
    pl.when(jnp.logical_not(first_step))(lambda: wait_out(seg - 1 + rep))
    pl.when(fetch_next)(lambda: x_copy(seg + 1).wait())
    lax.fori_loop(0, NPAIR - 1, lambda p, carry: memory_pair(p, False), 0)
    last_stage()
    pl.when((seg == NSEG - 1) & (rep == 1))(lambda: wait_out(seg))


@jax.jit
def pallas_interleave_layers__sliding_local_dilated__memory_aug_infini_attn__prompt_kernel(
        A_x, A_wqkv, A_wo, B_x, B_wq, B_wk, B_wv, B_wo, B_beta):
    del B_x
    hbm = pl.BlockSpec(memory_space=pl.ANY)
    out = pl.pallas_call(
        _kernel,
        grid=(NSEG, 2),
        in_specs=[hbm, pl.BlockSpec((1, H), lambda s, r: (0, 0)), hbm, hbm, hbm, hbm, hbm, hbm],
        out_specs=hbm,
        out_shape=jax.ShapeDtypeStruct((S, D), BF16),
        scratch_shapes=[
            pltpu.VMEM((L, D), BF16),
            pltpu.VMEM((4 * NCH, 128, HD), BF16),
            pltpu.VMEM((6, D, HD), BF16),
            pltpu.VMEM((2, HD, D), BF16),
            pltpu.VMEM((3, NPAIR, D, 256), BF16),
            pltpu.VMEM((D, D), BF16),
            pltpu.VMEM((3, NP, NPAIR, WROWS, 128), U32),
            pltpu.VMEM((NP, NPAIR, WROWS, 128), U32),
            pltpu.VMEM((NPAIR, NP, HD // 2, 256), U32),
            pltpu.VMEM((NPAIR, NP, 64, HD), U32),
            pltpu.VMEM((NP, HD // 2, HD), U32),
            pltpu.VMEM((L, D), F32),
            pltpu.VMEM((L, D), F32),
            pltpu.VMEM((NP, L // 4, HD), U32),
            pltpu.VMEM((NT, L, 128), F32),
            pltpu.VMEM((NT, HALO + L, 128), F32),
            pltpu.VMEM((NT, HALO + L, 128), F32),
            pltpu.VMEM((2, NT, HALO, 128), F32),
            pltpu.VMEM((2, NT, HALO, 128), F32),
            pltpu.VMEM((2, L, 128), F32),
            pltpu.VMEM((NPAIR, NP, L // 4, 128), U32),
            pltpu.VMEM((4, L, 128), F32),
            pltpu.VMEM((4, L, 128), F32),
            pltpu.VMEM((4, 64, L), U32),
            pltpu.VMEM((2 * NT, 128, 128), F32),
            pltpu.VMEM((2 * NT, 8, 128), F32),
            pltpu.VMEM((H, 8, 128), F32),
            pltpu.VMEM((128, 256), F32),
            pltpu.SemaphoreType.DMA((30,)),
        ],
        compiler_params=pltpu.CompilerParams(
            dimension_semantics=("arbitrary", "arbitrary"),
            vmem_limit_bytes=110 * 2**20),
        name="interleave",
    )(A_x.reshape(S, D), B_beta.reshape(1, H), A_wqkv, A_wo, B_wq, B_wk, B_wv, B_wo)
    return out.reshape(1, S, D)
```

```python
import functools
import math

import jax
import jax.numpy as jnp
from jax import lax
from jax.experimental import pallas as pl
from jax.experimental.pallas import tpu as pltpu

S, D, H, DH = 2048, 1024, 32, 32
NSEG = 4
L = S // NSEG
W, DIL = 8, 2
HALO = 16
NT = D // 128
NPAIR = NT // 2
HD = D // 2
RC = 256
NCH = L // RC
NP = 7
PITCH = 17
WROWS = 16 * PITCH + 16
LOG2E = math.log2(math.e)
QSCALE = DH ** -0.5 * LOG2E
NEG = -1e9 * LOG2E
F32, BF16, U32 = jnp.float32, jnp.bfloat16, jnp.uint32

TUNE = dict(
    pace=((24, 1.05, 80, 0.75), (56, 1.1, 110, 0.1)),
    due_norm=(0, 2, 3, 4, 2, 2, 3),
    due_probs=(0, 0, 0, 0, 0, 0, 0, 0, 3, 3, 4, 5, 4, 4, 4, 5, 3, 4, 4, 4, 4, 4, 3, 3, 3, 0, 0, 0),
    due_mix0=(0, 0, 1, 5, 7, 5, 10),
    due_mix1=(0, 0, 4, 3, 4, 4, 0),
    due_norm0=(0, 0, 1, 1, 3, 0, 1),
    due_next=(0, 0, 1, 5, 1, 2, 10, 1, 2, 2, 0, 5, 3, 0),
    split=2,
    plan="f f s3 f f s2 f n f p3 f p3 f p3 f f p3 s1 p2 f f p3 s0 p3 f f p3 f f p4 f u f p3 "
         "/ f f s3 s2 n f p3 f p2 f p3 f f p4 s1 f f p4 f p3 f p2 o s0 p3 f f f f p4 u p2 f f o F",
    plan_last="f s0 s1 n p4 s2 f p4 f p3 s3 f p3 f p2 p2 f f p3 f p3 f p3 f f p3 f u "
              "/ s0 s1 f n f p3 s2 p3 f p3 o f s3 p5 f p3 p2 f f x p3 x p3 f f x p4 x p3 o f x f x u F X",
)


def _dot(a, b):
    return jnp.dot(a, b, preferred_element_type=F32)


def _dot_nt(a, b):
    return lax.dot_general(a, b, (((1,), (1,)), ((), ())), preferred_element_type=F32)


def _pack(x):
    return pltpu.bitcast(x.astype(BF16), U32)


def _unpack(x):
    return pltpu.bitcast(x, BF16)


def _tile(i):
    return slice(i * 128, (i + 1) * 128)


def _lhs_blocks(a11, a12, a21, a22):
    return [a11 + a22, a21 + a22, a11, a22, a11 + a12, a21 - a11, a12 - a22]


def _rhs_blocks(b11, b12, b21, b22):
    return [b11 + b22, b11, b12 - b22, b21 - b11, b22, b11 + b12, b21 + b22]


def _row_blocks(x):
    return _lhs_blocks(x[:128, :HD], x[:128, HD:], x[128:, :HD], x[128:, HD:])


def _block_matmul(prod, done):
    p3 = yield from prod(2)
    p5 = yield from prod(4)
    done(0, 1, p3 + p5)
    p2 = yield from prod(1)
    p4 = yield from prod(3)
    done(1, 0, p2 + p4)
    u, v = p4 - p5, p3 - p2
    p1 = yield from prod(0)
    u, v = u + p1, v + p1
    p7 = yield from prod(6)
    done(0, 0, u + p7)
    p6 = yield from prod(5)
    done(1, 1, v + p6)


def _whole(fn):
    def prod(i):
        y = fn(i)
        yield
        return y
    return prod


def _tiled(dot, nk, nn, tick):
    def prod(i):
        acc = [None] * nn
        for n in range(nn):
            for k in range(nk):
                t = dot(i, k, n)
                acc[n] = t if k == 0 else acc[n] + t
            tick(t)
            yield
        return jnp.concatenate(acc, axis=1)
    return prod


def _run(gen, n=None):
    k = 0
    while (n is None or k < n) and next(gen, "end") != "end":
        k += 1


def _chain(*gens):
    for g in gens:
        yield from g


def _layernorm(x):
    m = jnp.mean(x, axis=-1, keepdims=True)
    xc = x - m
    v = jnp.mean(xc * xc, axis=-1, keepdims=True)
    return xc * lax.rsqrt(v + 1e-5)


def _phi(t):
    return jnp.where(t > 0, t + 1.0, jnp.exp(t))


def _kernel(x_hbm, beta_ref, wqkv_hbm, woa_hbm, wq_hbm, wk_hbm, wv_hbm, wob_hbm, out_hbm,
            xin, xout, raw_a, raw_ao, raw_b, raw_bo, wa, woa, wqk, wvt, wob,
            xs, xa, xb, qb, kb, vb, kc, vc, of, oc, bq, bk, bv, mt, zs, gate, cmask, sems):
    seg = pl.program_id(0)
    rep = pl.program_id(1)
    first_step = (seg == 0) & (rep == 0)

    def window_copy(i):
        m, j = divmod(i, 2)
        if m < 3:
            c0 = (1, 0, 2)[m] * D + j * HD
            return pltpu.make_async_copy(wqkv_hbm.at[:, pl.ds(c0, HD)], raw_a.at[i], sems.at[i])
        return pltpu.make_async_copy(woa_hbm.at[pl.ds(j * HD, HD)], raw_ao.at[j], sems.at[i])

    def pair_copies(p):
        return [pltpu.make_async_copy(w.at[:, pl.ds(p * 256, 256)], raw_b.at[m, p], sems.at[8 + 3 * p + m])
                for m, w in enumerate((wq_hbm, wk_hbm, wv_hbm))]

    def late_copies():
        return ([c for p in range(1, NPAIR) for c in pair_copies(p)]
                + [pltpu.make_async_copy(wob_hbm, raw_bo, sems.at[20])])

    def x_copy(s):
        return pltpu.make_async_copy(x_hbm.at[pl.ds(pl.multiple_of(s * L, L), L)], xin, sems.at[21])

    def out_copy(s, ch, i, j):
        rows = pl.ds(pl.multiple_of(s * L + ch * RC + i * 128, 128), 128)
        n = ch * 4 + i * 2 + j
        return pltpu.make_async_copy(xout.at[n], out_hbm.at[rows, pl.ds(j * HD, HD)], sems.at[22 + n])

    def wait_out(s):
        for n in range(4 * NCH):
            out_copy(s, n // 4, n // 2 % 2, n % 2).wait()

    def selector(reorder):
        row = lax.broadcasted_iota(jnp.int32, (128, 128), 0)
        col = lax.broadcasted_iota(jnp.int32, (128, 128), 1)
        if reorder:
            row = (((row >> 5) & 1) * 2 + (row & 1)) * DH + (row >> 6) * 16 + ((row >> 1) & 15)
        return jnp.where(row == col, 1.0, 0.0).astype(BF16)

    def packed_blocks(*quad):
        quad = [pltpu.bitcast(b, U32) for b in quad]
        vals = [_unpack(b).astype(F32) for b in quad]
        out = []
        for blk in _rhs_blocks(*vals):
            same = [i for i, v in enumerate(vals) if v is blk]
            out.append(quad[same[0]] if same else _pack(blk))
        return out

    def arrive(piece, lo, hi):
        for i in range(lo, hi):
            @pl.when(piece == i)
            def _():
                window_copy(i).wait()
                for n in {0: (1,), 1: (2, 3, 4, 5)}.get(i, ()):
                    window_copy(n).start()

    def scatter(dst, t, blocks):
        for i, v in enumerate(blocks):
            v = _pack(v)
            for c in range(NPAIR):
                for hp in range(2):
                    dst(i, c)[pl.ds(t * 2 + hp, 16, stride=PITCH), :] = v[hp * 16:(hp + 1) * 16, _tile(c)]

    def prep_window_in(piece, carry):
        arrive(piece, 0, 6)
        for t in range(4):
            top = _dot_nt(selector(True), raw_a[piece, 0:HD, _tile(t)])
            bot = _dot_nt(selector(True), raw_a[piece, HD:D, _tile(t)])
            scatter(lambda i, c: wa.at[piece // 2, i, c], (piece % 2) * 4 + t,
                    _rhs_blocks(top[:64], top[64:], bot[:64], bot[64:]))
        return carry

    def prep_window_out(j, carry):
        arrive(6 + j, 6, 8)
        for t in range(4):
            y = _dot(selector(True), raw_ao[j, _tile(t), :])
            scatter(lambda i, c: woa.at[i, c], j * 4 + t,
                    _rhs_blocks(y[:64, :HD], y[:64, HD:], y[64:, :HD], y[64:, HD:]))
        return carry

    def prep_pair(p, carry):
        quad = [_dot_nt(selector(False), raw_b[2, p, kh * HD:(kh + 1) * HD, _tile(e)])
                for kh in range(2) for e in range(2)]
        for i, v in enumerate(_rhs_blocks(*quad)):
            wvt[p, i] = _pack(v)

        def rows_qk(j, c):
            for m in range(2):
                quad = [raw_b[m, p, pl.ds(pl.multiple_of(kh * HD + j * 64, 64), 64), _tile(e)]
                        for kh in range(2) for e in range(2)]
                for i, v in enumerate(packed_blocks(*quad)):
                    wqk[p, i, pl.ds(pl.multiple_of(j * 32, 32), 32), _tile(m)] = v
            return c
        return lax.fori_loop(0, HD // 64, rows_qk, carry)

    def prep_memory_out(t, carry):
        r0 = (t // 4) * 256 + (t % 4) * 32
        quad = [raw_bo[pl.ds(pl.multiple_of(r0 + e * 128, 32), 32), c:c + HD] for e in range(2) for c in (0, HD)]
        for i, v in enumerate(packed_blocks(*quad)):
            wob[i, pl.ds(pl.multiple_of(t * 16, 16), 16), :] = v
        return carry

    @pl.when(first_step)
    def _start():
        window_copy(0).start()
        x_copy(0).start()
        kc[...] = jnp.zeros(kc.shape, F32)
        vc[...] = jnp.zeros(vc.shape, F32)
        mt[...] = jnp.zeros(mt.shape, F32)
        zs[...] = jnp.zeros(zs.shape, F32)
        g_all = jax.nn.sigmoid(beta_ref[...].astype(F32))
        head = lax.broadcasted_iota(jnp.int32, (1, H), 1)
        for h in range(H):
            gate[h] = jnp.broadcast_to(jnp.sum(jnp.where(head == h, g_all, 0.0), axis=1, keepdims=True), (8, 128))
        kk = lax.broadcasted_iota(jnp.int32, (128, 256), 0)
        qq = lax.broadcasted_iota(jnp.int32, (128, 256), 1)
        qq = jnp.where(kk >= 64, qq | 64, jnp.where(qq < 128, qq ^ 64, qq)) & 127
        cmask[...] = jnp.where(qq < kk, NEG, 0.0).astype(F32)
        prep_window_in(0, 0)
        x_copy(0).wait()

        def load_rows(j, carry):
            rows = pl.ds(pl.multiple_of(j * 64, 64), 64)
            later = pl.ds(pl.multiple_of(RC + j * 64, 64), 64)
            x0 = xin[rows, :].astype(F32)
            xs[rows, :] = x0
            xa[rows, :] = _layernorm(x0)
            xs[later, :] = xin[later, :].astype(F32)
            return carry
        lax.fori_loop(0, RC // 64, load_rows, 0)
        prep_window_in(1, 0)

    def _more_weights():
        for c in [window_copy(6), window_copy(7)] + pair_copies(0):
            c.start()
        lax.fori_loop(2, 6, prep_window_in, 0)
        lax.fori_loop(0, 2, prep_window_out, 0)
        for c in late_copies():
            c.start()
        for c in pair_copies(0):
            c.wait()
        prep_pair(0, 0)

    def _last_weights():
        for c in late_copies():
            c.wait()
        lax.fori_loop(1, NPAIR, prep_pair, 0)
        lax.fori_loop(0, HD // 32, prep_memory_out, 0)

    ticks = []

    def tick(y):
        ticks.extend(y[0:8, c:c + 128] for c in range(0, y.shape[1], 128))
        return y

    def never():
        return cmask[0:8, 0:128] > 1.0

    def after(t, x):
        return x if t < 0 else jnp.where(never(), ticks[min(t, len(ticks) - 1)], x)

    def before(deps, a):
        if not deps:
            return a
        dep = functools.reduce(jnp.maximum, deps)
        head = jnp.where(never(), dep if a.dtype == F32 else pltpu.bitcast(dep, a.dtype), a[0:8, 0:128])
        if a.shape[1] > 128:
            head = jnp.concatenate([head, a[0:8, 128:]], axis=1)
        return jnp.concatenate([head, a[8:]], axis=0)

    def held_for(blocks, counts, lhs):
        counts, seen = iter(counts), [0]

        def held(i):
            n = next(counts)
            deps = [b[r * 8:r * 8 + 8, _tile(c)] for r in range(seen[0], seen[0] + n)
                    for b in blocks[-2:] for c in range(NPAIR)]
            seen[0] += n
            return before(deps, lhs[i])
        return held

    def reordered(ref):
        return _unpack(jnp.concatenate([jnp.concatenate(
            [ref[c, d * PITCH:d * PITCH + 16, :] for d in range(16)], axis=0) for c in range(NPAIR)], axis=1))

    def window_in(ch, m, lhs):
        dst, off = ((kb, HALO), (qb, 0), (vb, HALO))[m]

        def done(i, j, y):
            r0 = off + ch * RC + i * 128
            if m == 1:
                y = y * QSCALE
            for c in range(NPAIR):
                dst[j * NPAIR + c, r0:r0 + 128, :] = y[:, _tile(c)]
        return _block_matmul(
            _whole(lambda i: tick(_dot_nt(lhs(i).astype(BF16), reordered(wa.at[m, i])))), done)

    def taps(ref, c, r0, w):
        o0 = HALO + r0 - DIL * w
        return ref[c, o0:o0 + 8, :]

    def row_group(i):
        return i // 2 + (i % 2) * (RC // 16)

    @functools.cache
    def window_probs(ch, i):
        r0 = ch * RC + row_group(i) * 8
        t = int(TUNE["pace"][ch][0] + i * TUNE["pace"][ch][1])
        qs = [after(t, qb[c, r0:r0 + 8, :]) for c in range(NT)]
        logits = []
        for w in range(W):
            acc = functools.reduce(jnp.add, [qs[c] * taps(kb, c, r0, w) for c in range(NT)])
            acc = acc + pltpu.roll(acc, 64, 1)
            acc = acc + pltpu.roll(acc, 32, 1)
            if r0 < DIL * w:
                pos = seg * L + r0 + lax.broadcasted_iota(jnp.int32, (8, 128), 0)
                acc = jnp.where(pos >= DIL * w, acc, NEG)
            logits.append(acc)
        mx = functools.reduce(jnp.maximum, logits)
        es = [jnp.exp2(v - mx) for v in logits]
        return es, 1.0 / functools.reduce(jnp.add, es)

    @functools.cache
    def window_rows(ch, i):
        r0 = ch * RC + row_group(i) * 8
        es, inv = window_probs(ch, i)
        inv = after(int(TUNE["pace"][ch][2] + i * TUNE["pace"][ch][3]), inv)
        ps = [e * inv for e in es]
        return jnp.concatenate(
            [functools.reduce(jnp.add, [ps[w] * taps(vb, c, r0, w) for w in range(W)]) for c in range(NT)], axis=1)

    def window_blocks(ch):
        rows = [None] * (RC // 8)
        for i in range(RC // 8):
            rows[row_group(i)] = window_rows(ch, i)
        return _row_blocks(jnp.concatenate(rows, axis=0))

    def add_rows(ch):
        def done(i, j, y):
            r0 = ch * RC + i * 128
            xs[r0:r0 + 128, j * HD:(j + 1) * HD] += y
        return done

    def window_out(ch, lhs):
        return _block_matmul(
            _whole(lambda i: tick(_dot(lhs(i).astype(BF16), reordered(woa.at[i])))), add_rows(ch))

    def memory_qk(p, ch, lhs=None):
        def done(i, j, y):
            r0 = ch * RC + i * 128
            bq[p % 2 * 2 + j, r0:r0 + 128, :] = y[:, :128]
            bk[p % 2 * 2 + j, r0:r0 + 128, :] = y[:, 128:]
        if lhs is not None:
            return _block_matmul(_whole(lambda i: tick(_dot(_unpack(lhs[i]), _unpack(wqk[p, i])))), done)
        return _block_matmul(_tiled(
            lambda i, k, n: _dot(_unpack(xb[i, ch * 64:(ch + 1) * 64, _tile(k)]),
                                 _unpack(wqk[p, i, k * 64:(k + 1) * 64, _tile(n)])), 4, 2, tick), done)

    def memory_v(p):
        def done(i, j, y):
            for ch in range(NCH):
                c0 = ch * RC + i * 128
                bv[p % 2 * 2 + j, :, c0:c0 + 128] = _pack(y[:, _tile(ch)])
        return _block_matmul(_tiled(
            lambda i, k, n: _dot_nt(_unpack(wvt[p, i, :, _tile(k)]),
                                    _unpack(xb[i, n * 64:(n + 1) * 64, _tile(k)])), 4, NCH, tick), done)

    def finish_rows(ch):
        def done(i, j, y):
            idx = (slice(ch * RC + i * 128, ch * RC + (i + 1) * 128), slice(j * HD, (j + 1) * HD))
            xnew = xs[idx] + y
            xout[ch * 4 + i * 2 + j] = xnew.astype(BF16)
            out_copy(seg, ch, i, j).start()
            xs[idx] = jnp.where(rep == 0, xnew, xin[idx].astype(F32))
        return done

    def memory_out(ch, p0, p1, hold=lambda a: a):
        def prod(i):
            acc = None
            for p in range(p0, p1):
                t = _dot(_unpack(hold(oc[p, i, ch * 64:(ch + 1) * 64, :])), _unpack(wob[i, p * 64:(p + 1) * 64, :]))
                acc = t if acc is None else acc + t
                tick(t[:, 0:128])
                yield
            return acc
        return _block_matmul(prod, finish_rows(ch) if p1 == NPAIR else add_rows(ch))

    lane_head = lax.broadcasted_iota(jnp.int32, (1, 128), 1) // DH

    def head_queries(q, j):
        qh = [q[_tile(j), :] * jnp.where(lane_head == h, QSCALE, 0.0) for h in range(4)]
        return [(t[:64], t[64:]) for t in qh]

    def corner(q, k, j):
        qm = jnp.concatenate([hi for _, hi in head_queries(q, j)], axis=0)
        return _dot_nt(k[j * 128 + 64:(j + 1) * 128, :].astype(BF16), qm.astype(BF16))

    def scores(q, k, j, cor):
        nk = 128 * j + 64
        qm = jnp.concatenate([part for h, (lo, hi) in enumerate(head_queries(q, j))
                              for part in ((lo, hi) if h % 2 else (hi, lo))], axis=0)
        st = _dot_nt(k[0:nk, :].astype(BF16), qm.astype(BF16))
        for i in range(j + 1):
            tick(st[i * 128:i * 128 + 8, 0:128])
        diag = st[nk - 64:] + jnp.concatenate([cmask[0:64, :]] * 2, axis=1)
        st = diag if j == 0 else jnp.concatenate([st[:nk - 64], diag], axis=0)
        return st, cor + jnp.concatenate([cmask[64:128, 0:128]] * 2, axis=1)

    def memory_read(g, q):
        zrow = lax.broadcasted_iota(jnp.int32, (16, 128), 0)
        zl = jnp.where(zrow == lane_head, jnp.broadcast_to(zs[rep * NT + g, 0:1, :], (16, 128)), 0.0)
        return _dot_nt(jnp.concatenate([mt[rep * NT + g], zl], axis=0).astype(BF16), _phi(q[...]).astype(BF16))

    def memory_update(g, k, vt):
        pk = _phi(k[...])
        upd = functools.reduce(jnp.add, [
            _dot(_unpack(vt[:, _tile(i)]), pk[_tile(i)].astype(BF16)) for i in range(L // 128)])
        row_head = lax.broadcasted_iota(jnp.int32, (128, 128), 0) // DH
        mt[rep * NT + g] += jnp.where(row_head == lane_head, upd, 0.0)
        zs[rep * NT + g] += jnp.sum(jnp.sum(pk.reshape(L // 64, 64, 128), axis=0), axis=0, keepdims=True)

    def attend(g, e, j, st, nd, vt, lag):
        st, cor = st
        low = lax.broadcasted_iota(jnp.int32, (1, 128), 1) < 64
        own = [low if h % 2 == 0 else ~low for h in range(4)]
        mc = jnp.max(cor.reshape(8, 8, 256), axis=0)
        mx = jnp.max(st.reshape(-1, 8, 512), axis=0)
        mx = jnp.concatenate([jnp.where(own[h], jnp.maximum(mx[:, _tile(h)], mc[:, _tile(h // 2)]), mx[:, _tile(h)])
                              for h in range(4)], axis=1)
        mx = jnp.broadcast_to(jnp.max(mx, axis=0, keepdims=True), (8, 512))
        pv, l = [None] * 4, None
        for i in range(j + 1):
            mi = [after(len(ticks) - lag[0], mx[:, _tile(h)]) for h in range(4)]
            n = 128 if i < j else 64
            p3 = jnp.exp2(st[i * 128:i * 128 + n].reshape(n // 8, 8, 512) - jnp.concatenate(mi, axis=1))
            if i == j:
                pc = jnp.exp2(cor.reshape(8, 8, 256) - jnp.concatenate(
                    [jnp.where(low, mi[h], mi[h + 1]) for h in (0, 2)], axis=1))
                p3 = jnp.concatenate([p3, jnp.concatenate(
                    [jnp.where(own[h], pc[:, :, _tile(h // 2)], 0.0) for h in range(4)], axis=2)], axis=0)
            p = p3.reshape(128, 512)
            li = jnp.sum(p3, axis=0)
            l = li if i == 0 else l + li
            for h in range(4):
                t = _dot(_unpack(vt[h * 16:(h + 1) * 16, _tile(i)]), p[:, _tile(h)].astype(BF16))
                pv[h] = t if i == 0 else pv[h] + t
            if i < j:
                yield
        l = jnp.sum(l, axis=0, keepdims=True)
        rows = []
        for h in range(4):
            gh = gate[g * 4 + h][0:1, :]
            num = nd[h * DH:(h + 1) * DH, _tile(j)]
            den = nd[128 + h:129 + h, _tile(j)] + 1e-6
            loc = pv[h] * ((1.0 - gh) / l[:, _tile(h)])
            rows.append(num * (gh / den) + (loc if h % 2 else pltpu.roll(loc, 64, 1)))
        of[e, _tile(j), :] = jnp.concatenate(rows, axis=0).T
        yield

    def keep_output(p, ch):
        r0 = ch * RC
        blocks = _lhs_blocks(of[0, r0:r0 + 128, :], of[1, r0:r0 + 128, :],
                             of[0, r0 + 128:r0 + 256, :], of[1, r0 + 128:r0 + 256, :])
        for i, b in enumerate(blocks):
            oc[p, i, ch * 64:(ch + 1) * 64, :] = _pack(b)

    def memory_pair(p, last):
        del ticks[:]
        if last:
            fill = _chain(memory_out(0, 0, p), memory_out(1, 0, TUNE["split"]))
            tail = memory_out(0, p, NPAIR)
        else:
            fill = _chain(memory_qk(p + 1, 0), memory_qk(p + 1, 1), memory_v(p + 1))
        for e, steps in enumerate(TUNE["plan_last" if last else "plan"].split("/")):
            g = 2 * p + e
            q, k, vt = (ref.at[p % 2 * 2 + e] for ref in (bq, bk, bv))
            todo, cur, nd, seen, corners, lag = [], None, None, [], {}, [0]
            for op in steps.split():
                if op == "f":
                    _run(fill, 1)
                elif op == "F":
                    _run(fill)
                elif op == "x":
                    _run(tail, 1)
                elif op == "X":
                    _run(tail)
                elif op[0] == "s":
                    j = int(op[1])
                    if j not in corners:
                        corners.update({i: corner(q, k, i) for i in (j, j ^ 1)})
                    todo.append((j, scores(q, k, j, corners[j])))
                elif op == "n":
                    nd = memory_read(g, q)
                elif op == "u":
                    memory_update(g, k, vt)
                elif op == "o":
                    keep_output(p, seen[-1] // 2)
                else:
                    lag[0] = int(op[1])
                    if cur is None or next(cur, "end") == "end":
                        j, st = todo.pop(0)
                        seen.append(j)
                        cur = attend(g, e, j, st, nd, vt, lag)
                        next(cur)
            assert len(seen) == L // 128 and next(cur, "end") == "end"
        return 0

    fetch_next = (rep == 1) & (seg < NSEG - 1)
    pl.when(fetch_next)(lambda: x_copy(seg + 1).start())

    def keys_stage():
        for c in range(NT):
            kb[c, 0:HALO, :] = kc[rep, c]
            vb[c, 0:HALO, :] = vc[rep, c]
        xn1 = _layernorm(xs[RC:L, :])
        xa[RC:L, :] = xn1
        in0, in1 = _row_blocks(xa[0:RC, :]), _row_blocks(xn1)
        _run(window_in(0, 0, held_for(in1, TUNE["due_norm"], in0)))
        _run(window_in(1, 0, lambda i: in1[i]))

    def window_stage():
        del ticks[:]
        a_in = [_row_blocks(xa[ch * RC:(ch + 1) * RC, :]) for ch in range(NCH)]
        due_probs, due_mix = iter(TUNE["due_probs"]), iter((0,) * (3 * NP) + TUNE["due_mix0"])
        seen = [0, 0]

        def held(ch, i):
            n, n2 = next(due_probs), next(due_mix)
            deps = [window_probs(*divmod(r, RC // 8))[1] for r in range(seen[0], seen[0] + n)]
            deps += [window_rows(0, r)[:, _tile(c)] for r in range(seen[1], seen[1] + n2) for c in range(NT)]
            seen[0] += n
            seen[1] += n2
            return before(deps, a_in[ch][i])
        for ch, m in ((0, 1), (1, 1), (0, 2), (1, 2)):
            _run(window_in(ch, m, functools.partial(held, ch)))
        o0, o1 = window_blocks(0), window_blocks(1)
        _run(window_out(0, held_for(o1, TUNE["due_mix1"], o0)))

        def memory_in(ch):
            blocks = [_pack(b) for b in _row_blocks(_layernorm(xs[ch * RC:(ch + 1) * RC, :]))]
            for i, b in enumerate(blocks):
                xb[i, ch * 64:(ch + 1) * 64, :] = b
            return blocks
        x0 = memory_in(0)
        _run(window_out(1, held_for([pltpu.bitcast(b, F32) for b in x0], TUNE["due_norm0"], o1)))
        for ch, blocks in enumerate((x0, memory_in(1))):
            _run(memory_qk(0, ch, blocks))
        _run(memory_v(0))
        for c in range(NT):
            kc[rep, c] = kb[c, L:L + HALO, :]
            vc[rep, c] = vb[c, L:L + HALO, :]

    def last_stage():
        memory_pair(NPAIR - 1, True)
        xn0 = _layernorm(xs[0:RC, :])
        xa[0:RC, :] = xn0
        counts, seen = iter(TUNE["due_next"]), [0]

        def hold(a):
            n = next(counts)
            deps = [xn0[r * 8:r * 8 + 8, _tile(c)] for r in range(seen[0], seen[0] + n) for c in (0, NT - 1)]
            seen[0] += n
            return before(deps, a)
        _run(memory_out(1, TUNE["split"], NPAIR, hold))

    keys_stage()
    pl.when(first_step)(_more_weights)
    window_stage()
    pl.when(first_step)(_last_weights)
    pl.when(jnp.logical_not(first_step))(lambda: wait_out(seg - 1 + rep))
    pl.when(fetch_next)(lambda: x_copy(seg + 1).wait())
    lax.fori_loop(0, NPAIR - 1, lambda p, carry: memory_pair(p, False), 0)
    last_stage()
    pl.when((seg == NSEG - 1) & (rep == 1))(lambda: wait_out(seg))


@jax.jit
def pallas_interleave_layers__sliding_local_dilated__memory_aug_infini_attn__prompt_kernel(
        A_x, A_wqkv, A_wo, B_x, B_wq, B_wk, B_wv, B_wo, B_beta):
    del B_x
    hbm = pl.BlockSpec(memory_space=pl.ANY)
    out = pl.pallas_call(
        _kernel,
        grid=(NSEG, 2),
        in_specs=[hbm, pl.BlockSpec((1, H), lambda s, r: (0, 0)), hbm, hbm, hbm, hbm, hbm, hbm],
        out_specs=hbm,
        out_shape=jax.ShapeDtypeStruct((S, D), BF16),
        scratch_shapes=[
            pltpu.VMEM((L, D), BF16),
            pltpu.VMEM((4 * NCH, 128, HD), BF16),
            pltpu.VMEM((6, D, HD), BF16),
            pltpu.VMEM((2, HD, D), BF16),
            pltpu.VMEM((3, NPAIR, D, 256), BF16),
            pltpu.VMEM((D, D), BF16),
            pltpu.VMEM((3, NP, NPAIR, WROWS, 128), U32),
            pltpu.VMEM((NP, NPAIR, WROWS, 128), U32),
            pltpu.VMEM((NPAIR, NP, HD // 2, 256), U32),
            pltpu.VMEM((NPAIR, NP, 64, HD), U32),
            pltpu.VMEM((NP, HD // 2, HD), U32),
            pltpu.VMEM((L, D), F32),
            pltpu.VMEM((L, D), F32),
            pltpu.VMEM((NP, L // 4, HD), U32),
            pltpu.VMEM((NT, L, 128), F32),
            pltpu.VMEM((NT, HALO + L, 128), F32),
            pltpu.VMEM((NT, HALO + L, 128), F32),
            pltpu.VMEM((2, NT, HALO, 128), F32),
            pltpu.VMEM((2, NT, HALO, 128), F32),
            pltpu.VMEM((2, L, 128), F32),
            pltpu.VMEM((NPAIR, NP, L // 4, 128), U32),
            pltpu.VMEM((4, L, 128), F32),
            pltpu.VMEM((4, L, 128), F32),
            pltpu.VMEM((4, 64, L), U32),
            pltpu.VMEM((2 * NT, 128, 128), F32),
            pltpu.VMEM((2 * NT, 8, 128), F32),
            pltpu.VMEM((H, 8, 128), F32),
            pltpu.VMEM((128, 256), F32),
            pltpu.SemaphoreType.DMA((30,)),
        ],
        compiler_params=pltpu.CompilerParams(
            dimension_semantics=("arbitrary", "arbitrary"),
            vmem_limit_bytes=110 * 2**20),
        name="interleave",
    )(A_x.reshape(S, D), B_beta.reshape(1, H), A_wqkv, A_wo, B_wq, B_wk, B_wv, B_wo)
    return out.reshape(1, S, D)
```

```python
import functools
import math

import jax
import jax.numpy as jnp
from jax import lax
from jax.experimental import pallas as pl
from jax.experimental.pallas import tpu as pltpu

S, D, H, DH = 2048, 1024, 32, 32
NSEG = 4
L = S // NSEG
W, DIL = 8, 2
HALO = 16
NT = D // 128
NPAIR = NT // 2
HD = D // 2
RC = 256
NCH = L // RC
NP = 7
PITCH = 17
WROWS = 16 * PITCH + 16
LOG2E = math.log2(math.e)
QSCALE = DH ** -0.5 * LOG2E
NEG = -1e9 * LOG2E
F32, BF16, U32 = jnp.float32, jnp.bfloat16, jnp.uint32

TUNE = dict(
    pace=((24, 1.05, 80, 0.75), (56, 1.1, 110, 0.1)),
    due_norm=(0, 2, 3, 4, 2, 2, 3),
    due_probs=(0, 0, 0, 0, 0, 0, 0, 0, 3, 3, 4, 5, 4, 4, 4, 4, 4, 4, 4, 4, 4, 4, 3, 3, 3, 0, 0, 0),
    due_mix0=(0, 0, 1, 5, 7, 5, 10),
    due_mix1=(0, 0, 4, 5, 4, 2, 0),
    due_norm0=(0, 0, 1, 1, 3, 0, 1),
    due_next=(0, 0, 1, 5, 1, 2, 10, 1, 2, 2, 0, 5, 3, 0),
    split=2,
    plan="f f s3 f f s2 f n f p3 f p3 f p3 f f p3 s1 p2 f f p3 s0 p3 f f p3 f f p4 f u f p3 "
         "/ f f s3 s2 n f p3 f p2 f p3 f f p4 s1 f f p4 f p3 f p2 o s0 p3 f f f f p4 u p2 f f o F",
    plan_last="f s0 s1 n p4 s2 f p4 f p3 s3 f p3 f p2 p2 f f p3 f p3 f p3 f f p3 f u "
              "/ s0 s1 f n f p3 s2 p3 f p3 o f s3 p5 f p3 p2 f f x p3 x p3 f f x p4 x p3 o f x f x u F X",
)


def _dot(a, b):
    return jnp.dot(a, b, preferred_element_type=F32)


def _dot_nt(a, b):
    return lax.dot_general(a, b, (((1,), (1,)), ((), ())), preferred_element_type=F32)


def _pack(x):
    return pltpu.bitcast(x.astype(BF16), U32)


def _unpack(x):
    return pltpu.bitcast(x, BF16)


def _tile(i):
    return slice(i * 128, (i + 1) * 128)


def _lhs_blocks(a11, a12, a21, a22):
    return [a11 + a22, a21 + a22, a11, a22, a11 + a12, a21 - a11, a12 - a22]


def _rhs_blocks(b11, b12, b21, b22):
    return [b11 + b22, b11, b12 - b22, b21 - b11, b22, b11 + b12, b21 + b22]


def _row_blocks(x):
    return _lhs_blocks(x[:128, :HD], x[:128, HD:], x[128:, :HD], x[128:, HD:])


def _block_matmul(prod, done):
    p3 = yield from prod(2)
    p5 = yield from prod(4)
    done(0, 1, p3 + p5)
    p2 = yield from prod(1)
    p4 = yield from prod(3)
    done(1, 0, p2 + p4)
    u, v = p4 - p5, p3 - p2
    p1 = yield from prod(0)
    u, v = u + p1, v + p1
    p7 = yield from prod(6)
    done(0, 0, u + p7)
    p6 = yield from prod(5)
    done(1, 1, v + p6)


def _whole(fn):
    def prod(i):
        y = fn(i)
        yield
        return y
    return prod


def _tiled(dot, nk, nn, tick):
    def prod(i):
        acc = [None] * nn
        for n in range(nn):
            for k in range(nk):
                t = dot(i, k, n)
                acc[n] = t if k == 0 else acc[n] + t
            tick(t)
            yield
        return jnp.concatenate(acc, axis=1)
    return prod


def _run(gen, n=None):
    k = 0
    while (n is None or k < n) and next(gen, "end") != "end":
        k += 1


def _chain(*gens):
    for g in gens:
        yield from g


def _layernorm(x):
    m = jnp.mean(x, axis=-1, keepdims=True)
    xc = x - m
    v = jnp.mean(xc * xc, axis=-1, keepdims=True)
    return xc * lax.rsqrt(v + 1e-5)


def _phi(t):
    return jnp.where(t > 0, t + 1.0, jnp.exp(t))


def _kernel(x_hbm, beta_ref, wqkv_hbm, woa_hbm, wq_hbm, wk_hbm, wv_hbm, wob_hbm, out_hbm,
            xin, xout, raw_a, raw_ao, raw_b, raw_bo, wa, woa, wqk, wvt, wob,
            xs, xa, xb, qb, kb, vb, kc, vc, of, oc, bq, bk, bv, mt, zs, gate, cmask, sems):
    seg = pl.program_id(0)
    rep = pl.program_id(1)
    first_step = (seg == 0) & (rep == 0)

    def window_copy(i):
        m, j = divmod(i, 2)
        if m < 3:
            c0 = (1, 0, 2)[m] * D + j * HD
            return pltpu.make_async_copy(wqkv_hbm.at[:, pl.ds(c0, HD)], raw_a.at[i], sems.at[i])
        return pltpu.make_async_copy(woa_hbm.at[pl.ds(j * HD, HD)], raw_ao.at[j], sems.at[i])

    def pair_copies(p):
        return [pltpu.make_async_copy(w.at[:, pl.ds(p * 256, 256)], raw_b.at[m, p], sems.at[8 + 3 * p + m])
                for m, w in enumerate((wq_hbm, wk_hbm, wv_hbm))]

    def late_copies():
        return ([c for p in range(1, NPAIR) for c in pair_copies(p)]
                + [pltpu.make_async_copy(wob_hbm, raw_bo, sems.at[20])])

    def x_copy(s):
        return pltpu.make_async_copy(x_hbm.at[pl.ds(pl.multiple_of(s * L, L), L)], xin, sems.at[21])

    def out_copy(s, ch, i, j):
        rows = pl.ds(pl.multiple_of(s * L + ch * RC + i * 128, 128), 128)
        n = ch * 4 + i * 2 + j
        return pltpu.make_async_copy(xout.at[n], out_hbm.at[rows, pl.ds(j * HD, HD)], sems.at[22 + n])

    def wait_out(s):
        for n in range(4 * NCH):
            out_copy(s, n // 4, n // 2 % 2, n % 2).wait()

    def selector(reorder):
        row = lax.broadcasted_iota(jnp.int32, (128, 128), 0)
        col = lax.broadcasted_iota(jnp.int32, (128, 128), 1)
        if reorder:
            row = (((row >> 5) & 1) * 2 + (row & 1)) * DH + (row >> 6) * 16 + ((row >> 1) & 15)
        return jnp.where(row == col, 1.0, 0.0).astype(BF16)

    def packed_blocks(*quad):
        quad = [pltpu.bitcast(b, U32) for b in quad]
        vals = [_unpack(b).astype(F32) for b in quad]
        out = []
        for blk in _rhs_blocks(*vals):
            same = [i for i, v in enumerate(vals) if v is blk]
            out.append(quad[same[0]] if same else _pack(blk))
        return out

    def arrive(piece, lo, hi):
        for i in range(lo, hi):
            @pl.when(piece == i)
            def _():
                window_copy(i).wait()
                for n in {0: (1,), 1: (2, 3, 4, 5)}.get(i, ()):
                    window_copy(n).start()

    def scatter(dst, t, blocks):
        for i, v in enumerate(blocks):
            v = _pack(v)
            for c in range(NPAIR):
                for hp in range(2):
                    dst(i, c)[pl.ds(t * 2 + hp, 16, stride=PITCH), :] = v[hp * 16:(hp + 1) * 16, _tile(c)]

    def prep_window_in(piece, carry):
        arrive(piece, 0, 6)
        for t in range(4):
            top = _dot_nt(selector(True), raw_a[piece, 0:HD, _tile(t)])
            bot = _dot_nt(selector(True), raw_a[piece, HD:D, _tile(t)])
            scatter(lambda i, c: wa.at[piece >> 1, i, c], (piece & 1) * 4 + t,
                    _rhs_blocks(top[:64], top[64:], bot[:64], bot[64:]))
        return carry

    def prep_window_out(j, carry):
        arrive(6 + j, 6, 8)
        for t in range(4):
            y = _dot(selector(True), raw_ao[j, _tile(t), :])
            scatter(lambda i, c: woa.at[i, c], j * 4 + t,
                    _rhs_blocks(y[:64, :HD], y[:64, HD:], y[64:, :HD], y[64:, HD:]))
        return carry

    def prep_pair(p, carry):
        quad = [_dot_nt(selector(False), raw_b[2, p, kh * HD:(kh + 1) * HD, _tile(e)])
                for kh in range(2) for e in range(2)]
        for i, v in enumerate(_rhs_blocks(*quad)):
            wvt[p, i] = _pack(v)

        def rows_qk(j, c):
            for m in range(2):
                quad = [raw_b[m, p, pl.ds(pl.multiple_of(kh * HD + j * 64, 64), 64), _tile(e)]
                        for kh in range(2) for e in range(2)]
                for i, v in enumerate(packed_blocks(*quad)):
                    wqk[p, i, pl.ds(pl.multiple_of(j * 32, 32), 32), _tile(m)] = v
            return c
        return lax.fori_loop(0, HD // 64, rows_qk, carry)

    def prep_memory_out(t, carry):
        r0 = (t // 4) * 256 + (t % 4) * 32
        quad = [raw_bo[pl.ds(pl.multiple_of(r0 + e * 128, 32), 32), c:c + HD] for e in range(2) for c in (0, HD)]
        for i, v in enumerate(packed_blocks(*quad)):
            wob[i, pl.ds(pl.multiple_of(t * 16, 16), 16), :] = v
        return carry

    @pl.when(first_step)
    def _start():
        window_copy(0).start()
        x_copy(0).start()
        kc[...] = jnp.zeros(kc.shape, F32)
        vc[...] = jnp.zeros(vc.shape, F32)
        mt[...] = jnp.zeros(mt.shape, F32)
        zs[...] = jnp.zeros(zs.shape, F32)
        g_all = jax.nn.sigmoid(beta_ref[...].astype(F32))
        head = lax.broadcasted_iota(jnp.int32, (1, H), 1)
        for h in range(H):
            gate[h] = jnp.broadcast_to(jnp.sum(jnp.where(head == h, g_all, 0.0), axis=1, keepdims=True), (8, 128))
        kk = lax.broadcasted_iota(jnp.int32, (128, 256), 0)
        qq = lax.broadcasted_iota(jnp.int32, (128, 256), 1)
        qq = jnp.where(kk >= 64, qq | 64, jnp.where(qq < 128, qq ^ 64, qq)) & 127
        cmask[...] = jnp.where(qq < kk, NEG, 0.0).astype(F32)
        prep_window_in(0, 0)
        x_copy(0).wait()

        def load_rows(j, carry):
            rows = pl.ds(pl.multiple_of(j * 64, 64), 64)
            later = pl.ds(pl.multiple_of(RC + j * 64, 64), 64)
            x0 = xin[rows, :].astype(F32)
            xs[rows, :] = x0
            xa[rows, :] = _layernorm(x0)
            xs[later, :] = xin[later, :].astype(F32)
            return carry
        lax.fori_loop(0, RC // 64, load_rows, 0)
        prep_window_in(1, 0)

    def _more_weights():
        for c in [window_copy(6), window_copy(7)] + pair_copies(0):
            c.start()
        lax.fori_loop(2, 6, prep_window_in, 0)
        lax.fori_loop(0, 2, prep_window_out, 0)
        for c in late_copies():
            c.start()
        for c in pair_copies(0):
            c.wait()
        prep_pair(0, 0)

    def _last_weights():
        for c in late_copies():
            c.wait()
        lax.fori_loop(1, NPAIR, prep_pair, 0)
        lax.fori_loop(0, HD // 32, prep_memory_out, 0)

    ticks = []

    def tick(y):
        ticks.extend(y[0:8, c:c + 128] for c in range(0, y.shape[1], 128))
        return y

    def never():
        return cmask[0:8, 0:128] > 1.0

    def after(t, x):
        return x if t < 0 else jnp.where(never(), ticks[min(t, len(ticks) - 1)], x)

    def before(deps, a):
        if not deps:
            return a
        dep = functools.reduce(jnp.maximum, deps)
        head = jnp.where(never(), dep if a.dtype == F32 else pltpu.bitcast(dep, a.dtype), a[0:8, 0:128])
        if a.shape[1] > 128:
            head = jnp.concatenate([head, a[0:8, 128:]], axis=1)
        return jnp.concatenate([head, a[8:]], axis=0)

    def held_for(blocks, counts, lhs):
        counts, seen = iter(counts), [0]

        def held(i):
            n = next(counts)
            deps = [b[r * 8:r * 8 + 8, _tile(c)] for r in range(seen[0], seen[0] + n)
                    for b in blocks[-2:] for c in range(NPAIR)]
            seen[0] += n
            return before(deps, lhs[i])
        return held

    def reordered(ref):
        w = jnp.concatenate([ref[:, d * PITCH:d * PITCH + 16, :] for d in range(16)], axis=1)
        return _unpack(jnp.concatenate([w[c] for c in range(NPAIR)], axis=1))

    def window_in(ch, m, lhs):
        dst, off = ((kb, HALO), (qb, 0), (vb, HALO))[m]

        def done(i, j, y):
            r0 = off + ch * RC + i * 128
            if m == 1:
                y = y * QSCALE
            for c in range(NPAIR):
                dst[j * NPAIR + c, r0:r0 + 128, :] = y[:, _tile(c)]
        return _block_matmul(
            _whole(lambda i: tick(_dot_nt(lhs(i).astype(BF16), reordered(wa.at[m, i])))), done)

    def taps(ref, r0, w):
        o0 = HALO + r0 - DIL * w
        return ref[:, o0:o0 + 8, :]

    def row_group(i):
        return i // 2 + (i % 2) * (RC // 16)

    @functools.cache
    def window_probs(ch, i):
        r0 = ch * RC + row_group(i) * 8
        t = int(TUNE["pace"][ch][0] + i * TUNE["pace"][ch][1])
        q = after(t, qb[:, r0:r0 + 8, :])
        logits = []
        for w in range(W):
            acc = jnp.sum(q * taps(kb, r0, w), axis=0)
            acc = acc + pltpu.roll(acc, 64, 1)
            acc = acc + pltpu.roll(acc, 32, 1)
            if r0 < DIL * w:
                pos = seg * L + r0 + lax.broadcasted_iota(jnp.int32, (8, 128), 0)
                acc = jnp.where(pos >= DIL * w, acc, NEG)
            logits.append(acc)
        mx = functools.reduce(jnp.maximum, logits)
        es = [jnp.exp2(v - mx) for v in logits]
        return es, 1.0 / functools.reduce(jnp.add, es)

    @functools.cache
    def window_rows(ch, i):
        r0 = ch * RC + row_group(i) * 8
        es, inv = window_probs(ch, i)
        inv = after(int(TUNE["pace"][ch][2] + i * TUNE["pace"][ch][3]), inv)
        ps = [e * inv for e in es]
        return functools.reduce(jnp.add, [ps[w] * taps(vb, r0, w) for w in range(W)])

    def window_blocks(ch):
        rows = [None] * (RC // 8)
        for i in range(RC // 8):
            rows[row_group(i)] = window_rows(ch, i)
        o = jnp.concatenate(rows, axis=1)
        return _row_blocks(jnp.concatenate([o[c] for c in range(NT)], axis=1))

    def add_rows(ch):
        def done(i, j, y):
            r0 = ch * RC + i * 128
            xs[r0:r0 + 128, j * HD:(j + 1) * HD] += y
        return done

    def window_out(ch, lhs):
        return _block_matmul(
            _whole(lambda i: tick(_dot(lhs(i).astype(BF16), reordered(woa.at[i])))), add_rows(ch))

    def memory_qk(p, ch, lhs=None):
        def done(i, j, y):
            r0 = ch * RC + i * 128
            bq[(p & 1) * 2 + j, r0:r0 + 128, :] = y[:, :128]
            bk[(p & 1) * 2 + j, r0:r0 + 128, :] = y[:, 128:]
        if lhs is not None:
            return _block_matmul(_whole(lambda i: tick(_dot(_unpack(lhs[i]), _unpack(wqk[p, i])))), done)
        return _block_matmul(_tiled(
            lambda i, k, n: _dot(_unpack(xb[i, ch * 64:(ch + 1) * 64, _tile(k)]),
                                 _unpack(wqk[p, i, k * 64:(k + 1) * 64, _tile(n)])), 4, 2, tick), done)

    def memory_v(p):
        def done(i, j, y):
            for ch in range(NCH):
                c0 = ch * RC + i * 128
                bv[(p & 1) * 2 + j, :, c0:c0 + 128] = _pack(y[:, _tile(ch)])
        return _block_matmul(_tiled(
            lambda i, k, n: _dot_nt(_unpack(wvt[p, i, :, _tile(k)]),
                                    _unpack(xb[i, n * 64:(n + 1) * 64, _tile(k)])), 4, NCH, tick), done)

    def finish_rows(ch):
        def done(i, j, y):
            idx = (slice(ch * RC + i * 128, ch * RC + (i + 1) * 128), slice(j * HD, (j + 1) * HD))
            xnew = xs[idx] + y
            xout[ch * 4 + i * 2 + j] = xnew.astype(BF16)
            out_copy(seg, ch, i, j).start()
            xs[idx] = jnp.where(rep == 0, xnew, xin[idx].astype(F32))
        return done

    def memory_out(ch, p0, p1, hold=lambda a: a):
        def prod(i):
            acc = None
            for p in range(p0, p1):
                t = _dot(_unpack(hold(oc[p, i, ch * 64:(ch + 1) * 64, :])), _unpack(wob[i, p * 64:(p + 1) * 64, :]))
                acc = t if acc is None else acc + t
                tick(t[:, 0:128])
                yield
            return acc
        return _block_matmul(prod, finish_rows(ch) if p1 == NPAIR else add_rows(ch))

    lane_head = lax.broadcasted_iota(jnp.int32, (1, 128), 1) >> 5

    def head_queries(q, j):
        qh = [q[_tile(j), :] * jnp.where(lane_head == h, QSCALE, 0.0) for h in range(4)]
        return [(t[:64], t[64:]) for t in qh]

    def corner(q, k, j):
        qm = jnp.concatenate([hi for _, hi in head_queries(q, j)], axis=0)
        return _dot_nt(k[j * 128 + 64:(j + 1) * 128, :].astype(BF16), qm.astype(BF16))

    def scores(q, k, j, cor):
        nk = 128 * j + 64
        qm = jnp.concatenate([part for h, (lo, hi) in enumerate(head_queries(q, j))
                              for part in ((lo, hi) if h % 2 else (hi, lo))], axis=0)
        st = _dot_nt(k[0:nk, :].astype(BF16), qm.astype(BF16))
        for i in range(j + 1):
            tick(st[i * 128:i * 128 + 8, 0:128])
        diag = st[nk - 64:] + jnp.concatenate([cmask[0:64, :]] * 2, axis=1)
        st = diag if j == 0 else jnp.concatenate([st[:nk - 64], diag], axis=0)
        return st, cor + jnp.concatenate([cmask[64:128, 0:128]] * 2, axis=1)

    def memory_read(g, q):
        zrow = lax.broadcasted_iota(jnp.int32, (16, 128), 0)
        zl = jnp.where(zrow == lane_head, jnp.broadcast_to(zs[rep * NT + g, 0:1, :], (16, 128)), 0.0)
        return _dot_nt(jnp.concatenate([mt[rep * NT + g], zl], axis=0).astype(BF16), _phi(q[...]).astype(BF16))

    def memory_update(g, k, vt):
        pk = _phi(k[...])
        upd = functools.reduce(jnp.add, [
            _dot(_unpack(vt[:, _tile(i)]), pk[_tile(i)].astype(BF16)) for i in range(L // 128)])
        row_head = lax.broadcasted_iota(jnp.int32, (128, 128), 0) >> 5
        mt[rep * NT + g] += jnp.where(row_head == lane_head, upd, 0.0)
        zs[rep * NT + g] += jnp.sum(jnp.sum(pk.reshape(L // 64, 64, 128), axis=0), axis=0, keepdims=True)

    def attend(g, e, j, st, nd, vt, lag):
        st, cor = st
        low = lax.broadcasted_iota(jnp.int32, (1, 128), 1) < 64
        own = [low if h % 2 == 0 else ~low for h in range(4)]
        mc = jnp.max(cor.reshape(8, 8, 256), axis=0)
        mx = jnp.max(st.reshape(-1, 8, 512), axis=0)
        mx = jnp.concatenate([jnp.where(own[h], jnp.maximum(mx[:, _tile(h)], mc[:, _tile(h // 2)]), mx[:, _tile(h)])
                              for h in range(4)], axis=1)
        mx = jnp.broadcast_to(jnp.max(mx, axis=0, keepdims=True), (8, 512))
        pv, l = [None] * 4, None
        for i in range(j + 1):
            mi = [after(len(ticks) - lag[0], mx[:, _tile(h)]) for h in range(4)]
            n = 128 if i < j else 64
            p3 = jnp.exp2(st[i * 128:i * 128 + n].reshape(n // 8, 8, 512) - jnp.concatenate(mi, axis=1))
            if i == j:
                pc = jnp.exp2(cor.reshape(8, 8, 256) - jnp.concatenate(
                    [jnp.where(low, mi[h], mi[h + 1]) for h in (0, 2)], axis=1))
                p3 = jnp.concatenate([p3, jnp.concatenate(
                    [jnp.where(own[h], pc[:, :, _tile(h // 2)], 0.0) for h in range(4)], axis=2)], axis=0)
            p = p3.reshape(128, 512)
            li = jnp.sum(p3, axis=0)
            l = li if i == 0 else l + li
            for h in range(4):
                t = _dot(_unpack(vt[h * 16:(h + 1) * 16, _tile(i)]), p[:, _tile(h)].astype(BF16))
                pv[h] = t if i == 0 else pv[h] + t
            if i < j:
                yield
        l = jnp.sum(l, axis=0, keepdims=True)
        rows = []
        for h in range(4):
            gh = gate[g * 4 + h][0:1, :]
            num = nd[h * DH:(h + 1) * DH, _tile(j)]
            den = nd[128 + h:129 + h, _tile(j)] + 1e-6
            loc = pv[h] * ((1.0 - gh) / l[:, _tile(h)])
            rows.append(num * (gh / den) + (loc if h % 2 else pltpu.roll(loc, 64, 1)))
        of[e, _tile(j), :] = jnp.concatenate(rows, axis=0).T
        yield

    def keep_output(p, ch):
        r0 = ch * RC
        blocks = _lhs_blocks(of[0, r0:r0 + 128, :], of[1, r0:r0 + 128, :],
                             of[0, r0 + 128:r0 + 256, :], of[1, r0 + 128:r0 + 256, :])
        for i, b in enumerate(blocks):
            oc[p, i, ch * 64:(ch + 1) * 64, :] = _pack(b)

    def memory_pair(p, last):
        del ticks[:]
        if last:
            fill = _chain(memory_out(0, 0, p), memory_out(1, 0, TUNE["split"]))
            tail = memory_out(0, p, NPAIR)
        else:
            fill = _chain(memory_qk(p + 1, 0), memory_qk(p + 1, 1), memory_v(p + 1))
        for e, steps in enumerate(TUNE["plan_last" if last else "plan"].split("/")):
            g = 2 * p + e
            q, k, vt = (ref.at[(p & 1) * 2 + e] for ref in (bq, bk, bv))
            todo, cur, nd, seen, corners, lag = [], None, None, [], {}, [0]
            for op in steps.split():
                if op == "f":
                    _run(fill, 1)
                elif op == "F":
                    _run(fill)
                elif op == "x":
                    _run(tail, 1)
                elif op == "X":
                    _run(tail)
                elif op[0] == "s":
                    j = int(op[1])
                    if j not in corners:
                        corners.update({i: corner(q, k, i) for i in (j, j ^ 1)})
                    todo.append((j, scores(q, k, j, corners[j])))
                elif op == "n":
                    nd = memory_read(g, q)
                elif op == "u":
                    memory_update(g, k, vt)
                elif op == "o":
                    keep_output(p, seen[-1] // 2)
                else:
                    lag[0] = int(op[1])
                    if cur is None or next(cur, "end") == "end":
                        j, st = todo.pop(0)
                        seen.append(j)
                        cur = attend(g, e, j, st, nd, vt, lag)
                        next(cur)
            assert len(seen) == L // 128 and next(cur, "end") == "end"
        return 0

    fetch_next = (rep == 1) & (seg < NSEG - 1)
    pl.when(fetch_next)(lambda: x_copy(seg + 1).start())

    def keys_stage():
        for c in range(NT):
            kb[c, 0:HALO, :] = kc[rep, c]
            vb[c, 0:HALO, :] = vc[rep, c]
        xn1 = _layernorm(xs[RC:L, :])
        xa[RC:L, :] = xn1
        in0, in1 = _row_blocks(xa[0:RC, :]), _row_blocks(xn1)
        _run(window_in(0, 0, held_for(in1, TUNE["due_norm"], in0)))
        _run(window_in(1, 0, lambda i: in1[i]))

    def window_stage():
        del ticks[:]
        a_in = [_row_blocks(xa[ch * RC:(ch + 1) * RC, :]) for ch in range(NCH)]
        due_probs, due_mix = iter(TUNE["due_probs"]), iter((0,) * (3 * NP) + TUNE["due_mix0"])
        seen = [0, 0]

        def held(ch, i):
            n, n2 = next(due_probs), next(due_mix)
            deps = [window_probs(*divmod(r, RC // 8))[1] for r in range(seen[0], seen[0] + n)]
            deps += [window_rows(0, r)[c] for r in range(seen[1], seen[1] + n2) for c in range(NT)]
            seen[0] += n
            seen[1] += n2
            return before(deps, a_in[ch][i])
        for ch, m in ((0, 1), (1, 1), (0, 2), (1, 2)):
            _run(window_in(ch, m, functools.partial(held, ch)))
        o0, o1 = window_blocks(0), window_blocks(1)
        _run(window_out(0, held_for(o1, TUNE["due_mix1"], o0)))

        def memory_in(ch):
            blocks = [_pack(b) for b in _row_blocks(_layernorm(xs[ch * RC:(ch + 1) * RC, :]))]
            for i, b in enumerate(blocks):
                xb[i, ch * 64:(ch + 1) * 64, :] = b
            return blocks
        x0 = memory_in(0)
        _run(window_out(1, held_for([pltpu.bitcast(b, F32) for b in x0], TUNE["due_norm0"], o1)))
        for ch, blocks in enumerate((x0, memory_in(1))):
            _run(memory_qk(0, ch, blocks))
        _run(memory_v(0))
        for c in range(NT):
            kc[rep, c] = kb[c, L:L + HALO, :]
            vc[rep, c] = vb[c, L:L + HALO, :]

    def last_stage():
        memory_pair(NPAIR - 1, True)
        xn0 = _layernorm(xs[0:RC, :])
        xa[0:RC, :] = xn0
        counts, seen = iter(TUNE["due_next"]), [0]

        def hold(a):
            n = next(counts)
            deps = [xn0[r * 8:r * 8 + 8, _tile(c)] for r in range(seen[0], seen[0] + n) for c in (0, NT - 1)]
            seen[0] += n
            return before(deps, a)
        _run(memory_out(1, TUNE["split"], NPAIR, hold))

    keys_stage()
    pl.when(first_step)(_more_weights)
    window_stage()
    pl.when(first_step)(_last_weights)
    pl.when(jnp.logical_not(first_step))(lambda: wait_out(seg - 1 + rep))
    pl.when(fetch_next)(lambda: x_copy(seg + 1).wait())
    lax.fori_loop(0, NPAIR - 1, lambda p, carry: memory_pair(p, False), 0)
    last_stage()
    pl.when((seg == NSEG - 1) & (rep == 1))(lambda: wait_out(seg))


@jax.jit
def pallas_interleave_layers__sliding_local_dilated__memory_aug_infini_attn__prompt_kernel(
        A_x, A_wqkv, A_wo, B_x, B_wq, B_wk, B_wv, B_wo, B_beta):
    del B_x
    hbm = pl.BlockSpec(memory_space=pl.ANY)
    out = pl.pallas_call(
        _kernel,
        grid=(NSEG, 2),
        in_specs=[hbm, pl.BlockSpec((1, H), lambda s, r: (0, 0)), hbm, hbm, hbm, hbm, hbm, hbm],
        out_specs=hbm,
        out_shape=jax.ShapeDtypeStruct((S, D), BF16),
        scratch_shapes=[
            pltpu.VMEM((L, D), BF16),
            pltpu.VMEM((4 * NCH, 128, HD), BF16),
            pltpu.VMEM((6, D, HD), BF16),
            pltpu.VMEM((2, HD, D), BF16),
            pltpu.VMEM((3, NPAIR, D, 256), BF16),
            pltpu.VMEM((D, D), BF16),
            pltpu.VMEM((3, NP, NPAIR, WROWS, 128), U32),
            pltpu.VMEM((NP, NPAIR, WROWS, 128), U32),
            pltpu.VMEM((NPAIR, NP, HD // 2, 256), U32),
            pltpu.VMEM((NPAIR, NP, 64, HD), U32),
            pltpu.VMEM((NP, HD // 2, HD), U32),
            pltpu.VMEM((L, D), F32),
            pltpu.VMEM((L, D), F32),
            pltpu.VMEM((NP, L // 4, HD), U32),
            pltpu.VMEM((NT, L, 128), F32),
            pltpu.VMEM((NT, HALO + L, 128), F32),
            pltpu.VMEM((NT, HALO + L, 128), F32),
            pltpu.VMEM((2, NT, HALO, 128), F32),
            pltpu.VMEM((2, NT, HALO, 128), F32),
            pltpu.VMEM((2, L, 128), F32),
            pltpu.VMEM((NPAIR, NP, L // 4, 128), U32),
            pltpu.VMEM((4, L, 128), F32),
            pltpu.VMEM((4, L, 128), F32),
            pltpu.VMEM((4, 64, L), U32),
            pltpu.VMEM((2 * NT, 128, 128), F32),
            pltpu.VMEM((2 * NT, 8, 128), F32),
            pltpu.VMEM((H, 8, 128), F32),
            pltpu.VMEM((128, 256), F32),
            pltpu.SemaphoreType.DMA((30,)),
        ],
        compiler_params=pltpu.CompilerParams(
            dimension_semantics=("arbitrary", "arbitrary"),
            vmem_limit_bytes=110 * 2**20),
        name="interleave",
    )(A_x.reshape(S, D), B_beta.reshape(1, H), A_wqkv, A_wo, B_wq, B_wk, B_wv, B_wo)
    return out.reshape(1, S, D)
```

```python
import functools
import math

import jax
import jax.numpy as jnp
from jax import lax
from jax.experimental import pallas as pl
from jax.experimental.pallas import tpu as pltpu

S, D, H, DH = 2048, 1024, 32, 32
NSEG = 4
L = S // NSEG
W, DIL = 8, 2
HALO = 16
NT = D // 128
NPAIR = NT // 2
HD = D // 2
RC = 256
NCH = L // RC
NP = 7
PITCH = 17
WROWS = 16 * PITCH + 16
LOG2E = math.log2(math.e)
QSCALE = DH ** -0.5 * LOG2E
NEG = -1e9 * LOG2E
F32, BF16, U32 = jnp.float32, jnp.bfloat16, jnp.uint32

TUNE = dict(
    pace=((24, 1.05, 80, 0.75), (56, 1.1, 110, 0.1)),
    due_norm=(0, 2, 3, 4, 2, 2, 3),
    due_probs=(0, 0, 0, 0, 0, 0, 0, 0, 3, 3, 4, 5, 4, 4, 4, 4, 4, 4, 4, 4, 4, 4, 3, 3, 3, 0, 0, 0),
    due_mix0=(0, 0, 1, 5, 7, 5, 10),
    due_mix1=(0, 0, 4, 5, 4, 2, 0),
    due_norm0=(0, 0, 1, 1, 3, 0, 1),
    due_next=(0, 0, 1, 5, 1, 2, 10, 1, 2, 2, 0, 5, 3, 0),
    split=2,
    plan="f s0 f n s1 f p3 f f s2 p3 f p2 f s3 f p3 f p3 f p5 f f p3 f p3 f p3 f p3 f u "
         "/ s0 f s1 f n p4 f f p3 s2 f p2 o f s3 f p3 f p3 f p3 f f f f p3 f p3 f p3 f p3 f u o F",
    plan_last="f s0 s1 n p4 s2 f p4 f p3 s3 f p3 f p2 p2 f f p3 f p3 f p3 f f p3 f u "
              "/ s0 s1 f n f p3 s2 p3 f p3 o f s3 p5 f p3 p2 f f x p3 x p3 f f x p4 x p3 o f x f x u F X",
)


def _dot(a, b):
    return jnp.dot(a, b, preferred_element_type=F32)


def _dot_nt(a, b):
    return lax.dot_general(a, b, (((1,), (1,)), ((), ())), preferred_element_type=F32)


def _pack(x):
    return pltpu.bitcast(x.astype(BF16), U32)


def _unpack(x):
    return pltpu.bitcast(x, BF16)


def _tile(i):
    return slice(i * 128, (i + 1) * 128)


def _lhs_blocks(a11, a12, a21, a22):
    return [a11 + a22, a21 + a22, a11, a22, a11 + a12, a21 - a11, a12 - a22]


def _rhs_blocks(b11, b12, b21, b22):
    return [b11 + b22, b11, b12 - b22, b21 - b11, b22, b11 + b12, b21 + b22]


def _row_blocks(x):
    return _lhs_blocks(x[:128, :HD], x[:128, HD:], x[128:, :HD], x[128:, HD:])


def _block_matmul(prod, done):
    p3 = yield from prod(2)
    p5 = yield from prod(4)
    done(0, 1, p3 + p5)
    p2 = yield from prod(1)
    p4 = yield from prod(3)
    done(1, 0, p2 + p4)
    u, v = p4 - p5, p3 - p2
    p1 = yield from prod(0)
    u, v = u + p1, v + p1
    p7 = yield from prod(6)
    done(0, 0, u + p7)
    p6 = yield from prod(5)
    done(1, 1, v + p6)


def _whole(fn):
    def prod(i):
        y = fn(i)
        yield
        return y
    return prod


def _tiled(dot, nk, nn, tick):
    def prod(i):
        acc = [None] * nn
        for n in range(nn):
            for k in range(nk):
                t = dot(i, k, n)
                acc[n] = t if k == 0 else acc[n] + t
            tick(t)
            yield
        return jnp.concatenate(acc, axis=1)
    return prod


def _run(gen, n=None):
    k = 0
    while (n is None or k < n) and next(gen, "end") != "end":
        k += 1


def _chain(*gens):
    for g in gens:
        yield from g


def _layernorm(x):
    m = jnp.mean(x, axis=-1, keepdims=True)
    xc = x - m
    v = jnp.mean(xc * xc, axis=-1, keepdims=True)
    return xc * lax.rsqrt(v + 1e-5)


def _phi(t):
    return jnp.where(t > 0, t + 1.0, jnp.exp(t))


def _kernel(x_hbm, beta_ref, wqkv_hbm, woa_hbm, wq_hbm, wk_hbm, wv_hbm, wob_hbm, out_hbm,
            xin, xout, raw_a, raw_ao, raw_b, raw_bo, wa, woa, wqk, wvt, wob,
            xs, xa, xb, qb, kb, vb, kc, vc, of, oc, bq, bk, bv, mt, zs, gate, cmask, sems):
    seg = pl.program_id(0)
    rep = pl.program_id(1)
    first_step = (seg == 0) & (rep == 0)

    def window_copy(i):
        m, j = divmod(i, 2)
        if m < 3:
            c0 = (1, 0, 2)[m] * D + j * HD
            return pltpu.make_async_copy(wqkv_hbm.at[:, pl.ds(c0, HD)], raw_a.at[i], sems.at[i])
        return pltpu.make_async_copy(woa_hbm.at[pl.ds(j * HD, HD)], raw_ao.at[j], sems.at[i])

    def pair_copies(p):
        return [pltpu.make_async_copy(w.at[:, pl.ds(p * 256, 256)], raw_b.at[m, p], sems.at[8 + 3 * p + m])
                for m, w in enumerate((wq_hbm, wk_hbm, wv_hbm))]

    def late_copies():
        return ([c for p in range(1, NPAIR) for c in pair_copies(p)]
                + [pltpu.make_async_copy(wob_hbm, raw_bo, sems.at[20])])

    def x_copy(s):
        return pltpu.make_async_copy(x_hbm.at[pl.ds(pl.multiple_of(s * L, L), L)], xin, sems.at[21])

    def out_copy(s, ch, i, j):
        rows = pl.ds(pl.multiple_of(s * L + ch * RC + i * 128, 128), 128)
        n = ch * 4 + i * 2 + j
        return pltpu.make_async_copy(xout.at[n], out_hbm.at[rows, pl.ds(j * HD, HD)], sems.at[22 + n])

    def wait_out(s):
        for n in range(4 * NCH):
            out_copy(s, n // 4, n // 2 % 2, n % 2).wait()

    def selector(reorder):
        row = lax.broadcasted_iota(jnp.int32, (128, 128), 0)
        col = lax.broadcasted_iota(jnp.int32, (128, 128), 1)
        if reorder:
            row = (((row >> 5) & 1) * 2 + (row & 1)) * DH + (row >> 6) * 16 + ((row >> 1) & 15)
        return jnp.where(row == col, 1.0, 0.0).astype(BF16)

    def packed_blocks(*quad):
        quad = [pltpu.bitcast(b, U32) for b in quad]
        vals = [_unpack(b).astype(F32) for b in quad]
        out = []
        for blk in _rhs_blocks(*vals):
            same = [i for i, v in enumerate(vals) if v is blk]
            out.append(quad[same[0]] if same else _pack(blk))
        return out

    def arrive(piece, lo, hi):
        for i in range(lo, hi):
            @pl.when(piece == i)
            def _():
                window_copy(i).wait()
                for n in {0: (1,), 1: (2, 3, 4, 5)}.get(i, ()):
                    window_copy(n).start()

    def scatter(dst, t, blocks):
        for i, v in enumerate(blocks):
            v = _pack(v)
            for c in range(NPAIR):
                for hp in range(2):
                    dst(i, c)[pl.ds(t * 2 + hp, 16, stride=PITCH), :] = v[hp * 16:(hp + 1) * 16, _tile(c)]

    def prep_window_in(piece, carry):
        arrive(piece, 0, 6)
        for t in range(4):
            top = _dot_nt(selector(True), raw_a[piece, 0:HD, _tile(t)])
            bot = _dot_nt(selector(True), raw_a[piece, HD:D, _tile(t)])
            scatter(lambda i, c: wa.at[piece >> 1, i, c], (piece & 1) * 4 + t,
                    _rhs_blocks(top[:64], top[64:], bot[:64], bot[64:]))
        return carry

    def prep_window_out(j, carry):
        arrive(6 + j, 6, 8)
        for t in range(4):
            y = _dot(selector(True), raw_ao[j, _tile(t), :])
            scatter(lambda i, c: woa.at[i, c], j * 4 + t,
                    _rhs_blocks(y[:64, :HD], y[:64, HD:], y[64:, :HD], y[64:, HD:]))
        return carry

    def prep_pair(p, carry):
        quad = [_dot_nt(selector(False), raw_b[2, p, kh * HD:(kh + 1) * HD, _tile(e)])
                for kh in range(2) for e in range(2)]
        for i, v in enumerate(_rhs_blocks(*quad)):
            wvt[p, i] = _pack(v)

        def rows_qk(j, c):
            for m in range(2):
                quad = [raw_b[m, p, pl.ds(pl.multiple_of(kh * HD + j * 64, 64), 64), _tile(e)]
                        for kh in range(2) for e in range(2)]
                for i, v in enumerate(packed_blocks(*quad)):
                    wqk[p, i, pl.ds(pl.multiple_of(j * 32, 32), 32), _tile(m)] = v
            return c
        return lax.fori_loop(0, HD // 64, rows_qk, carry)

    def prep_memory_out(t, carry):
        r0 = (t // 4) * 256 + (t % 4) * 32
        quad = [raw_bo[pl.ds(pl.multiple_of(r0 + e * 128, 32), 32), c:c + HD] for e in range(2) for c in (0, HD)]
        for i, v in enumerate(packed_blocks(*quad)):
            wob[i, pl.ds(pl.multiple_of(t * 16, 16), 16), :] = v
        return carry

    @pl.when(first_step)
    def _start():
        window_copy(0).start()
        x_copy(0).start()
        kc[...] = jnp.zeros(kc.shape, F32)
        vc[...] = jnp.zeros(vc.shape, F32)
        mt[...] = jnp.zeros(mt.shape, F32)
        zs[...] = jnp.zeros(zs.shape, F32)
        g_all = jax.nn.sigmoid(beta_ref[...].astype(F32))
        head = lax.broadcasted_iota(jnp.int32, (1, H), 1)
        for h in range(H):
            gate[h] = jnp.broadcast_to(jnp.sum(jnp.where(head == h, g_all, 0.0), axis=1, keepdims=True), (8, 128))
        kk = lax.broadcasted_iota(jnp.int32, (128, 256), 0)
        qq = lax.broadcasted_iota(jnp.int32, (128, 256), 1)
        qq = jnp.where(kk >= 64, qq | 64, jnp.where(qq < 128, qq ^ 64, qq)) & 127
        cmask[...] = jnp.where(qq < kk, NEG, 0.0).astype(F32)
        prep_window_in(0, 0)
        x_copy(0).wait()

        def load_rows(j, carry):
            rows = pl.ds(pl.multiple_of(j * 64, 64), 64)
            later = pl.ds(pl.multiple_of(RC + j * 64, 64), 64)
            x0 = xin[rows, :].astype(F32)
            xs[rows, :] = x0
            xa[rows, :] = _layernorm(x0)
            xs[later, :] = xin[later, :].astype(F32)
            return carry
        lax.fori_loop(0, RC // 64, load_rows, 0)
        prep_window_in(1, 0)

    def _more_weights():
        for c in [window_copy(6), window_copy(7)] + pair_copies(0):
            c.start()
        lax.fori_loop(2, 6, prep_window_in, 0)
        lax.fori_loop(0, 2, prep_window_out, 0)
        for c in late_copies():
            c.start()
        for c in pair_copies(0):
            c.wait()
        prep_pair(0, 0)

    def _last_weights():
        for c in late_copies():
            c.wait()
        lax.fori_loop(1, NPAIR, prep_pair, 0)
        lax.fori_loop(0, HD // 32, prep_memory_out, 0)

    ticks = []

    def tick(y):
        ticks.extend(y[0:8, c:c + 128] for c in range(0, y.shape[1], 128))
        return y

    def never():
        return cmask[0:8, 0:128] > 1.0

    def after(t, x):
        return x if t < 0 else jnp.where(never(), ticks[min(t, len(ticks) - 1)], x)

    def before(deps, a):
        if not deps:
            return a
        dep = functools.reduce(jnp.maximum, deps)
        head = jnp.where(never(), dep if a.dtype == F32 else pltpu.bitcast(dep, a.dtype), a[0:8, 0:128])
        if a.shape[1] > 128:
            head = jnp.concatenate([head, a[0:8, 128:]], axis=1)
        return jnp.concatenate([head, a[8:]], axis=0)

    def held_for(blocks, counts, lhs):
        counts, seen = iter(counts), [0]

        def held(i):
            n = next(counts)
            deps = [b[r * 8:r * 8 + 8, _tile(c)] for r in range(seen[0], seen[0] + n)
                    for b in blocks[-2:] for c in range(NPAIR)]
            seen[0] += n
            return before(deps, lhs[i])
        return held

    def reordered(ref):
        w = jnp.concatenate([ref[:, d * PITCH:d * PITCH + 16, :] for d in range(16)], axis=1)
        return _unpack(jnp.concatenate([w[c] for c in range(NPAIR)], axis=1))

    def window_in(ch, m, lhs):
        dst, off = ((kb, HALO), (qb, 0), (vb, HALO))[m]

        def done(i, j, y):
            r0 = off + ch * RC + i * 128
            if m == 1:
                y = y * QSCALE
            for c in range(NPAIR):
                dst[j * NPAIR + c, r0:r0 + 128, :] = y[:, _tile(c)]
        return _block_matmul(
            _whole(lambda i: tick(_dot_nt(lhs(i).astype(BF16), reordered(wa.at[m, i])))), done)

    def taps(ref, r0, w, tiles=slice(None)):
        o0 = HALO + r0 - DIL * w
        return ref[tiles, o0:o0 + 8, :]

    def row_group(i):
        return i // 2 + (i % 2) * (RC // 16)

    @functools.cache
    def window_probs(ch, i):
        r0 = ch * RC + row_group(i) * 8
        t = int(TUNE["pace"][ch][0] + i * TUNE["pace"][ch][1])
        q = after(t, qb[:, r0:r0 + 8, :])
        logits = []
        for w in range(W):
            acc = jnp.sum(q * taps(kb, r0, w), axis=0)
            acc = acc + pltpu.roll(acc, 64, 1)
            acc = acc + pltpu.roll(acc, 32, 1)
            if r0 < DIL * w:
                pos = seg * L + r0 + lax.broadcasted_iota(jnp.int32, (8, 128), 0)
                acc = jnp.where(pos >= DIL * w, acc, NEG)
            logits.append(acc)
        mx = functools.reduce(jnp.maximum, logits)
        es = [jnp.exp2(v - mx) for v in logits]
        return es, 1.0 / functools.reduce(jnp.add, es)

    @functools.cache
    def window_rows(ch, i):
        r0 = ch * RC + row_group(i) * 8
        es, inv = window_probs(ch, i)
        inv = after(int(TUNE["pace"][ch][2] + i * TUNE["pace"][ch][3]), inv)
        ps = [e * inv for e in es]
        return jnp.concatenate([
            functools.reduce(jnp.add, [ps[w] * taps(vb, r0, w, slice(c, c + 2)) for w in range(W)])
            for c in range(0, NT, 2)], axis=0)

    def window_blocks(ch):
        rows = [None] * (RC // 8)
        for i in range(RC // 8):
            rows[row_group(i)] = window_rows(ch, i)
        o = jnp.concatenate(rows, axis=1)
        return _row_blocks(jnp.concatenate([o[c] for c in range(NT)], axis=1))

    def add_rows(ch):
        def done(i, j, y):
            r0 = ch * RC + i * 128
            xs[r0:r0 + 128, j * HD:(j + 1) * HD] += y
        return done

    def window_out(ch, lhs):
        return _block_matmul(
            _whole(lambda i: tick(_dot(lhs(i).astype(BF16), reordered(woa.at[i])))), add_rows(ch))

    def memory_qk(p, ch, lhs=None):
        def done(i, j, y):
            r0 = ch * RC + i * 128
            bq[(p & 1) * 2 + j, r0:r0 + 128, :] = y[:, :128]
            bk[(p & 1) * 2 + j, r0:r0 + 128, :] = y[:, 128:]
        if lhs is not None:
            return _block_matmul(_whole(lambda i: tick(_dot(_unpack(lhs[i]), _unpack(wqk[p, i])))), done)
        return _block_matmul(_tiled(
            lambda i, k, n: _dot(_unpack(xb[i, ch * 64:(ch + 1) * 64, _tile(k)]),
                                 _unpack(wqk[p, i, k * 64:(k + 1) * 64, _tile(n)])), 4, 2, tick), done)

    def memory_v(p):
        def done(i, j, y):
            for ch in range(NCH):
                c0 = ch * RC + i * 128
                bv[(p & 1) * 2 + j, :, c0:c0 + 128] = _pack(y[:, _tile(ch)])
        return _block_matmul(_tiled(
            lambda i, k, n: _dot_nt(_unpack(wvt[p, i, :, _tile(k)]),
                                    _unpack(xb[i, n * 64:(n + 1) * 64, _tile(k)])), 4, NCH, tick), done)

    def finish_rows(ch):
        def done(i, j, y):
            idx = (slice(ch * RC + i * 128, ch * RC + (i + 1) * 128), slice(j * HD, (j + 1) * HD))
            xnew = xs[idx] + y
            xout[ch * 4 + i * 2 + j] = xnew.astype(BF16)
            out_copy(seg, ch, i, j).start()
            xs[idx] = jnp.where(rep == 0, xnew, xin[idx].astype(F32))
        return done

    def memory_out(ch, p0, p1, hold=lambda a: a):
        def prod(i):
            acc = None
            for p in range(p0, p1):
                t = _dot(_unpack(hold(oc[p, i, ch * 64:(ch + 1) * 64, :])), _unpack(wob[i, p * 64:(p + 1) * 64, :]))
                acc = t if acc is None else acc + t
                tick(t[:, 0:128])
                yield
            return acc
        return _block_matmul(prod, finish_rows(ch) if p1 == NPAIR else add_rows(ch))

    lane_head = lax.broadcasted_iota(jnp.int32, (1, 128), 1) >> 5

    def head_queries(q, j):
        qh = [q[_tile(j), :] * jnp.where(lane_head == h, QSCALE, 0.0) for h in range(4)]
        return [(t[:64], t[64:]) for t in qh]

    def corner(q, k, j):
        qm = jnp.concatenate([hi for _, hi in head_queries(q, j)], axis=0)
        return _dot_nt(k[j * 128 + 64:(j + 1) * 128, :].astype(BF16), qm.astype(BF16))

    def scores(q, k, j, cor):
        nk = 128 * j + 64
        qm = jnp.concatenate([part for h, (lo, hi) in enumerate(head_queries(q, j))
                              for part in ((lo, hi) if h % 2 else (hi, lo))], axis=0)
        st = _dot_nt(k[0:nk, :].astype(BF16), qm.astype(BF16))
        for i in range(j + 1):
            tick(st[i * 128:i * 128 + 8, 0:128])
        diag = st[nk - 64:] + jnp.concatenate([cmask[0:64, :]] * 2, axis=1)
        st = diag if j == 0 else jnp.concatenate([st[:nk - 64], diag], axis=0)
        return st, cor + jnp.concatenate([cmask[64:128, 0:128]] * 2, axis=1)

    def memory_read(g, q):
        zrow = lax.broadcasted_iota(jnp.int32, (16, 128), 0)
        zl = jnp.where(zrow == lane_head, jnp.broadcast_to(zs[rep * NT + g, 0:1, :], (16, 128)), 0.0)
        return _dot_nt(jnp.concatenate([mt[rep * NT + g], zl], axis=0).astype(BF16), _phi(q[...]).astype(BF16))

    def memory_update(g, k, vt):
        pk = _phi(k[...])
        upd = functools.reduce(jnp.add, [
            _dot(_unpack(vt[:, _tile(i)]), pk[_tile(i)].astype(BF16)) for i in range(L // 128)])
        row_head = lax.broadcasted_iota(jnp.int32, (128, 128), 0) >> 5
        mt[rep * NT + g] += jnp.where(row_head == lane_head, upd, 0.0)
        zs[rep * NT + g] += jnp.sum(jnp.sum(pk.reshape(L // 64, 64, 128), axis=0), axis=0, keepdims=True)

    def attend(g, e, j, st, nd, vt, lag):
        st, cor = st
        low = lax.broadcasted_iota(jnp.int32, (1, 128), 1) < 64
        own = [low if h % 2 == 0 else ~low for h in range(4)]
        mc = jnp.max(cor.reshape(8, 8, 256), axis=0)
        mx = jnp.max(st.reshape(-1, 8, 512), axis=0)
        mx = jnp.concatenate([jnp.where(own[h], jnp.maximum(mx[:, _tile(h)], mc[:, _tile(h // 2)]), mx[:, _tile(h)])
                              for h in range(4)], axis=1)
        mx = jnp.broadcast_to(jnp.max(mx, axis=0, keepdims=True), (8, 512))
        pv, l = [None] * 4, None
        for i in range(j + 1):
            mi = [after(len(ticks) - lag[0], mx[:, _tile(h)]) for h in range(4)]
            n = 128 if i < j else 64
            p3 = jnp.exp2(st[i * 128:i * 128 + n].reshape(n // 8, 8, 512) - jnp.concatenate(mi, axis=1))
            if i == j:
                pc = jnp.exp2(cor.reshape(8, 8, 256) - jnp.concatenate(
                    [jnp.where(low, mi[h], mi[h + 1]) for h in (0, 2)], axis=1))
                p3 = jnp.concatenate([p3, jnp.concatenate(
                    [jnp.where(own[h], pc[:, :, _tile(h // 2)], 0.0) for h in range(4)], axis=2)], axis=0)
            p = p3.reshape(128, 512)
            li = jnp.sum(p3, axis=0)
            l = li if i == 0 else l + li
            for h in range(4):
                t = _dot(_unpack(vt[h * 16:(h + 1) * 16, _tile(i)]), p[:, _tile(h)].astype(BF16))
                pv[h] = t if i == 0 else pv[h] + t
            if i < j:
                yield
        l = jnp.sum(l, axis=0, keepdims=True)
        rows = []
        for h in range(4):
            gh = gate[g * 4 + h][0:1, :]
            num = nd[h * DH:(h + 1) * DH, _tile(j)]
            den = nd[128 + h:129 + h, _tile(j)] + 1e-6
            loc = pv[h] * ((1.0 - gh) / l[:, _tile(h)])
            rows.append(num * (gh / den) + (loc if h % 2 else pltpu.roll(loc, 64, 1)))
        of[e, _tile(j), :] = jnp.concatenate(rows, axis=0).T
        yield

    def keep_output(p, ch):
        r0 = ch * RC
        blocks = _lhs_blocks(of[0, r0:r0 + 128, :], of[1, r0:r0 + 128, :],
                             of[0, r0 + 128:r0 + 256, :], of[1, r0 + 128:r0 + 256, :])
        for i, b in enumerate(blocks):
            oc[p, i, ch * 64:(ch + 1) * 64, :] = _pack(b)

    def memory_pair(p, last):
        del ticks[:]
        if last:
            fill = _chain(memory_out(0, 0, p), memory_out(1, 0, TUNE["split"]))
            tail = memory_out(0, p, NPAIR)
        else:
            fill = _chain(memory_qk(p + 1, 0), memory_qk(p + 1, 1), memory_v(p + 1))
        for e, steps in enumerate(TUNE["plan_last" if last else "plan"].split("/")):
            g = 2 * p + e
            q, k, vt = (ref.at[(p & 1) * 2 + e] for ref in (bq, bk, bv))
            todo, cur, nd, seen, corners, lag = [], None, None, [], {}, [0]
            for op in steps.split():
                if op == "f":
                    _run(fill, 1)
                elif op == "F":
                    _run(fill)
                elif op == "x":
                    _run(tail, 1)
                elif op == "X":
                    _run(tail)
                elif op[0] == "s":
                    j = int(op[1])
                    if j not in corners:
                        corners.update({i: corner(q, k, i) for i in (j, j ^ 1)})
                    todo.append((j, scores(q, k, j, corners[j])))
                elif op == "n":
                    nd = memory_read(g, q)
                elif op == "u":
                    memory_update(g, k, vt)
                elif op == "o":
                    keep_output(p, seen[-1] // 2)
                else:
                    lag[0] = int(op[1])
                    if cur is None or next(cur, "end") == "end":
                        j, st = todo.pop(0)
                        seen.append(j)
                        cur = attend(g, e, j, st, nd, vt, lag)
                        next(cur)
            assert len(seen) == L // 128 and next(cur, "end") == "end"
        return 0

    fetch_next = (rep == 1) & (seg < NSEG - 1)
    pl.when(fetch_next)(lambda: x_copy(seg + 1).start())

    def keys_stage():
        for c in range(NT):
            kb[c, 0:HALO, :] = kc[rep, c]
            vb[c, 0:HALO, :] = vc[rep, c]
        xn1 = _layernorm(xs[RC:L, :])
        xa[RC:L, :] = xn1
        in0, in1 = _row_blocks(xa[0:RC, :]), _row_blocks(xn1)
        _run(window_in(0, 0, held_for(in1, TUNE["due_norm"], in0)))
        _run(window_in(1, 0, lambda i: in1[i]))

    def window_stage():
        del ticks[:]
        a_in = [_row_blocks(xa[ch * RC:(ch + 1) * RC, :]) for ch in range(NCH)]
        due_probs, due_mix = iter(TUNE["due_probs"]), iter((0,) * (3 * NP) + TUNE["due_mix0"])
        seen = [0, 0]

        def held(ch, i):
            n, n2 = next(due_probs), next(due_mix)
            deps = [window_probs(*divmod(r, RC // 8))[1] for r in range(seen[0], seen[0] + n)]
            deps += [window_rows(0, r)[c] for r in range(seen[1], seen[1] + n2) for c in range(NT)]
            seen[0] += n
            seen[1] += n2
            return before(deps, a_in[ch][i])
        for ch, m in ((0, 1), (1, 1), (0, 2), (1, 2)):
            _run(window_in(ch, m, functools.partial(held, ch)))
        o0, o1 = window_blocks(0), window_blocks(1)
        _run(window_out(0, held_for(o1, TUNE["due_mix1"], o0)))

        def memory_in(ch):
            blocks = [_pack(b) for b in _row_blocks(_layernorm(xs[ch * RC:(ch + 1) * RC, :]))]
            for i, b in enumerate(blocks):
                xb[i, ch * 64:(ch + 1) * 64, :] = b
            return blocks
        x0 = memory_in(0)
        _run(window_out(1, held_for([pltpu.bitcast(b, F32) for b in x0], TUNE["due_norm0"], o1)))
        for ch, blocks in enumerate((x0, memory_in(1))):
            _run(memory_qk(0, ch, blocks))
        _run(memory_v(0))
        for c in range(NT):
            kc[rep, c] = kb[c, L:L + HALO, :]
            vc[rep, c] = vb[c, L:L + HALO, :]

    def last_stage():
        memory_pair(NPAIR - 1, True)
        xn0 = _layernorm(xs[0:RC, :])
        xa[0:RC, :] = xn0
        counts, seen = iter(TUNE["due_next"]), [0]

        def hold(a):
            n = next(counts)
            deps = [xn0[r * 8:r * 8 + 8, _tile(c)] for r in range(seen[0], seen[0] + n) for c in (0, NT - 1)]
            seen[0] += n
            return before(deps, a)
        _run(memory_out(1, TUNE["split"], NPAIR, hold))

    keys_stage()
    pl.when(first_step)(_more_weights)
    window_stage()
    pl.when(first_step)(_last_weights)
    pl.when(jnp.logical_not(first_step))(lambda: wait_out(seg - 1 + rep))
    pl.when(fetch_next)(lambda: x_copy(seg + 1).wait())
    lax.fori_loop(0, NPAIR - 1, lambda p, carry: memory_pair(p, False), 0)
    last_stage()
    pl.when((seg == NSEG - 1) & (rep == 1))(lambda: wait_out(seg))


@jax.jit
def pallas_interleave_layers__sliding_local_dilated__memory_aug_infini_attn__prompt_kernel(
        A_x, A_wqkv, A_wo, B_x, B_wq, B_wk, B_wv, B_wo, B_beta):
    del B_x
    hbm = pl.BlockSpec(memory_space=pl.ANY)
    out = pl.pallas_call(
        _kernel,
        grid=(NSEG, 2),
        in_specs=[hbm, pl.BlockSpec((1, H), lambda s, r: (0, 0)), hbm, hbm, hbm, hbm, hbm, hbm],
        out_specs=hbm,
        out_shape=jax.ShapeDtypeStruct((S, D), BF16),
        scratch_shapes=[
            pltpu.VMEM((L, D), BF16),
            pltpu.VMEM((4 * NCH, 128, HD), BF16),
            pltpu.VMEM((6, D, HD), BF16),
            pltpu.VMEM((2, HD, D), BF16),
            pltpu.VMEM((3, NPAIR, D, 256), BF16),
            pltpu.VMEM((D, D), BF16),
            pltpu.VMEM((3, NP, NPAIR, WROWS, 128), U32),
            pltpu.VMEM((NP, NPAIR, WROWS, 128), U32),
            pltpu.VMEM((NPAIR, NP, HD // 2, 256), U32),
            pltpu.VMEM((NPAIR, NP, 64, HD), U32),
            pltpu.VMEM((NP, HD // 2, HD), U32),
            pltpu.VMEM((L, D), F32),
            pltpu.VMEM((L, D), F32),
            pltpu.VMEM((NP, L // 4, HD), U32),
            pltpu.VMEM((NT, L, 128), F32),
            pltpu.VMEM((NT, HALO + L, 128), F32),
            pltpu.VMEM((NT, HALO + L, 128), F32),
            pltpu.VMEM((2, NT, HALO, 128), F32),
            pltpu.VMEM((2, NT, HALO, 128), F32),
            pltpu.VMEM((2, L, 128), F32),
            pltpu.VMEM((NPAIR, NP, L // 4, 128), U32),
            pltpu.VMEM((4, L, 128), F32),
            pltpu.VMEM((4, L, 128), F32),
            pltpu.VMEM((4, 64, L), U32),
            pltpu.VMEM((2 * NT, 128, 128), F32),
            pltpu.VMEM((2 * NT, 8, 128), F32),
            pltpu.VMEM((H, 8, 128), F32),
            pltpu.VMEM((128, 256), F32),
            pltpu.SemaphoreType.DMA((30,)),
        ],
        compiler_params=pltpu.CompilerParams(
            dimension_semantics=("arbitrary", "arbitrary"),
            vmem_limit_bytes=110 * 2**20),
        name="interleave",
    )(A_x.reshape(S, D), B_beta.reshape(1, H), A_wqkv, A_wo, B_wq, B_wk, B_wv, B_wo)
    return out.reshape(1, S, D)
```
